```python
import jax
import jax.numpy as jnp

def _softmax(x, axis=-1):
    return jax.nn.softmax(x, axis=axis)

def _gelu(x):
    return jax.nn.gelu(x, approximate=True)

def _silu(x):
    return jax.nn.silu(x)

def _sigmoid(x):
    return jax.nn.sigmoid(x)

def _layernorm(x, axis=-1, eps=1e-05):
    m = jnp.mean(x, axis=axis, keepdims=True)
    v = jnp.var(x, axis=axis, keepdims=True)
    return (x - m) / jnp.sqrt(v + eps)

def _scatter_add(tgt, idx, src, axis=0):
    return tgt.at[idx].add(src)

def _segment_sum(src, seg, n):
    return jax.ops.segment_sum(src, seg, n)

class _Rng:

    def __init__(self, key):
        self._k = key

    def _next(self):
        self._k, sub = jax.random.split(self._k)
        return sub

    def normal(self, shape):
        return jax.random.normal(self._next(), shape, dtype=jnp.bfloat16)

    def randint(self, lo, hi, shape):
        return jax.random.randint(self._next(), shape, lo, hi, dtype=jnp.int32)

    def uniform(self, shape, lo=0.0, hi=1.0):
        return jax.random.uniform(self._next(), shape, jnp.bfloat16, lo, hi)

    def permutation(self, n):
        return jax.random.permutation(self._next(), n)
kernel_name = 'concat_heads__memory_aug_recurrent_mem_tr__compressed_kv_cla__prompt'

def setup_inputs():
    _rng = _Rng(jax.random.key(int.from_bytes(__import__("os").urandom(4), "little")))
    _w = lambda a: (lambda t: t.astype(jnp.bfloat16) if jnp.issubdtype(t.dtype, jnp.floating) else t)(jnp.asarray(a))

    def _A_setup():
        B, S, Dm = (1, 2048, 448)
        H, Dh = (16, 256)
        M, seg = (8, 32)
        seg = min(seg, S)
        S = S // seg * seg
        return {'x': _w((lambda *s: _rng.normal(s) * 0.05)(B, S, Dm)), 'mem0': _w((lambda *s: _rng.normal(s) * 0.05)(B, M, Dm)), 'Wq': _w((lambda *s: _rng.normal(s) * 0.05)(Dm, H, Dh) * Dm ** (-0.5)), 'Wk': _w((lambda *s: _rng.normal(s) * 0.05)(Dm, H, Dh) * Dm ** (-0.5)), 'Wv': _w((lambda *s: _rng.normal(s) * 0.05)(Dm, H, Dh) * Dm ** (-0.5)), 'Wo': _w((lambda *s: _rng.normal(s) * 0.05)(H, Dh, Dm) * (H * Dh) ** (-0.5)), 'seg_len': seg}
    _A_in = _A_setup()

    def _B_setup():
        B, H, Sq, Sk, D, M = (1, 16, 2048, 2048, 256, 448)
        Dc = 4 * D
        return {'x': _w((lambda *s: _rng.normal(s) * 0.05)(B, Sq, M)), 'c_kv': _w((lambda *s: _rng.normal(s) * 0.05)(B, Sk, Dc)), 'w_q': _w((lambda *s: _rng.normal(s) * 0.05)(M, H, D) * M ** (-0.5)), 'w_uk': _w((lambda *s: _rng.normal(s) * 0.05)(Dc, H, D) * Dc ** (-0.5)), 'w_uv': _w((lambda *s: _rng.normal(s) * 0.05)(Dc, H, D) * Dc ** (-0.5)), 'w_o': _w((lambda *s: _rng.normal(s) * 0.05)(H, D, M) * (H * D) ** (-0.5))}
    _B_in = _B_setup()
    return {'A_x': _A_in['x'], 'A_mem0': _A_in['mem0'], 'A_Wq': _A_in['Wq'], 'A_Wk': _A_in['Wk'], 'A_Wv': _A_in['Wv'], 'A_Wo': _A_in['Wo'], 'A_seg_len': _A_in['seg_len'], 'B_x': _B_in['x'], 'B_c_kv': _B_in['c_kv'], 'B_w_q': _B_in['w_q'], 'B_w_uk': _B_in['w_uk'], 'B_w_uv': _B_in['w_uv'], 'B_w_o': _B_in['w_o']}

def reference(A_x, A_mem0, A_Wq, A_Wk, A_Wv, A_Wo, A_seg_len, B_x, B_c_kv, B_w_q, B_w_uk, B_w_uv, B_w_o):

    def _A_ref(x, mem0, Wq, Wk, Wv, Wo, seg_len):
        B, S, Dm = x.shape
        H, Dh = (Wq.shape[1], Wq.shape[2])
        M = mem0.shape[1]
        scale = Dh ** (-0.5)
        n_seg = S // seg_len
        L = M + seg_len
        idx = jnp.arange(L)
        mask = (idx[:, None] < M) | (idx[:, None] >= idx[None, :])
        mem = mem0
        outs = []
        for s in range(n_seg):
            xs = x[:, s * seg_len:(s + 1) * seg_len, :].copy()
            h = jnp.concatenate([mem, xs], axis=1)
            q = jnp.einsum('btd,dhe->bhte', h, Wq)
            k = jnp.einsum('btd,dhe->bhte', h, Wk)
            v = jnp.einsum('btd,dhe->bhte', h, Wv)
            scores = jnp.einsum('bhqe,bhke->bhqk', q, k) * scale
            scores = jnp.where(mask[None, None], scores, -1000000000.0)
            p = _softmax(scores, axis=-1)
            o = jnp.einsum('bhqk,bhke->bhqe', p, v)
            o = jnp.einsum('bhte,hed->btd', o, Wo)
            mem = o[:, :M, :].copy()
            outs.append(o[:, M:, :])
        return jnp.concatenate(outs, axis=1)

    def _B_ref(x, c_kv, w_q, w_uk, w_uv, w_o):
        B, Sq, M = (x.shape[0], x.shape[1], x.shape[2])
        Sk = c_kv.shape[1]
        H, D = (w_q.shape[1], w_q.shape[2])
        q = jnp.einsum('bqm,mhd->bhqd', x, w_q)
        k = jnp.einsum('bkc,chd->bhkd', c_kv, w_uk)
        v = jnp.einsum('bkc,chd->bhkd', c_kv, w_uv)
        scores = jnp.einsum('bhqd,bhkd->bhqk', q, k) * D ** (-0.5)
        off = Sk - Sq
        qi = jnp.arange(Sq)[:, None]
        kj = jnp.arange(Sk)[None, :]
        cmask = kj <= qi + off
        scores = jnp.where(cmask[None, None], scores, -1000000000.0)
        p = _softmax(scores, axis=-1)
        ctx = jnp.einsum('bhqk,bhkd->bhqd', p, v)
        return jnp.einsum('bhqd,hdm->bqm', ctx, w_o)
    a = _A_ref(A_x, A_mem0, A_Wq, A_Wk, A_Wv, A_Wo, A_seg_len)
    b = _B_ref(B_x, B_c_kv, B_w_q, B_w_uk, B_w_uv, B_w_o)
    return jnp.concatenate([a, b], axis=-1)
```

```python
import numpy as np
import jax
import jax.numpy as jnp
import jax.experimental.pallas as pl
import jax.experimental.pallas.tpu as pltpu

F32 = jnp.float32
BF16 = jnp.bfloat16
U32 = jnp.uint32
LOG2E = 1.4426950408889634
NEG = -1e30
NT = (((1,), (1,)), ((), ()))


def _dot(a, b):
    return jnp.dot(a, b, preferred_element_type=F32)


def _dot_nt(a, b):
    return jax.lax.dot_general(a, b, NT, preferred_element_type=F32)


def _unpack(u, parity):
    if isinstance(parity, int):
        w = (u << 16) if parity == 0 else (u & jnp.uint32(0xFFFF0000))
    else:
        w = (u >> (16 * parity).astype(U32)) << 16
    return pltpu.bitcast(w, F32).astype(BF16)


def _interleave(ga, na, gb, nb):
    ia = ib = 0
    while ia < na or ib < nb:
        if ib >= nb or (ia < na and ia * nb <= ib * na):
            next(ga, None)
            ia += 1
        else:
            next(gb, None)
            ib += 1
    for _ in ga:
        pass
    for _ in gb:
        pass


def _count(gen):
    return sum(1 for _ in gen)


def _make_kernel(S, DM, H, DH, M, SEG, DC):
    NP = H // 2
    NSEG = S // SEG
    DP = 512
    PW = 2 * DM
    STEPS = NSEG // H
    QB = 128

    def kernel(ax_h, mem_h, awq_h, awk_h, awv_h, awo_h, bx_h, ckv_h, bwq_h, bwk_h, bwv_h, bwo_h,
               out_h,
               xraw, he, xo, mem0, memall, awq, awk, awv, awo, wqk, wvo, qa,
               bx, ckv, bwq, bwk, bwv, bwo,
               wq_s, wk_s, wv_s, q_s, k_s, v_s, acca, accb, ostage,
               sem_x, sem_aq, sem_ak, sem_av, sem_ao, sem_bq, sem_bk, sem_bv, sem_bo, sem_out):

        def pair_copy(src, dst, sem, i):
            return pltpu.make_async_copy(src.bitcast(U32).at[:, i, :], dst.at[i], sem.at[i])

        def wo_copy(src, dst, sem, i):
            return pltpu.make_async_copy(src.at[pl.ds(2 * i, 2)], dst.at[pl.ds(2 * i, 2)], sem.at[i])

        cp_ax = pltpu.make_async_copy(ax_h.at[0], xraw, sem_x.at[0])
        cp_mem = pltpu.make_async_copy(mem_h.at[0], mem0, sem_x.at[1])
        cp_bx = pltpu.make_async_copy(bx_h.at[0], bx, sem_x.at[2])
        cp_ckv = pltpu.make_async_copy(ckv_h.at[0], ckv, sem_x.at[3])

        cp_ax.start()
        cp_mem.start()
        for i in range(NP):
            pair_copy(awq_h, awq, sem_aq, i).start()
        for i in range(NP):
            pair_copy(awk_h, awk, sem_ak, i).start()
            pair_copy(awv_h, awv, sem_av, i).start()
            wo_copy(awo_h, awo, sem_ao, i).start()
        cp_bx.start()
        cp_ckv.start()
        for i in range(NP):
            pair_copy(bwq_h, bwq, sem_bq, i).start()
            pair_copy(bwk_h, bwk, sem_bk, i).start()
            pair_copy(bwv_h, bwv, sem_bv, i).start()
            wo_copy(bwo_h, bwo, sem_bo, i).start()

        accb[...] = jnp.zeros(accb.shape, F32)
        acca[...] = jnp.zeros(acca.shape, F32)

        cp_ax.wait()

        def pad_body(r, c):
            rows = pl.ds(pl.multiple_of(r * 256, 256), 256)
            x = xraw[rows, :].astype(F32)
            xe = jnp.concatenate([x, jnp.zeros((256, DP - DM), F32)], axis=1)
            he[rows, :] = xe.astype(BF16)
            xo[rows, :] = pltpu.roll(xe, DP - DM, 1).astype(BF16)
            return c
        with jax.named_scope('pad_body'):
            jax.lax.fori_loop(0, S // 256, pad_body, 0)

        def qa_body(i, c):
            pair_copy(awq_h, awq, sem_aq, i).wait()
            u = awq[i]
            for par in range(2):
                w = _unpack(u, par)
                for r in range(S // 512):
                    rows = pl.ds(r * 512, 512)
                    qa[2 * i + par, rows, :] = (_dot(he[rows, :DM], w) * (LOG2E * DH ** -0.5)).astype(BF16)
            return c
        with jax.named_scope('qa_body'):
            jax.lax.fori_loop(0, NP, qa_body, 0)

        def absorb_body(i, c):
            pair_copy(awk_h, awk, sem_ak, i).wait()
            pair_copy(awv_h, awv, sem_av, i).wait()
            wo_copy(awo_h, awo, sem_ao, i).wait()
            uq, uk, uv = awq[i], awk[i], awv[i]
            zpad = jnp.zeros((DP - DM, DH), BF16)
            sc = LOG2E * DH ** -0.5
            e = _dot_nt(_unpack(uq, 0), jnp.concatenate([_unpack(uk, 0), zpad], axis=0)) * sc
            o = _dot_nt(_unpack(uq, 1), jnp.concatenate([zpad, _unpack(uk, 1)], axis=0)) * sc
            slab = jnp.concatenate([e[:, :DP - 128], e[:, DP - 128:] + o[:, :128], o[:, 128:]], axis=1)
            wqk[i] = slab.astype(BF16)
            for par in range(2):
                r = _dot(_unpack(uv, par), awo[2 * i + par])
                r = jnp.concatenate([r, jnp.zeros((DM, DP - DM), F32)], axis=1)
                wvo[i, pl.ds(par * DM, DM), :] = r.astype(BF16)
            return c
        with jax.named_scope('absorb_body'):
            jax.lax.fori_loop(0, NP, absorb_body, 0)

        cp_mem.wait()
        memall[pl.ds(0, M), :] = jnp.concatenate([mem0[...].astype(F32), jnp.zeros((M, DP - DM), F32)], axis=1)
        cp_bx.wait()
        cp_ckv.wait()

        def chain_step(s):
            mem = memall[pl.ds(pl.multiple_of(s * M, M), M), :]
            mb = mem.astype(BF16)
            rows = []
            for i in range(NP):
                tiles = []
                for n0, n1 in ((0, 256), (256, 512), (512, PW)):
                    acc = None
                    for k0, k1 in ((0, 256), (256, DM)):
                        d = _dot(mb[:, k0:k1], wqk[i, k0:k1, n0:n1])
                        acc = d if acc is None else acc + d
                        yield
                    tiles.append(acc)
                t = jnp.concatenate(tiles, axis=1)
                rows.append(t[:, :DP])
                rows.append(t[:, PW - DP:])
            tq = jnp.concatenate(rows, axis=0).astype(BF16)
            xr = pl.ds(pl.multiple_of(s * SEG, SEG), SEG)
            z8 = jnp.zeros((16 - M, DP), F32)
            keys = jnp.concatenate([
                he[xr, :], jnp.concatenate([mem, z8], axis=0).astype(BF16),
                xo[xr, :], jnp.concatenate([pltpu.roll(mem, DP - DM, 1), z8], axis=0).astype(BF16),
            ], axis=0)
            sc = _dot_nt(tq, keys)
            yield
            kw = SEG + 16
            ri = jax.lax.broadcasted_iota(jnp.int32, sc.shape, 0)
            ci = jax.lax.broadcasted_iota(jnp.int32, sc.shape, 1)
            lo = ((ri // M) % 2) * kw
            sc = jnp.where((ci >= lo) & (ci < lo + SEG + M), sc, NEG)
            p = jnp.exp2(sc - jnp.max(sc, axis=1, keepdims=True))
            p = p / jnp.sum(p, axis=1, keepdims=True)
            z = _dot(p.astype(BF16), keys)
            yield
            acc = [None, None]
            for i in range(NP):
                ze = z[2 * i * M:(2 * i + 1) * M]
                zo = z[(2 * i + 1) * M:(2 * i + 2) * M]
                zp = jnp.concatenate([ze[:, :DP - 128], ze[:, DP - 128:] + zo[:, :128], zo[:, 128:]],
                                     axis=1).astype(BF16)
                for k0, k1 in ((0, 256), (256, 512), (512, PW)):
                    for n in range(2):
                        d = _dot(zp[:, k0:k1], wvo[i, k0:k1, n * 256:(n + 1) * 256])
                        acc[n] = d if acc[n] is None else acc[n] + d
                        yield
            new = jnp.concatenate(acc, axis=1).astype(BF16).astype(F32)
            memall[pl.ds(pl.multiple_of((s + 1) * M, M), M), :] = new

        def chain(h):
            for j in range(STEPS):
                yield from chain_step(h * STEPS + j)

        def b_head(h):
            i = h // 2
            par = h % 2
            wq_s[...] = _unpack(bwq[i], par)
            wk_s[...] = _unpack(bwk[i], par)
            wv_s[...] = _unpack(bwv[i], par)
            for w_s, dst in ((wk_s, k_s), (wv_s, v_s)):
                for r in range(S // QB):
                    rows = pl.ds(r * QB, QB)
                    acc = None
                    for k0 in range(0, DC, 256):
                        d = _dot(ckv[rows, k0:k0 + 256], w_s[k0:k0 + 256, :])
                        acc = d if acc is None else acc + d
                        yield
                    dst[rows, :] = acc.astype(BF16)
            for r in range(S // QB):
                rows = pl.ds(r * QB, QB)
                acc = None
                for k0, k1 in ((0, 256), (256, DM)):
                    d = _dot(bx[rows, k0:k1], wq_s[k0:k1, :])
                    acc = d if acc is None else acc + d
                    yield
                q = (acc * (LOG2E * DH ** -0.5)).astype(BF16)
                nk = (r + 1) * QB
                chunks = [(c0, min(c0 + 256, nk)) for c0 in range(0, nk, 256)]
                ss = []
                for c0, c1 in chunks:
                    sc = _dot_nt(q, k_s[c0:c1, :])
                    if c1 == nk:
                        ri = jax.lax.broadcasted_iota(jnp.int32, sc.shape, 0) + r * QB
                        ci = jax.lax.broadcasted_iota(jnp.int32, sc.shape, 1) + c0
                        sc = jnp.where(ci <= ri, sc, NEG)
                    ss.append(sc)
                    yield
                m = None
                for sc in ss:
                    for t0 in range(0, sc.shape[1], 128):
                        m = sc[:, t0:t0 + 128] if m is None else jnp.maximum(m, sc[:, t0:t0 + 128])
                m = jnp.max(m, axis=1, keepdims=True)
                l = None
                acc = None
                for (c0, c1), sc in zip(chunks, ss):
                    p = jnp.exp2(sc - m)
                    for t0 in range(0, p.shape[1], 128):
                        l = p[:, t0:t0 + 128] if l is None else l + p[:, t0:t0 + 128]
                    d = _dot(p.astype(BF16), v_s[c0:c1, :])
                    acc = d if acc is None else acc + d
                    yield
                ctx = (acc / jnp.sum(l, axis=1, keepdims=True)).astype(BF16)
                for n0, n1 in ((0, 256), (256, DM)):
                    accb[rows, n0:n1] += _dot(ctx, bwo[h, :, n0:n1])
                    yield

        n_chain = STEPS * (NP * 6 * 2 + 2)
        n_head = (S // QB) * (2 * DC // 256 + 4) + 2 * sum((r + 2) // 2 for r in range(S // QB))

        def b_body(h, c):
            i = h // 2

            @pl.when(h % 2 == 0)
            def _():
                pair_copy(bwq_h, bwq, sem_bq, i).wait()
                pair_copy(bwk_h, bwk, sem_bk, i).wait()
                pair_copy(bwv_h, bwv, sem_bv, i).wait()
                wo_copy(bwo_h, bwo, sem_bo, i).wait()
            _interleave(chain(h), n_chain, b_head(h), n_head)
            return c
        with jax.named_scope('b_body'):
            jax.lax.fori_loop(0, H, b_body, 0)

        he[pl.ds(S, NSEG * M), :] = memall[pl.ds(0, NSEG * M), :].astype(BF16)
        AB = 2 * SEG
        ri = jax.lax.broadcasted_iota(jnp.int32, (AB, AB + 2 * M), 0)
        ci = jax.lax.broadcasted_iota(jnp.int32, (AB, AB + 2 * M), 1)
        amask = ((ci < AB) & ((ci // SEG) == (ri // SEG)) & (ci <= ri)) | ((ci >= AB) & (((ci - AB) // M) == (ri // SEG)))

        def a_body(h, c):
            i = h // 2
            par = h % 2
            wk = _unpack(awk[i], par)
            wv = _unpack(awv[i], par)
            for r in range((S + NSEG * M) // 512):
                rows = pl.ds(r * 512, 512)
                k_s[rows, :] = _dot(he[rows, :DM], wk).astype(BF16)
                v_s[rows, :] = _dot(he[rows, :DM], wv).astype(BF16)
            for r in range(S // 512):
                ctxs = []
                for j in range(r * 512 // AB, (r + 1) * 512 // AB):
                    xr = pl.ds(j * AB, AB)
                    mr = pl.ds(S + j * 2 * M, 2 * M)
                    kc = jnp.concatenate([k_s[xr, :], k_s[mr, :]], axis=0)
                    vc = jnp.concatenate([v_s[xr, :], v_s[mr, :]], axis=0)
                    sc = jnp.where(amask, _dot_nt(qa[h, xr, :], kc), NEG)
                    p = jnp.exp2(sc - jnp.max(sc, axis=1, keepdims=True))
                    p = p / jnp.sum(p, axis=1, keepdims=True)
                    ctxs.append(_dot(p.astype(BF16), vc).astype(BF16))
                rows = pl.ds(r * 512, 512)
                acca[rows, :] += _dot(jnp.concatenate(ctxs, axis=0), awo[h])
            return c
        with jax.named_scope('a_body'):
            jax.lax.fori_loop(0, H, a_body, 0)

        cps = []
        for r in range(S // 512):
            rows = pl.ds(r * 512, 512)
            ostage[rows, :] = jnp.concatenate([acca[rows, :], accb[rows, :]], axis=1).astype(BF16)
            cp = pltpu.make_async_copy(ostage.at[rows, :], out_h.at[0, rows, :], sem_out.at[r])
            cp.start()
            cps.append(cp)
        for cp in cps:
            cp.wait()

    scratch = [
        pltpu.VMEM((S, DM), BF16),
        pltpu.VMEM((S + NSEG * M, DP), BF16),
        pltpu.VMEM((S, DP), BF16),
        pltpu.VMEM((M, DM), BF16),
        pltpu.VMEM(((NSEG + 1) * M, DP), F32),
        pltpu.VMEM((NP, DM, DH), U32),
        pltpu.VMEM((NP, DM, DH), U32),
        pltpu.VMEM((NP, DM, DH), U32),
        pltpu.VMEM((H, DH, DM), BF16),
        pltpu.VMEM((NP, DM, PW), BF16),
        pltpu.VMEM((NP, PW, DP), BF16),
        pltpu.VMEM((H, S, DH), BF16),
        pltpu.VMEM((S, DM), BF16),
        pltpu.VMEM((S, DC), BF16),
        pltpu.VMEM((NP, DM, DH), U32),
        pltpu.VMEM((NP, DC, DH), U32),
        pltpu.VMEM((NP, DC, DH), U32),
        pltpu.VMEM((H, DH, DM), BF16),
        pltpu.VMEM((DM, DH), BF16),
        pltpu.VMEM((DC, DH), BF16),
        pltpu.VMEM((DC, DH), BF16),
        pltpu.VMEM((S, DH), BF16),
        pltpu.VMEM((S + NSEG * M, DH), BF16),
        pltpu.VMEM((S + NSEG * M, DH), BF16),
        pltpu.VMEM((S, DM), F32),
        pltpu.VMEM((S, DM), F32),
        pltpu.VMEM((S, 2 * DM), BF16),
        pltpu.SemaphoreType.DMA((4,)),
    ] + [pltpu.SemaphoreType.DMA((NP,)) for _ in range(8)] + [pltpu.SemaphoreType.DMA((S // 512,))]
    return kernel, scratch


@jax.jit
def pallas_concat_heads__memory_aug_recurrent_mem_tr__compressed_kv_cla__prompt_kernel(
    A_x, A_mem0, A_Wq, A_Wk, A_Wv, A_Wo, A_seg_len, B_x, B_c_kv, B_w_q, B_w_uk, B_w_uv, B_w_o,
):
    del A_seg_len
    _, S, DM = A_x.shape
    M = A_mem0.shape[1]
    H, DH = A_Wq.shape[1], A_Wq.shape[2]
    DC = B_c_kv.shape[2]
    kernel, scratch = _make_kernel(S, DM, H, DH, M, 32, DC)
    return pl.pallas_call(
        kernel,
        out_shape=jax.ShapeDtypeStruct((1, S, 2 * DM), BF16),
        in_specs=[pl.BlockSpec(memory_space=pl.ANY)] * 12,
        out_specs=pl.BlockSpec(memory_space=pl.ANY),
        scratch_shapes=scratch,
        compiler_params=pltpu.CompilerParams(vmem_limit_bytes=124 * 1024 * 1024),
    )(A_x, A_mem0, A_Wq, A_Wk, A_Wv, A_Wo, B_x, B_c_kv, B_w_q, B_w_uk, B_w_uv, B_w_o)
```

```python
import numpy as np
import jax
import jax.numpy as jnp
import jax.experimental.pallas as pl
import jax.experimental.pallas.tpu as pltpu

F32 = jnp.float32
BF16 = jnp.bfloat16
U32 = jnp.uint32
LOG2E = 1.4426950408889634
NEG = -1e30
NT = (((1,), (1,)), ((), ()))


def _dot(a, b):
    return jnp.dot(a, b, preferred_element_type=F32)


def _dot_nt(a, b):
    return jax.lax.dot_general(a, b, NT, preferred_element_type=F32)


def _unpack(u, parity):
    if isinstance(parity, int):
        w = (u << 16) if parity == 0 else (u & jnp.uint32(0xFFFF0000))
    else:
        w = (u >> (16 * parity).astype(U32)) << 16
    return pltpu.bitcast(w, F32).astype(BF16)


def _interleave(ga, na, gb, nb):
    ia = ib = 0
    while ia < na or ib < nb:
        if ib >= nb or (ia < na and ia * nb <= ib * na):
            next(ga, None)
            ia += 1
        else:
            next(gb, None)
            ib += 1
    for _ in ga:
        pass
    for _ in gb:
        pass


def _count(gen):
    return sum(1 for _ in gen)


def _make_kernel(S, DM, H, DH, M, SEG, DC):
    NP = H // 2
    NSEG = S // SEG
    DP = 512
    PW = 2 * DM
    STEPS = NSEG // H
    QB = 128
    OB = DM // 4

    def kernel(ax_h, mem_h, awq_h, awk_h, awv_h, awo_h, bx_h, ckv_h, bwq_h, bwk_h, bwv_h, bwo_h,
               out_h,
               xraw, he, xo, mem0, memall, awq, awk, awv, awo, wqk, wvo, qa,
               bxraw, bx, ckv, bwq, bwk, bwv, bwo,
               wq_s, wk_s, wv_s, k_s, v_s, acca, accb, ostage,
               sem_x, sem_aq, sem_ak, sem_av, sem_ao, sem_bq, sem_bk, sem_bv, sem_bo, sem_out):

        def pair_copy(src, dst, sem, i):
            return pltpu.make_async_copy(src.bitcast(U32).at[:, i, :], dst.at[i], sem.at[i])

        def wo_copy(src, dst, sem, i):
            return pltpu.make_async_copy(src.at[pl.ds(2 * i, 2)], dst.at[pl.ds(2 * i, 2)], sem.at[i])

        cp_ax = pltpu.make_async_copy(ax_h, xraw, sem_x.at[0])
        cp_mem = pltpu.make_async_copy(mem_h.at[0], mem0, sem_x.at[1])
        cp_bx = pltpu.make_async_copy(bx_h, bxraw, sem_x.at[2])
        cp_ckv = pltpu.make_async_copy(ckv_h.at[0], ckv, sem_x.at[3])

        cp_ax.start()
        cp_mem.start()
        for i in range(NP):
            pair_copy(awq_h, awq, sem_aq, i).start()
        for i in range(NP):
            pair_copy(awk_h, awk, sem_ak, i).start()
            pair_copy(awv_h, awv, sem_av, i).start()
            wo_copy(awo_h, awo, sem_ao, i).start()
        cp_bx.start()
        cp_ckv.start()
        for i in range(NP):
            pair_copy(bwq_h, bwq, sem_bq, i).start()
            pair_copy(bwk_h, bwk, sem_bk, i).start()
            pair_copy(bwv_h, bwv, sem_bv, i).start()
            wo_copy(bwo_h, bwo, sem_bo, i).start()

        accb[...] = jnp.zeros(accb.shape, F32)
        acca[...] = jnp.zeros(acca.shape, F32)

        cp_ax.wait()

        def pad_body(r, c):
            rows = pl.ds(pl.multiple_of(r * 256, 256), 256)
            xt = xraw[:, rows]
            zpad = jnp.zeros((DP - DM, 256), BF16)
            he[rows, :] = jnp.concatenate([xt, zpad], axis=0).T
            xo[rows, :] = jnp.concatenate([zpad, xt], axis=0).T
            return c
        with jax.named_scope('pad_body'):
            jax.lax.fori_loop(0, S // 256, pad_body, 0)

        def qa_body(i, c):
            pair_copy(awq_h, awq, sem_aq, i).wait()
            u = awq[i]
            for par in range(2):
                w = _unpack(u, par)
                for r in range(S // 512):
                    rows = pl.ds(r * 512, 512)
                    qa[2 * i + par, rows, :] = (_dot(he[rows, :DM], w) * (LOG2E * DH ** -0.5)).astype(BF16)
            return c
        with jax.named_scope('qa_body'):
            jax.lax.fori_loop(0, NP, qa_body, 0)

        def absorb_body(i, c):
            pair_copy(awk_h, awk, sem_ak, i).wait()
            pair_copy(awv_h, awv, sem_av, i).wait()
            wo_copy(awo_h, awo, sem_ao, i).wait()
            uq, uk, uv = awq[i], awk[i], awv[i]
            zpad = jnp.zeros((DP - DM, DH), BF16)
            sc = LOG2E * DH ** -0.5
            e = _dot_nt(_unpack(uq, 0), jnp.concatenate([_unpack(uk, 0), zpad], axis=0)) * sc
            o = _dot_nt(_unpack(uq, 1), jnp.concatenate([zpad, _unpack(uk, 1)], axis=0)) * sc
            slab = jnp.concatenate([e[:, :DP - 128], e[:, DP - 128:] + o[:, :128], o[:, 128:]], axis=1)
            wqk[i] = slab.astype(BF16)
            for par in range(2):
                r = _dot_nt(_unpack(uv, par), jnp.concatenate([awo[2 * i + par], zpad], axis=0))
                wvo[i, pl.ds(par * DM, DM), :] = r.astype(BF16)
            return c
        with jax.named_scope('absorb_body'):
            jax.lax.fori_loop(0, NP, absorb_body, 0)

        cp_mem.wait()
        memall[pl.ds(0, M), :] = jnp.concatenate([mem0[...].astype(F32), jnp.zeros((M, DP - DM), F32)], axis=1)
        cp_bx.wait()
        cp_ckv.wait()

        def bx_body(r, c):
            rows = pl.ds(pl.multiple_of(r * 256, 256), 256)
            bx[rows, :] = jnp.concatenate([bxraw[:, rows], jnp.zeros((DP - DM, 256), BF16)], axis=0).T
            return c
        with jax.named_scope('bx_body'):
            jax.lax.fori_loop(0, S // 256, bx_body, 0)

        def chain_step(s):
            mem = memall[pl.ds(pl.multiple_of(s * M, M), M), :]
            mb = mem.astype(BF16)
            rows = []
            for i in range(NP):
                tiles = []
                for n0, n1 in ((0, 256), (256, 512), (512, PW)):
                    acc = None
                    for k0, k1 in ((0, 256), (256, DM)):
                        d = _dot(mb[:, k0:k1], wqk[i, k0:k1, n0:n1])
                        acc = d if acc is None else acc + d
                        yield
                    tiles.append(acc)
                t = jnp.concatenate(tiles, axis=1)
                rows.append(t[:, :DP])
                rows.append(t[:, PW - DP:])
            tq = jnp.concatenate(rows, axis=0).astype(BF16)
            xr = pl.ds(pl.multiple_of(s * SEG, SEG), SEG)
            z8 = jnp.zeros((16 - M, DP), F32)
            keys = jnp.concatenate([
                he[xr, :], jnp.concatenate([mem, z8], axis=0).astype(BF16),
                xo[xr, :], jnp.concatenate([pltpu.roll(mem, DP - DM, 1), z8], axis=0).astype(BF16),
            ], axis=0)
            sc = _dot_nt(tq, keys)
            yield
            kw = SEG + 16
            ri = jax.lax.broadcasted_iota(jnp.int32, sc.shape, 0)
            ci = jax.lax.broadcasted_iota(jnp.int32, sc.shape, 1)
            lo = ((ri // M) % 2) * kw
            sc = jnp.where((ci >= lo) & (ci < lo + SEG + M), sc, NEG)
            p = jnp.exp2(sc - jnp.max(sc, axis=1, keepdims=True))
            p = p / jnp.sum(p, axis=1, keepdims=True)
            z = _dot(p.astype(BF16), keys)
            yield
            acc = [None, None]
            for i in range(NP):
                ze = z[2 * i * M:(2 * i + 1) * M]
                zo = z[(2 * i + 1) * M:(2 * i + 2) * M]
                zp = jnp.concatenate([ze[:, :DP - 128], ze[:, DP - 128:] + zo[:, :128], zo[:, 128:]],
                                     axis=1).astype(BF16)
                for k0, k1 in ((0, 256), (256, 512), (512, PW)):
                    for n in range(2):
                        d = _dot(zp[:, k0:k1], wvo[i, k0:k1, n * 256:(n + 1) * 256])
                        acc[n] = d if acc[n] is None else acc[n] + d
                        yield
            new = jnp.concatenate(acc, axis=1).astype(BF16).astype(F32)
            memall[pl.ds(pl.multiple_of((s + 1) * M, M), M), :] = new

        def chain(h):
            for j in range(STEPS):
                yield from chain_step(h * STEPS + j)

        def b_head(h):
            i = h // 2
            par = h % 2
            wq_s[...] = _unpack(bwq[i], par)
            wk_s[...] = _unpack(bwk[i], par)
            wv_s[...] = _unpack(bwv[i], par)
            for w_s, dst in ((wk_s, k_s), (wv_s, v_s)):
                for r in range(S // QB):
                    rows = pl.ds(r * QB, QB)
                    acc = None
                    for k0 in range(0, DC, 256):
                        d = _dot(ckv[rows, k0:k0 + 256], w_s[k0:k0 + 256, :])
                        acc = d if acc is None else acc + d
                        yield
                    dst[rows, :] = acc.astype(BF16)
            ctxs = []
            for r in range(S // QB):
                rows = pl.ds(r * QB, QB)
                acc = None
                for k0, k1 in ((0, 256), (256, DM)):
                    d = _dot(bx[rows, k0:k1], wq_s[k0:k1, :])
                    acc = d if acc is None else acc + d
                    yield
                q = (acc * (LOG2E * DH ** -0.5)).astype(BF16)
                nk = (r + 1) * QB
                chunks = [(c0, min(c0 + 256, nk)) for c0 in range(0, nk, 256)]
                ss = []
                for c0, c1 in chunks:
                    sc = _dot_nt(q, k_s[c0:c1, :])
                    if c1 == nk:
                        ri = jax.lax.broadcasted_iota(jnp.int32, sc.shape, 0) + r * QB
                        ci = jax.lax.broadcasted_iota(jnp.int32, sc.shape, 1) + c0
                        sc = jnp.where(ci <= ri, sc, NEG)
                    ss.append(sc)
                    yield
                m = None
                for sc in ss:
                    for t0 in range(0, sc.shape[1], 128):
                        m = sc[:, t0:t0 + 128] if m is None else jnp.maximum(m, sc[:, t0:t0 + 128])
                m = jnp.max(m, axis=1, keepdims=True)
                l = None
                acc = None
                for (c0, c1), sc in zip(chunks, ss):
                    p = jnp.exp2(sc - m)
                    for t0 in range(0, p.shape[1], 128):
                        l = p[:, t0:t0 + 128] if l is None else l + p[:, t0:t0 + 128]
                    d = _dot(p.astype(BF16), v_s[c0:c1, :])
                    acc = d if acc is None else acc + d
                    yield
                ctxs.append((acc / jnp.sum(l, axis=1, keepdims=True)).astype(BF16))
                if len(ctxs) == 2:
                    ctx = jnp.concatenate(ctxs, axis=0)
                    ctxs = []
                    cols = pl.ds((r - 1) * QB, 2 * QB)
                    for n0 in range(0, DM, OB):
                        accb[n0:n0 + OB, cols] += _dot_nt(bwo[h, n0:n0 + OB, :], ctx)
                        yield

        n_chain = STEPS * (NP * 6 * 2 + 2)
        n_head = (S // QB) * (2 * DC // 256 + 4) + 2 * sum((r + 2) // 2 for r in range(S // QB))

        def b_body(h, c):
            i = h // 2

            @pl.when(h % 2 == 0)
            def _():
                pair_copy(bwq_h, bwq, sem_bq, i).wait()
                pair_copy(bwk_h, bwk, sem_bk, i).wait()
                pair_copy(bwv_h, bwv, sem_bv, i).wait()
                wo_copy(bwo_h, bwo, sem_bo, i).wait()
            _interleave(chain(h), n_chain, b_head(h), n_head)
            return c
        with jax.named_scope('b_body'):
            jax.lax.fori_loop(0, H, b_body, 0)

        he[pl.ds(S, NSEG * M), :] = memall[pl.ds(0, NSEG * M), :].astype(BF16)
        AB = 2 * SEG
        ri = jax.lax.broadcasted_iota(jnp.int32, (AB, AB + 2 * M), 0)
        ci = jax.lax.broadcasted_iota(jnp.int32, (AB, AB + 2 * M), 1)
        amask = ((ci < AB) & ((ci // SEG) == (ri // SEG)) & (ci <= ri)) | ((ci >= AB) & (((ci - AB) // M) == (ri // SEG)))

        def a_body(h, c):
            i = h // 2
            par = h % 2
            wk = _unpack(awk[i], par)
            wv = _unpack(awv[i], par)
            for r in range((S + NSEG * M) // 512):
                rows = pl.ds(r * 512, 512)
                k_s[rows, :] = _dot(he[rows, :DM], wk).astype(BF16)
                v_s[rows, :] = _dot(he[rows, :DM], wv).astype(BF16)
            for r in range(S // 512):
                ctxs = []
                for j in range(r * 512 // AB, (r + 1) * 512 // AB):
                    xr = pl.ds(j * AB, AB)
                    mr = pl.ds(S + j * 2 * M, 2 * M)
                    kc = jnp.concatenate([k_s[xr, :], k_s[mr, :]], axis=0)
                    vc = jnp.concatenate([v_s[xr, :], v_s[mr, :]], axis=0)
                    sc = jnp.where(amask, _dot_nt(qa[h, xr, :], kc), NEG)
                    p = jnp.exp2(sc - jnp.max(sc, axis=1, keepdims=True))
                    p = p / jnp.sum(p, axis=1, keepdims=True)
                    ctxs.append(_dot(p.astype(BF16), vc).astype(BF16))
                acca[:, pl.ds(r * 512, 512)] += _dot_nt(awo[h], jnp.concatenate(ctxs, axis=0))
            return c
        with jax.named_scope('a_body'):
            jax.lax.fori_loop(0, H, a_body, 0)

        cps = []
        for r in range(S // 512):
            rows = pl.ds(r * 512, 512)
            ostage[rows, :] = jnp.concatenate([acca[:, rows], accb[:, rows]], axis=0).astype(BF16).T
            cp = pltpu.make_async_copy(ostage.at[rows, :], out_h.at[0, rows, :], sem_out.at[r])
            cp.start()
            cps.append(cp)
        for cp in cps:
            cp.wait()

    scratch = [
        pltpu.VMEM((DM, S), BF16),
        pltpu.VMEM((S + NSEG * M, DP), BF16),
        pltpu.VMEM((S, DP), BF16),
        pltpu.VMEM((M, DM), BF16),
        pltpu.VMEM(((NSEG + 1) * M, DP), F32),
        pltpu.VMEM((NP, DM, DH), U32),
        pltpu.VMEM((NP, DM, DH), U32),
        pltpu.VMEM((NP, DM, DH), U32),
        pltpu.VMEM((H, DM, DH), BF16),
        pltpu.VMEM((NP, DM, PW), BF16),
        pltpu.VMEM((NP, PW, DP), BF16),
        pltpu.VMEM((H, S, DH), BF16),
        pltpu.VMEM((DM, S), BF16),
        pltpu.VMEM((S, DP), BF16),
        pltpu.VMEM((S, DC), BF16),
        pltpu.VMEM((NP, DM, DH), U32),
        pltpu.VMEM((NP, DC, DH), U32),
        pltpu.VMEM((NP, DC, DH), U32),
        pltpu.VMEM((H, DM, DH), BF16),
        pltpu.VMEM((DM, DH), BF16),
        pltpu.VMEM((DC, DH), BF16),
        pltpu.VMEM((DC, DH), BF16),
        pltpu.VMEM((S + NSEG * M, DH), BF16),
        pltpu.VMEM((S + NSEG * M, DH), BF16),
        pltpu.VMEM((DM, S), F32),
        pltpu.VMEM((DM, S), F32),
        pltpu.VMEM((S, 2 * DM), BF16),
        pltpu.SemaphoreType.DMA((4,)),
    ] + [pltpu.SemaphoreType.DMA((NP,)) for _ in range(8)] + [pltpu.SemaphoreType.DMA((S // 512,))]
    return kernel, scratch


@jax.jit
def pallas_concat_heads__memory_aug_recurrent_mem_tr__compressed_kv_cla__prompt_kernel(
    A_x, A_mem0, A_Wq, A_Wk, A_Wv, A_Wo, A_seg_len, B_x, B_c_kv, B_w_q, B_w_uk, B_w_uv, B_w_o,
):
    del A_seg_len
    _, S, DM = A_x.shape
    M = A_mem0.shape[1]
    H, DH = A_Wq.shape[1], A_Wq.shape[2]
    DC = B_c_kv.shape[2]
    kernel, scratch = _make_kernel(S, DM, H, DH, M, 32, DC)
    return pl.pallas_call(
        kernel,
        out_shape=jax.ShapeDtypeStruct((1, S, 2 * DM), BF16),
        in_specs=[pl.BlockSpec(memory_space=pl.ANY)] * 12,
        out_specs=pl.BlockSpec(memory_space=pl.ANY),
        scratch_shapes=scratch,
        compiler_params=pltpu.CompilerParams(vmem_limit_bytes=124 * 1024 * 1024),
    )(A_x[0].T, A_mem0, A_Wq, A_Wk, A_Wv, A_Wo.transpose(0, 2, 1),
      B_x[0].T, B_c_kv, B_w_q, B_w_uk, B_w_uv, B_w_o.transpose(0, 2, 1))
```

```python
import numpy as np
import jax
import jax.numpy as jnp
import jax.experimental.pallas as pl
import jax.experimental.pallas.tpu as pltpu

F32 = jnp.float32
BF16 = jnp.bfloat16
U32 = jnp.uint32
LOG2E = 1.4426950408889634
NEG = -1e30
NT = (((1,), (1,)), ((), ()))


def _dot(a, b):
    return jnp.dot(a, b, preferred_element_type=F32)


def _dot_nt(a, b):
    return jax.lax.dot_general(a, b, NT, preferred_element_type=F32)


def _bf(u):
    return pltpu.bitcast(u, BF16)


def _u32(x):
    return pltpu.bitcast(x.astype(BF16), U32)


def _half(start, size):
    if isinstance(start, int):
        return pl.ds(start // 2, size // 2)
    return pl.ds(pl.multiple_of(start // 2, 8), size // 2)


def _unpack(u, parity):
    if isinstance(parity, int):
        w = (u << 16) if parity == 0 else (u & jnp.uint32(0xFFFF0000))
    else:
        w = (u >> (16 * parity).astype(U32)) << 16
    return pltpu.bitcast(w, F32).astype(BF16)


def _interleave(ga, na, gb, nb):
    ia = ib = 0
    while ia < na or ib < nb:
        if ib >= nb or (ia < na and ia * nb <= ib * na):
            next(ga, None)
            ia += 1
        else:
            next(gb, None)
            ib += 1
    for _ in ga:
        pass
    for _ in gb:
        pass


def _make_kernel(S, DM, H, DH, M, SEG, DC):
    NP = H // 2
    NSEG = S // SEG
    DP = 512
    PW = 2 * DM
    PT = PW // 128
    NT_ = NP * PT
    KM = DM // 128 * 128
    STEPS = NSEG // H
    QB = 128
    OB = DM // 4
    QSC = LOG2E * DH ** -0.5

    def kernel(ax_h, mem_h, awq_h, awk_h, awv_h, awo_h, bx_h, ckv_h, bwq_h, bwk_h, bwv_h, bwo_h,
               out_h,
               xraw, he, xo, mem0, memall, awq, awk, awv, awo, wqk, wqk_t, wvo, wvo_t, qa,
               bxraw, bx, ckv, bwq, bwk, bwv, bwo,
               wq_s, wk_s, wv_s, k_s, v_s, acca, accb, ostage,
               sem_x, sem_aq, sem_ak, sem_av, sem_ao, sem_bq, sem_bk, sem_bv, sem_bo, sem_out):

        def pair_copy(src, dst, sem, i):
            return pltpu.make_async_copy(src.bitcast(U32).at[:, i, :], dst.at[i], sem.at[i])

        def wo_copy(src, dst, sem, i):
            return pltpu.make_async_copy(src.bitcast(U32).at[pl.ds(2 * i, 2)], dst.at[pl.ds(2 * i, 2)], sem.at[i])

        cp_ax = pltpu.make_async_copy(ax_h.bitcast(U32), xraw, sem_x.at[0])
        cp_mem = pltpu.make_async_copy(mem_h.at[0], mem0, sem_x.at[1])
        cp_bx = pltpu.make_async_copy(bx_h.bitcast(U32), bxraw, sem_x.at[2])
        cp_ckv = pltpu.make_async_copy(ckv_h.bitcast(U32).at[0], ckv, sem_x.at[3])

        cp_ax.start()
        cp_mem.start()
        for i in range(NP):
            pair_copy(awq_h, awq, sem_aq, i).start()
        for i in range(NP):
            pair_copy(awk_h, awk, sem_ak, i).start()
            pair_copy(awv_h, awv, sem_av, i).start()
            wo_copy(awo_h, awo, sem_ao, i).start()
        cp_bx.start()
        cp_ckv.start()
        for i in range(NP):
            pair_copy(bwq_h, bwq, sem_bq, i).start()
            pair_copy(bwk_h, bwk, sem_bk, i).start()
            pair_copy(bwv_h, bwv, sem_bv, i).start()
            wo_copy(bwo_h, bwo, sem_bo, i).start()

        accb[...] = jnp.zeros(accb.shape, F32)
        acca[...] = jnp.zeros(acca.shape, F32)

        cp_ax.wait()

        def pad_body(r, c):
            xt = _bf(xraw[:, pl.ds(pl.multiple_of(r * 256, 256), 256)])
            zpad = jnp.zeros((DP - DM, 256), BF16)
            he[_half(r * 256, 256), :] = _u32(jnp.concatenate([xt, zpad], axis=0).T)
            xo[_half(r * 256, 256), :] = _u32(jnp.concatenate([zpad, xt], axis=0).T)
            return c
        with jax.named_scope('pad_body'):
            jax.lax.fori_loop(0, S // 256, pad_body, 0)

        def qa_body(i, c):
            pair_copy(awq_h, awq, sem_aq, i).wait()
            u = awq[i]
            for par in range(2):
                w = _unpack(u, par)
                for r in range(S // 512):
                    rows = _half(r * 512, 512)
                    qa[2 * i + par, rows, :] = _u32(_dot(_bf(he[rows, :])[:, :DM], w) * QSC)
            return c
        with jax.named_scope('qa_body'):
            jax.lax.fori_loop(0, NP, qa_body, 0)

        def absorb_body(i, c):
            pair_copy(awk_h, awk, sem_ak, i).wait()
            pair_copy(awv_h, awv, sem_av, i).wait()
            wo_copy(awo_h, awo, sem_ao, i).wait()
            uq, uk, uv = awq[i], awk[i], awv[i]
            zpad = jnp.zeros((DP - DM, DH), BF16)
            e = _dot_nt(_unpack(uq, 0), jnp.concatenate([_unpack(uk, 0), zpad], axis=0)) * QSC
            o = _dot_nt(_unpack(uq, 1), jnp.concatenate([zpad, _unpack(uk, 1)], axis=0)) * QSC
            slab = _u32(jnp.concatenate([e[:, :DP - 128], e[:, DP - 128:] + o[:, :128], o[:, 128:]], axis=1))
            for j in range(PT):
                t = PT * i + j
                wqk[t] = slab[:KM // 2, j * 128:(j + 1) * 128]
                wqk_t[t // 2, _half((t % 2) * 64, 64), :] = slab[KM // 2:, j * 128:(j + 1) * 128]
            for par in range(2):
                r = _dot_nt(_unpack(uv, par), jnp.concatenate([_bf(awo[2 * i + par]), zpad], axis=0))
                wvo[_half((2 * i + par) * DM, DM), :] = _u32(r)
            return c
        with jax.named_scope('absorb_body'):
            jax.lax.fori_loop(0, NP, absorb_body, 0)


        def tail_body(j, c):
            wvo_t[_half(j * 128, 128), :] = (wvo[_half(2 * j * 128, 128), KM:]
                                             | pltpu.roll(wvo[_half((2 * j + 1) * 128, 128), KM:], 64, 1))
            return c
        jax.lax.fori_loop(0, NT_ // 2, tail_body, 0)

        cp_mem.wait()
        memall[pl.ds(0, M), :] = jnp.concatenate([mem0[...].astype(F32), jnp.zeros((M, DP - DM), F32)], axis=1)
        cp_bx.wait()
        cp_ckv.wait()

        def bx_body(r, c):
            xt = _bf(bxraw[:, pl.ds(pl.multiple_of(r * 256, 256), 256)])
            bx[_half(r * 256, 256), :] = _u32(jnp.concatenate([xt, jnp.zeros((DP - DM, 256), BF16)], axis=0).T)
            return c
        with jax.named_scope('bx_body'):
            jax.lax.fori_loop(0, S // 256, bx_body, 0)

        def chain_step(s):
            mem = memall[pl.ds(pl.multiple_of(s * M, M), M), :]
            mb = mem.astype(BF16)
            zero = s // (2 * NSEG)
            mt = mem[:, KM:]
            mtail = jnp.concatenate([mt, pltpu.roll(mt, 64, 1)], axis=0).astype(BF16)
            t = []
            for g in range(0, NT_, 8):
                for t0 in (g, g + 4):
                    acc = None
                    for k0 in range(0, KM, 128):
                        w = jnp.concatenate([wqk[t0 + j + zero, _half(k0, 128), :] for j in range(4)], axis=1)
                        d = _dot(mb[:, k0:k0 + 128], _bf(w))
                        acc = d if acc is None else acc + d
                        yield
                    t += [acc[:, j * 128:(j + 1) * 128] for j in range(4)]
                w = jnp.concatenate([wqk_t[g // 2 + j + zero] for j in range(4)], axis=1)
                d = _dot(mtail, _bf(w))
                yield
                for j in range(8):
                    t[g + j] = t[g + j] + d[(j % 2) * M:(j % 2 + 1) * M, (j // 2) * 128:(j // 2 + 1) * 128]
            tq = jnp.concatenate([jnp.concatenate(t[h * PT // 2:h * PT // 2 + 4], axis=1) for h in range(H)],
                                 axis=0).astype(BF16)
            xr = _half(s * SEG, SEG)
            z8 = jnp.zeros((16 - M, DP), F32)
            keys = jnp.concatenate([
                _bf(he[xr, :]), jnp.concatenate([mem, z8], axis=0).astype(BF16),
                _bf(xo[xr, :]), jnp.concatenate([pltpu.roll(mem, DP - DM, 1), z8], axis=0).astype(BF16),
            ], axis=0)
            sc = _dot_nt(tq, keys)
            yield
            kw = SEG + 16
            ri = jax.lax.broadcasted_iota(jnp.int32, sc.shape, 0)
            ci = jax.lax.broadcasted_iota(jnp.int32, sc.shape, 1)
            lo = ((ri // M) % 2) * kw
            sc = jnp.where((ci >= lo) & (ci < lo + SEG + M), sc, NEG)
            p = jnp.exp2(sc - jnp.max(sc, axis=1, keepdims=True))
            p = p / jnp.sum(p, axis=1, keepdims=True)
            z = _dot(p.astype(BF16), keys)
            yield
            zt = []
            for i in range(NP):
                ze = z[2 * i * M:(2 * i + 1) * M]
                zo = z[(2 * i + 1) * M:(2 * i + 2) * M]
                zt += [ze[:, 0:128], ze[:, 128:256], ze[:, 256:384], ze[:, 384:] + zo[:, :128],
                       zo[:, 128:256], zo[:, 256:384], zo[:, 384:]]
            acc = [None] * 4
            for g in range(0, NT_, 8):
                for t0 in (g, g + 4):
                    zp = jnp.concatenate(zt[t0:t0 + 4], axis=1).astype(BF16)
                    for n in range(KM // 128):
                        d = _dot(zp, _bf(wvo[_half((t0 + zero) * 128, 512), n * 128:(n + 1) * 128]))
                        acc[n] = d if acc[n] is None else acc[n] + d
                        yield
                zp = jnp.concatenate([jnp.concatenate(zt[g:g + 8:2], axis=1),
                                      jnp.concatenate(zt[g + 1:g + 8:2], axis=1)], axis=0).astype(BF16)
                d = _dot(zp, _bf(wvo_t[_half((g // 2 + zero) * 128, 512), :]))
                acc[3] = d if acc[3] is None else acc[3] + d
                yield
            lane = jax.lax.broadcasted_iota(jnp.int32, (M, 128), 1)
            last = jnp.where(lane < 64, acc[3][:M] + pltpu.roll(acc[3][M:], 64, 1), 0.0)
            new = jnp.concatenate(acc[:3] + [last], axis=1).astype(BF16).astype(F32)
            memall[pl.ds(pl.multiple_of((s + 1) * M, M), M), :] = new

        def chain(h):
            for j in range(STEPS):
                yield from chain_step(h * STEPS + j)

        def b_head(h):
            i = h // 2
            par = h % 2
            wq_s[...] = _u32(_unpack(bwq[i], par))
            wk_s[...] = _u32(_unpack(bwk[i], par))
            wv_s[...] = _u32(_unpack(bwv[i], par))
            for w_s, dst in ((wk_s, k_s), (wv_s, v_s)):
                for r in range(S // QB):
                    rows = _half(r * QB, QB)
                    acc = None
                    for k0 in range(0, DC, 256):
                        d = _dot(_bf(ckv[rows, k0:k0 + 256]), _bf(w_s[_half(k0, 256), :]))
                        acc = d if acc is None else acc + d
                        yield
                    dst[rows, :] = _u32(acc)
            ctxs = []
            for r in range(S // QB):
                rows = _half(r * QB, QB)
                acc = None
                for k0, k1 in ((0, 256), (256, DM)):
                    d = _dot(_bf(bx[rows, k0:k0 + 256])[:, :k1 - k0], _bf(wq_s[_half(k0, k1 - k0), :]))
                    acc = d if acc is None else acc + d
                    yield
                q = (acc * QSC).astype(BF16)
                nk = (r + 1) * QB
                chunks = [(c0, min(c0 + 256, nk)) for c0 in range(0, nk, 256)]
                ss = []
                for c0, c1 in chunks:
                    sc = _dot_nt(q, _bf(k_s[_half(c0, c1 - c0), :]))
                    if c1 == nk:
                        ri = jax.lax.broadcasted_iota(jnp.int32, sc.shape, 0) + r * QB
                        ci = jax.lax.broadcasted_iota(jnp.int32, sc.shape, 1) + c0
                        sc = jnp.where(ci <= ri, sc, NEG)
                    ss.append(sc)
                    yield
                m = None
                for sc in ss:
                    for t0 in range(0, sc.shape[1], 128):
                        m = sc[:, t0:t0 + 128] if m is None else jnp.maximum(m, sc[:, t0:t0 + 128])
                m = jnp.max(m, axis=1, keepdims=True)
                l = None
                acc = None
                for (c0, c1), sc in zip(chunks, ss):
                    p = jnp.exp2(sc - m)
                    for t0 in range(0, p.shape[1], 128):
                        l = p[:, t0:t0 + 128] if l is None else l + p[:, t0:t0 + 128]
                    d = _dot(p.astype(BF16), _bf(v_s[_half(c0, c1 - c0), :]))
                    acc = d if acc is None else acc + d
                    yield
                ctxs.append((acc / jnp.sum(l, axis=1, keepdims=True)).astype(BF16))
                if len(ctxs) == 2:
                    ctx = jnp.concatenate(ctxs, axis=0)
                    ctxs = []
                    cols = pl.ds((r - 1) * QB, 2 * QB)
                    for n0 in range(0, DM, OB):
                        accb[n0:n0 + OB, cols] += _dot_nt(_bf(bwo[h, _half(n0, OB), :]), ctx)
                        yield

        n_chain = STEPS * (NT_ // 8 * 7 * 2 + 2)
        n_head = (S // QB) * (2 * DC // 256 + 4) + 2 * sum((r + 2) // 2 for r in range(S // QB))

        def b_body(h, c):
            i = h // 2

            @pl.when(h % 2 == 0)
            def _():
                pair_copy(bwq_h, bwq, sem_bq, i).wait()
                pair_copy(bwk_h, bwk, sem_bk, i).wait()
                pair_copy(bwv_h, bwv, sem_bv, i).wait()
                wo_copy(bwo_h, bwo, sem_bo, i).wait()
            _interleave(chain(h), n_chain, b_head(h), n_head)
            return c
        with jax.named_scope('b_body'):
            jax.lax.fori_loop(0, H, b_body, 0)

        he[_half(S, NSEG * M), :] = _u32(memall[pl.ds(0, NSEG * M), :])
        AB = 2 * SEG
        ri = jax.lax.broadcasted_iota(jnp.int32, (AB, AB + 2 * M), 0)
        ci = jax.lax.broadcasted_iota(jnp.int32, (AB, AB + 2 * M), 1)
        amask = ((ci < AB) & ((ci // SEG) == (ri // SEG)) & (ci <= ri)) | ((ci >= AB) & (((ci - AB) // M) == (ri // SEG)))

        def a_body(h, c):
            i = h // 2
            par = h % 2
            wk = _unpack(awk[i], par)
            wv = _unpack(awv[i], par)
            for r in range((S + NSEG * M) // 512):
                rows = _half(r * 512, 512)
                x = _bf(he[rows, :])[:, :DM]
                k_s[rows, :] = _u32(_dot(x, wk))
                v_s[rows, :] = _u32(_dot(x, wv))
            for r in range(S // 512):
                ctxs = []
                for j in range(r * 512 // AB, (r + 1) * 512 // AB):
                    xr = _half(j * AB, AB)
                    mr = _half(S + j * 2 * M, 2 * M)
                    kc = _bf(jnp.concatenate([k_s[xr, :], k_s[mr, :]], axis=0))
                    vc = _bf(jnp.concatenate([v_s[xr, :], v_s[mr, :]], axis=0))
                    sc = jnp.where(amask, _dot_nt(_bf(qa[h, xr, :]), kc), NEG)
                    p = jnp.exp2(sc - jnp.max(sc, axis=1, keepdims=True))
                    p = p / jnp.sum(p, axis=1, keepdims=True)
                    ctxs.append(_dot(p.astype(BF16), vc).astype(BF16))
                acca[:, pl.ds(r * 512, 512)] += _dot_nt(_bf(awo[h]), jnp.concatenate(ctxs, axis=0))
            return c
        with jax.named_scope('a_body'):
            jax.lax.fori_loop(0, H, a_body, 0)

        cps = []
        for r in range(S // 512):
            cols = pl.ds(r * 512, 512)
            rows = _half(r * 512, 512)
            ostage[rows, :] = _u32(jnp.concatenate([acca[:, cols], accb[:, cols]], axis=0).astype(BF16).T)
            cp = pltpu.make_async_copy(ostage.at[rows, :], out_h.bitcast(U32).at[0, rows, :], sem_out.at[r])
            cp.start()
            cps.append(cp)
        for cp in cps:
            cp.wait()

    def packed(*shape):
        return pltpu.VMEM(shape[:-2] + (shape[-2] // 2, shape[-1]), U32)

    scratch = [
        packed(DM, S),
        packed(S + NSEG * M, DP),
        packed(S, DP),
        pltpu.VMEM((M, DM), BF16),
        pltpu.VMEM(((NSEG + 1) * M, DP), F32),
        pltpu.VMEM((NP, DM, DH), U32),
        pltpu.VMEM((NP, DM, DH), U32),
        pltpu.VMEM((NP, DM, DH), U32),
        packed(H, DM, DH),
        packed(NT_, KM, 128),
        packed(NT_ // 2, 128, 128),
        packed(NT_ * 128, DP),
        packed(NT_ * 64, 128),
        packed(H, S, DH),
        packed(DM, S),
        packed(S, DP),
        packed(S, DC),
        pltpu.VMEM((NP, DM, DH), U32),
        pltpu.VMEM((NP, DC, DH), U32),
        pltpu.VMEM((NP, DC, DH), U32),
        packed(H, DM, DH),
        packed(DM, DH),
        packed(DC, DH),
        packed(DC, DH),
        packed(S + NSEG * M, DH),
        packed(S + NSEG * M, DH),
        pltpu.VMEM((DM, S), F32),
        pltpu.VMEM((DM, S), F32),
        packed(S, 2 * DM),
        pltpu.SemaphoreType.DMA((4,)),
    ] + [pltpu.SemaphoreType.DMA((NP,)) for _ in range(8)] + [pltpu.SemaphoreType.DMA((S // 512,))]
    return kernel, scratch


@jax.jit
def pallas_concat_heads__memory_aug_recurrent_mem_tr__compressed_kv_cla__prompt_kernel(
    A_x, A_mem0, A_Wq, A_Wk, A_Wv, A_Wo, A_seg_len, B_x, B_c_kv, B_w_q, B_w_uk, B_w_uv, B_w_o,
):
    del A_seg_len
    _, S, DM = A_x.shape
    M = A_mem0.shape[1]
    H, DH = A_Wq.shape[1], A_Wq.shape[2]
    DC = B_c_kv.shape[2]
    kernel, scratch = _make_kernel(S, DM, H, DH, M, 32, DC)
    return pl.pallas_call(
        kernel,
        out_shape=jax.ShapeDtypeStruct((1, S, 2 * DM), BF16),
        in_specs=[pl.BlockSpec(memory_space=pl.ANY)] * 12,
        out_specs=pl.BlockSpec(memory_space=pl.ANY),
        scratch_shapes=scratch,
        compiler_params=pltpu.CompilerParams(vmem_limit_bytes=124 * 1024 * 1024),
    )(A_x[0].T, A_mem0, A_Wq, A_Wk, A_Wv, A_Wo.transpose(0, 2, 1),
      B_x[0].T, B_c_kv, B_w_q, B_w_uk, B_w_uv, B_w_o.transpose(0, 2, 1))
```

```python
import numpy as np
import jax
import jax.numpy as jnp
import jax.experimental.pallas as pl
import jax.experimental.pallas.tpu as pltpu

F32 = jnp.float32
BF16 = jnp.bfloat16
U32 = jnp.uint32
LOG2E = 1.4426950408889634
NEG = -1e30
NN = (((1,), (0,)), ((), ()))
NT = (((1,), (1,)), ((), ()))


def _dot(a, b):
    return jax.lax.dot_general(a, b, NN, preferred_element_type=F32)


def _dot_nt(a, b):
    return jax.lax.dot_general(a, b, NT, preferred_element_type=F32)


def _bf(u):
    return pltpu.bitcast(u, BF16)


def _u32(x):
    return pltpu.bitcast(x.astype(BF16), U32)


def _half(start, size):
    if isinstance(start, int):
        return pl.ds(start // 2, size // 2)
    return pl.ds(pl.multiple_of(start // 2, 8), size // 2)


def _unpack(u, parity):
    if isinstance(parity, int):
        w = (u << 16) if parity == 0 else (u & jnp.uint32(0xFFFF0000))
    else:
        w = (u >> (16 * parity).astype(U32)) << 16
    return pltpu.bitcast(w, F32).astype(BF16)


def _merge(*streams):
    streams = [(g, n) for g, n in streams if n > 0]
    done = [0] * len(streams)
    for _ in range(sum(n for _, n in streams)):
        j = min(range(len(streams)), key=lambda a: ((done[a] + 0.5) / streams[a][1], a))
        next(streams[j][0])
        done[j] += 1
        yield
    for g, _ in streams:
        for _ in g:
            raise AssertionError("stream longer than announced")


def _make_kernel(S, DM, H, DH, M, SEG, DC):
    NP = H // 2
    NSEG = S // SEG
    DP = 512
    PW = 2 * DM
    PT = PW // 128
    NT_ = NP * PT
    KM = DM // 128 * 128
    STEPS = NSEG // H
    QB = 128
    OB = DM // 4
    QSC = LOG2E * DH ** -0.5

    def kernel(ax_h, mem_h, awq_h, awk_h, awv_h, awo_h, bx_h, ckv_h, bwq_h, bwk_h, bwv_h, bwo_h,
               out_h,
               xraw, he, xo, mem0, memall, awq, awk, awv, awo, wqk, wqk_t, wvo, wvo_t, qa,
               bxraw, bx, ckv, bwq, bwk, bwv, bwo,
               wq_s, wk_s, wv_s, k_s, v_s, acca, accb, ostage,
               sem_x, sem_aq, sem_ak, sem_av, sem_ao, sem_bq, sem_bk, sem_bv, sem_bo, sem_out):

        def pair_copy(src, dst, sem, i):
            return pltpu.make_async_copy(src.bitcast(U32).at[:, i, :], dst.at[i], sem.at[i])

        def wo_copy(src, dst, sem, i):
            return pltpu.make_async_copy(src.bitcast(U32).at[pl.ds(2 * i, 2)], dst.at[pl.ds(2 * i, 2)], sem.at[i])

        cp_ax = pltpu.make_async_copy(ax_h.bitcast(U32), xraw, sem_x.at[0])
        cp_mem = pltpu.make_async_copy(mem_h.at[0], mem0, sem_x.at[1])
        cp_bx = pltpu.make_async_copy(bx_h.bitcast(U32), bxraw, sem_x.at[2])
        cp_ckv = pltpu.make_async_copy(ckv_h.bitcast(U32).at[0], ckv, sem_x.at[3])

        cp_ax.start()
        cp_mem.start()
        for i in range(NP):
            pair_copy(awq_h, awq, sem_aq, i).start()
        for i in range(NP):
            pair_copy(awk_h, awk, sem_ak, i).start()
            pair_copy(awv_h, awv, sem_av, i).start()
            wo_copy(awo_h, awo, sem_ao, i).start()
        cp_bx.start()
        cp_ckv.start()
        for i in range(NP):
            pair_copy(bwq_h, bwq, sem_bq, i).start()
            pair_copy(bwk_h, bwk, sem_bk, i).start()
            pair_copy(bwv_h, bwv, sem_bv, i).start()
            wo_copy(bwo_h, bwo, sem_bo, i).start()

        accb[...] = jnp.zeros(accb.shape, F32)
        acca[...] = jnp.zeros(acca.shape, F32)

        cp_ax.wait()

        def pad_body(r, c):
            xt = _bf(xraw[:, pl.ds(pl.multiple_of(r * 256, 256), 256)])
            zpad = jnp.zeros((DP - DM, 256), BF16)
            he[_half(r * 256, 256), :] = _u32(jnp.concatenate([xt, zpad], axis=0).T)
            xo[_half(r * 256, 256), :] = _u32(jnp.concatenate([zpad, xt], axis=0).T)
            return c
        with jax.named_scope('pad_body'):
            jax.lax.fori_loop(0, S // 256, pad_body, 0)

        def qa_body(i, c):
            pair_copy(awq_h, awq, sem_aq, i).wait()
            u = awq[i]
            for par in range(2):
                w = _unpack(u, par)
                for r in range(S // 512):
                    rows = _half(r * 512, 512)
                    qa[2 * i + par, rows, :] = _u32(_dot(_bf(he[rows, :])[:, :DM], w) * QSC)
            return c
        with jax.named_scope('qa_body'):
            jax.lax.fori_loop(0, NP, qa_body, 0)

        def absorb_body(i, c):
            pair_copy(awk_h, awk, sem_ak, i).wait()
            pair_copy(awv_h, awv, sem_av, i).wait()
            wo_copy(awo_h, awo, sem_ao, i).wait()
            uq, uk, uv = awq[i], awk[i], awv[i]
            zpad = jnp.zeros((DP - DM, DH), BF16)
            e = _dot_nt(_unpack(uq, 0), jnp.concatenate([_unpack(uk, 0), zpad], axis=0)) * QSC
            o = _dot_nt(_unpack(uq, 1), jnp.concatenate([zpad, _unpack(uk, 1)], axis=0)) * QSC
            slab = _u32(jnp.concatenate([e[:, :DP - 128], e[:, DP - 128:] + o[:, :128], o[:, 128:]], axis=1))
            for j in range(PT):
                t = PT * i + j
                wqk[t] = slab[:KM // 2, j * 128:(j + 1) * 128]
                wqk_t[t // 2, _half((t % 2) * 64, 64), :] = slab[KM // 2:, j * 128:(j + 1) * 128]
            for par in range(2):
                r = _dot_nt(_unpack(uv, par), jnp.concatenate([_bf(awo[2 * i + par]), zpad], axis=0))
                wvo[_half((2 * i + par) * DM, DM), :] = _u32(r)
            return c
        with jax.named_scope('absorb_body'):
            jax.lax.fori_loop(0, NP, absorb_body, 0)


        def tail_body(j, c):
            wvo_t[_half(j * 128, 128), :] = (wvo[_half(2 * j * 128, 128), KM:]
                                             | pltpu.roll(wvo[_half((2 * j + 1) * 128, 128), KM:], 64, 1))
            return c
        jax.lax.fori_loop(0, NT_ // 2, tail_body, 0)

        cp_mem.wait()
        memall[pl.ds(0, M), :] = jnp.concatenate([mem0[...].astype(F32), jnp.zeros((M, DP - DM), F32)], axis=1)
        cp_bx.wait()
        cp_ckv.wait()

        def bx_body(r, c):
            xt = _bf(bxraw[:, pl.ds(pl.multiple_of(r * 256, 256), 256)])
            bx[_half(r * 256, 256), :] = _u32(jnp.concatenate([xt, jnp.zeros((DP - DM, 256), BF16)], axis=0).T)
            return c
        with jax.named_scope('bx_body'):
            jax.lax.fori_loop(0, S // 256, bx_body, 0)

        def chain_step(s):
            mem = memall[pl.ds(pl.multiple_of(s * M, M), M), :]
            zero = s // (2 * NSEG)
            mt = mem[:, KM:]
            mtail = jnp.concatenate([mt, pltpu.roll(mt, 64, 1)], axis=0).astype(BF16)
            t = []
            for g in range(0, NT_, 8):
                for t0 in (g, g + 4):
                    acc = None
                    for k0 in range(0, KM, 128):
                        w = jnp.concatenate([wqk[t0 + j + zero, _half(k0, 128), :] for j in range(4)], axis=1)
                        d = _dot(mem[:, k0:k0 + 128], _bf(w))
                        acc = d if acc is None else acc + d
                        yield
                    t += [acc[:, j * 128:(j + 1) * 128] for j in range(4)]
                w = jnp.concatenate([wqk_t[g // 2 + j + zero] for j in range(4)], axis=1)
                d = _dot(mtail, _bf(w))
                yield
                for j in range(8):
                    t[g + j] = t[g + j] + d[(j % 2) * M:(j % 2 + 1) * M, (j // 2) * 128:(j // 2 + 1) * 128]
            tq = jnp.concatenate([jnp.concatenate(t[h * PT // 2:h * PT // 2 + 4], axis=1) for h in range(H)],
                                 axis=0).astype(BF16)
            xr = _half(s * SEG, SEG)
            z8 = jnp.zeros((16 - M, DP), F32)
            keys = jnp.concatenate([
                _bf(he[xr, :]), jnp.concatenate([mem, z8], axis=0).astype(BF16),
                _bf(xo[xr, :]), jnp.concatenate([pltpu.roll(mem, DP - DM, 1), z8], axis=0).astype(BF16),
            ], axis=0)
            sc = _dot_nt(tq, keys)
            yield
            kw = SEG + 16
            ri = jax.lax.broadcasted_iota(jnp.int32, sc.shape, 0)
            ci = jax.lax.broadcasted_iota(jnp.int32, sc.shape, 1)
            lo = ((ri // M) % 2) * kw
            sc = jnp.where((ci >= lo) & (ci < lo + SEG + M), sc, NEG)
            p = jnp.exp2(sc - jnp.max(sc, axis=1, keepdims=True))
            p = p / jnp.sum(p, axis=1, keepdims=True)
            z = _dot(p.astype(BF16), keys)
            yield
            zt = []
            for i in range(NP):
                ze = z[2 * i * M:(2 * i + 1) * M]
                zo = z[(2 * i + 1) * M:(2 * i + 2) * M]
                zt += [ze[:, 0:128], ze[:, 128:256], ze[:, 256:384], ze[:, 384:] + zo[:, :128],
                       zo[:, 128:256], zo[:, 256:384], zo[:, 384:]]
            acc = [None] * 4
            for g in range(0, NT_, 8):
                for t0 in (g, g + 4):
                    zp = jnp.concatenate(zt[t0:t0 + 4], axis=1).astype(BF16).astype(F32)
                    for n in range(KM // 128):
                        d = _dot(zp, _bf(wvo[_half((t0 + zero) * 128, 512), n * 128:(n + 1) * 128]))
                        acc[n] = d if acc[n] is None else acc[n] + d
                        yield
                zp = jnp.concatenate([jnp.concatenate(zt[g:g + 8:2], axis=1),
                                      jnp.concatenate(zt[g + 1:g + 8:2], axis=1)], axis=0).astype(BF16)
                d = _dot(zp, _bf(wvo_t[_half((g // 2 + zero) * 128, 512), :]))
                acc[3] = d if acc[3] is None else acc[3] + d
                if g + 8 < NT_:
                    yield
            lane = jax.lax.broadcasted_iota(jnp.int32, (M, 128), 1)
            last = jnp.where(lane < 64, acc[3][:M] + pltpu.roll(acc[3][M:], 64, 1), 0.0)
            new = jnp.concatenate(acc[:3] + [last], axis=1).astype(BF16).astype(F32)
            memall[pl.ds(pl.multiple_of((s + 1) * M, M), M), :] = new
            yield

        def chain(h):
            for j in range(STEPS):
                yield from chain_step(h * STEPS + j)

        def b_head(h):
            i = h // 2
            par = h % 2
            wq_s[...] = _u32(_unpack(bwq[i], par))
            wk_s[...] = _u32(_unpack(bwk[i], par))
            wv_s[...] = _u32(_unpack(bwv[i], par))
            qs, ss, ctxs = {}, {}, {}

            def chunks(r):
                nk = (r + 1) * QB
                return [(c0, min(c0 + 256, nk)) for c0 in range(0, nk, 256)]

            def project(r):
                rows = _half(r * QB, QB)
                acc = None
                for k0, k1 in ((0, 256), (256, DM)):
                    d = _dot(_bf(bx[rows, k0:k0 + 256])[:, :k1 - k0], _bf(wq_s[_half(k0, k1 - k0), :]))
                    acc = d if acc is None else acc + d
                    if k1 == DM:
                        qs[r] = (acc * QSC).astype(BF16)
                    yield
                for w_s, dst in ((wk_s, k_s), (wv_s, v_s)):
                    acc = None
                    for k0 in range(0, DC, 256):
                        d = _dot(_bf(ckv[rows, k0:k0 + 256]), _bf(w_s[_half(k0, 256), :]))
                        acc = d if acc is None else acc + d
                        if k0 + 256 == DC:
                            dst[rows, :] = _u32(acc)
                        yield

            def scores(r):
                ss[r] = []
                for c0, c1 in chunks(r):
                    sc = _dot_nt(qs[r], _bf(k_s[_half(c0, c1 - c0), :]))
                    if c1 == (r + 1) * QB:
                        ri = jax.lax.broadcasted_iota(jnp.int32, sc.shape, 0) + r * QB
                        ci = jax.lax.broadcasted_iota(jnp.int32, sc.shape, 1) + c0
                        sc = jnp.where(ci <= ri, sc, NEG)
                    ss[r].append(sc)
                    yield

            def context(r):
                m = None
                for sc in ss[r]:
                    for t0 in range(0, sc.shape[1], 128):
                        m = sc[:, t0:t0 + 128] if m is None else jnp.maximum(m, sc[:, t0:t0 + 128])
                m = jnp.max(m, axis=1, keepdims=True)
                l = None
                acc = None
                for (c0, c1), sc in zip(chunks(r), ss[r]):
                    p = jnp.exp2(sc - m)
                    for t0 in range(0, p.shape[1], 128):
                        l = p[:, t0:t0 + 128] if l is None else l + p[:, t0:t0 + 128]
                    d = _dot(p.astype(BF16), _bf(v_s[_half(c0, c1 - c0), :]))
                    acc = d if acc is None else acc + d
                    if c1 == (r + 1) * QB:
                        ctxs[r] = (acc / jnp.sum(l, axis=1, keepdims=True)).astype(BF16)
                    yield

            def output(r):
                ctx = jnp.concatenate([ctxs[r - 1], ctxs[r]], axis=0)
                cols = pl.ds((r - 1) * QB, 2 * QB)
                for n0 in range(0, DM, OB):
                    accb[n0:n0 + OB, cols] += _dot_nt(_bf(bwo[h, _half(n0, OB), :]), ctx)
                    yield

            nb = S // QB
            for r in range(nb + 3):
                parts = []
                if r < nb:
                    parts.append((project(r), 2 + 2 * DC // 256))
                if 0 <= r - 3 < nb and (r - 3) % 2 == 1:
                    parts.append((output(r - 3), DM // OB))
                if 0 <= r - 1 < nb:
                    parts.append((scores(r - 1), len(chunks(r - 1))))
                if 0 <= r - 2 < nb:
                    parts.append((context(r - 2), len(chunks(r - 2))))
                yield from _merge(*parts)

        n_chain = STEPS * (NT_ // 8 * 7 * 2 + 2)
        n_head = (S // QB) * (2 * DC // 256 + 4) + 2 * sum((r + 2) // 2 for r in range(S // QB))

        def b_body(h, c):
            i = h // 2

            @pl.when(h % 2 == 0)
            def _():
                pair_copy(bwq_h, bwq, sem_bq, i).wait()
                pair_copy(bwk_h, bwk, sem_bk, i).wait()
                pair_copy(bwv_h, bwv, sem_bv, i).wait()
                wo_copy(bwo_h, bwo, sem_bo, i).wait()
            for _ in _merge((chain(h), n_chain), (b_head(h), n_head)):
                pass
            return c
        with jax.named_scope('b_body'):
            jax.lax.fori_loop(0, H, b_body, 0)

        he[_half(S, NSEG * M), :] = _u32(memall[pl.ds(0, NSEG * M), :])
        AB = 2 * SEG
        ri = jax.lax.broadcasted_iota(jnp.int32, (AB, AB + 2 * M), 0)
        ci = jax.lax.broadcasted_iota(jnp.int32, (AB, AB + 2 * M), 1)
        amask = ((ci < AB) & ((ci // SEG) == (ri // SEG)) & (ci <= ri)) | ((ci >= AB) & (((ci - AB) // M) == (ri // SEG)))

        def a_body(h, c):
            i = h // 2
            par = h % 2
            wk = _unpack(awk[i], par)
            wv = _unpack(awv[i], par)
            for r in range((S + NSEG * M) // 512):
                rows = _half(r * 512, 512)
                x = _bf(he[rows, :])[:, :DM]
                k_s[rows, :] = _u32(_dot(x, wk))
                v_s[rows, :] = _u32(_dot(x, wv))
            for r in range(S // 512):
                ctxs = []
                for j in range(r * 512 // AB, (r + 1) * 512 // AB):
                    xr = _half(j * AB, AB)
                    mr = _half(S + j * 2 * M, 2 * M)
                    kc = _bf(jnp.concatenate([k_s[xr, :], k_s[mr, :]], axis=0))
                    vc = _bf(jnp.concatenate([v_s[xr, :], v_s[mr, :]], axis=0))
                    sc = jnp.where(amask, _dot_nt(_bf(qa[h, xr, :]), kc), NEG)
                    p = jnp.exp2(sc - jnp.max(sc, axis=1, keepdims=True))
                    p = p / jnp.sum(p, axis=1, keepdims=True)
                    ctxs.append(_dot(p.astype(BF16), vc).astype(BF16))
                acca[:, pl.ds(r * 512, 512)] += _dot_nt(_bf(awo[h]), jnp.concatenate(ctxs, axis=0))
            return c
        with jax.named_scope('a_body'):
            jax.lax.fori_loop(0, H, a_body, 0)

        cps = []
        for r in range(S // 512):
            cols = pl.ds(r * 512, 512)
            rows = _half(r * 512, 512)
            ostage[rows, :] = _u32(jnp.concatenate([acca[:, cols], accb[:, cols]], axis=0).astype(BF16).T)
            cp = pltpu.make_async_copy(ostage.at[rows, :], out_h.bitcast(U32).at[0, rows, :], sem_out.at[r])
            cp.start()
            cps.append(cp)
        for cp in cps:
            cp.wait()

    def packed(*shape):
        return pltpu.VMEM(shape[:-2] + (shape[-2] // 2, shape[-1]), U32)

    scratch = [
        packed(DM, S),
        packed(S + NSEG * M, DP),
        packed(S, DP),
        pltpu.VMEM((M, DM), BF16),
        pltpu.VMEM(((NSEG + 1) * M, DP), F32),
        pltpu.VMEM((NP, DM, DH), U32),
        pltpu.VMEM((NP, DM, DH), U32),
        pltpu.VMEM((NP, DM, DH), U32),
        packed(H, DM, DH),
        packed(NT_, KM, 128),
        packed(NT_ // 2, 128, 128),
        packed(NT_ * 128, DP),
        packed(NT_ * 64, 128),
        packed(H, S, DH),
        packed(DM, S),
        packed(S, DP),
        packed(S, DC),
        pltpu.VMEM((NP, DM, DH), U32),
        pltpu.VMEM((NP, DC, DH), U32),
        pltpu.VMEM((NP, DC, DH), U32),
        packed(H, DM, DH),
        packed(DM, DH),
        packed(DC, DH),
        packed(DC, DH),
        packed(S + NSEG * M, DH),
        packed(S + NSEG * M, DH),
        pltpu.VMEM((DM, S), F32),
        pltpu.VMEM((DM, S), F32),
        packed(S, 2 * DM),
        pltpu.SemaphoreType.DMA((4,)),
    ] + [pltpu.SemaphoreType.DMA((NP,)) for _ in range(8)] + [pltpu.SemaphoreType.DMA((S // 512,))]
    return kernel, scratch


@jax.jit
def pallas_concat_heads__memory_aug_recurrent_mem_tr__compressed_kv_cla__prompt_kernel(
    A_x, A_mem0, A_Wq, A_Wk, A_Wv, A_Wo, A_seg_len, B_x, B_c_kv, B_w_q, B_w_uk, B_w_uv, B_w_o,
):
    del A_seg_len
    _, S, DM = A_x.shape
    M = A_mem0.shape[1]
    H, DH = A_Wq.shape[1], A_Wq.shape[2]
    DC = B_c_kv.shape[2]
    kernel, scratch = _make_kernel(S, DM, H, DH, M, 32, DC)
    return pl.pallas_call(
        kernel,
        out_shape=jax.ShapeDtypeStruct((1, S, 2 * DM), BF16),
        in_specs=[pl.BlockSpec(memory_space=pl.ANY)] * 12,
        out_specs=pl.BlockSpec(memory_space=pl.ANY),
        scratch_shapes=scratch,
        compiler_params=pltpu.CompilerParams(vmem_limit_bytes=124 * 1024 * 1024),
    )(A_x[0].T, A_mem0, A_Wq, A_Wk, A_Wv, A_Wo.transpose(0, 2, 1),
      B_x[0].T, B_c_kv, B_w_q, B_w_uk, B_w_uv, B_w_o.transpose(0, 2, 1))
```

```python
import numpy as np
import jax
import jax.numpy as jnp
import jax.experimental.pallas as pl
import jax.experimental.pallas.tpu as pltpu

F32 = jnp.float32
BF16 = jnp.bfloat16
U32 = jnp.uint32
LOG2E = 1.4426950408889634
NEG = -1e30
NN = (((1,), (0,)), ((), ()))
NT = (((1,), (1,)), ((), ()))


def _dot(a, b):
    return jax.lax.dot_general(a, b, NN, preferred_element_type=F32)


def _dot_nt(a, b):
    return jax.lax.dot_general(a, b, NT, preferred_element_type=F32)


def _bf(u):
    return pltpu.bitcast(u, BF16)


def _u32(x):
    return pltpu.bitcast(x.astype(BF16), U32)


def _half(start, size):
    if isinstance(start, int):
        return pl.ds(start // 2, size // 2)
    return pl.ds(pl.multiple_of(start // 2, 8), size // 2)


def _unpack(u, parity):
    if isinstance(parity, int):
        w = (u << 16) if parity == 0 else (u & jnp.uint32(0xFFFF0000))
    else:
        w = (u >> (16 * parity).astype(U32)) << 16
    return pltpu.bitcast(w, F32).astype(BF16)


def _merge(*streams):
    streams = [(g, n) for g, n in streams if n > 0]
    done = [0] * len(streams)
    order = []
    for _ in range(sum(n for _, n in streams)):
        j = min(range(len(streams)), key=lambda a: ((done[a] + 0.5) / streams[a][1], a))
        done[j] += 1
        order.append(j)
    started = set()
    for j in order:
        if j not in started:
            next(streams[j][0])
            started.add(j)
        yield
        next(streams[j][0], None)
    for g, _ in streams:
        for _ in g:
            raise AssertionError("stream longer than announced")


def _make_kernel(S, DM, H, DH, M, SEG, DC):
    NP = H // 2
    NSEG = S // SEG
    DP = 512
    PW = 2 * DM
    PT = PW // 128
    NT_ = NP * PT
    KM = DM // 128 * 128
    STEPS = NSEG // H
    QB = 128
    OB = DM // 4
    MBQ, MBK, MBV = 64, 64, 64
    GAPS = (2, 3, 2, 2)
    n_proj = 2 * (QB // MBQ) + (DC // 256) * (QB // MBK + QB // MBV)
    QSC = LOG2E * DH ** -0.5

    def kernel(ax_h, mem_h, awq_h, awk_h, awv_h, awo_h, bx_h, ckv_h, bwq_h, bwk_h, bwv_h, bwo_h,
               out_h,
               xraw, he, xo, mem0, memall, awq, awk, awv, awo, wqk, wqk_t, wvo, wvo_t, qa,
               bxraw, bx, ckv, bwq, bwk, bwv, bwo,
               wq_s, wk_s, wv_s, k_s, v_s, acca, accb, ostage,
               sem_x, sem_aq, sem_ak, sem_av, sem_ao, sem_bq, sem_bk, sem_bv, sem_bo, sem_out):

        def pair_copy(src, dst, sem, i):
            return pltpu.make_async_copy(src.bitcast(U32).at[:, i, :], dst.at[i], sem.at[i])

        def wo_copy(src, dst, sem, i):
            return pltpu.make_async_copy(src.bitcast(U32).at[pl.ds(2 * i, 2)], dst.at[pl.ds(2 * i, 2)], sem.at[i])

        cp_ax = pltpu.make_async_copy(ax_h.bitcast(U32), xraw, sem_x.at[0])
        cp_mem = pltpu.make_async_copy(mem_h.at[0], mem0, sem_x.at[1])
        cp_bx = pltpu.make_async_copy(bx_h.bitcast(U32), bxraw, sem_x.at[2])
        cp_ckv = pltpu.make_async_copy(ckv_h.bitcast(U32).at[0], ckv, sem_x.at[3])

        cp_ax.start()
        cp_mem.start()
        for i in range(NP):
            pair_copy(awq_h, awq, sem_aq, i).start()
        for i in range(NP):
            pair_copy(awk_h, awk, sem_ak, i).start()
            pair_copy(awv_h, awv, sem_av, i).start()
            wo_copy(awo_h, awo, sem_ao, i).start()
        cp_bx.start()
        cp_ckv.start()
        for i in range(NP):
            pair_copy(bwq_h, bwq, sem_bq, i).start()
            pair_copy(bwk_h, bwk, sem_bk, i).start()
            pair_copy(bwv_h, bwv, sem_bv, i).start()
            wo_copy(bwo_h, bwo, sem_bo, i).start()

        accb[...] = jnp.zeros(accb.shape, F32)
        acca[...] = jnp.zeros(acca.shape, F32)

        cp_ax.wait()

        def pad_body(r, c):
            xt = _bf(xraw[:, pl.ds(pl.multiple_of(r * 256, 256), 256)])
            zpad = jnp.zeros((DP - DM, 256), BF16)
            he[_half(r * 256, 256), :] = _u32(jnp.concatenate([xt, zpad], axis=0).T)
            xo[_half(r * 256, 256), :] = _u32(jnp.concatenate([zpad, xt], axis=0).T)
            return c
        with jax.named_scope('pad_body'):
            jax.lax.fori_loop(0, S // 256, pad_body, 0)

        def qa_body(i, c):
            pair_copy(awq_h, awq, sem_aq, i).wait()
            u = awq[i]
            for par in range(2):
                w = _unpack(u, par)
                for r in range(S // 512):
                    rows = _half(r * 512, 512)
                    qa[2 * i + par, rows, :] = _u32(_dot(_bf(he[rows, :])[:, :DM], w) * QSC)
            return c
        with jax.named_scope('qa_body'):
            jax.lax.fori_loop(0, NP, qa_body, 0)

        def absorb_body(i, c):
            pair_copy(awk_h, awk, sem_ak, i).wait()
            pair_copy(awv_h, awv, sem_av, i).wait()
            wo_copy(awo_h, awo, sem_ao, i).wait()
            uq, uk, uv = awq[i], awk[i], awv[i]
            zpad = jnp.zeros((DP - DM, DH), BF16)
            e = _dot_nt(_unpack(uq, 0), jnp.concatenate([_unpack(uk, 0), zpad], axis=0)) * QSC
            o = _dot_nt(_unpack(uq, 1), jnp.concatenate([zpad, _unpack(uk, 1)], axis=0)) * QSC
            slab = _u32(jnp.concatenate([e[:, :DP - 128], e[:, DP - 128:] + o[:, :128], o[:, 128:]], axis=1))
            for j in range(PT):
                t = PT * i + j
                wqk[t] = slab[:KM // 2, j * 128:(j + 1) * 128]
                wqk_t[t // 2, _half((t % 2) * 64, 64), :] = slab[KM // 2:, j * 128:(j + 1) * 128]
            for par in range(2):
                r = _dot_nt(_unpack(uv, par), jnp.concatenate([_bf(awo[2 * i + par]), zpad], axis=0))
                wvo[_half((2 * i + par) * DM, DM), :] = _u32(r)
            return c
        with jax.named_scope('absorb_body'):
            jax.lax.fori_loop(0, NP, absorb_body, 0)


        def tail_body(j, c):
            wvo_t[_half(j * 128, 128), :] = (wvo[_half(2 * j * 128, 128), KM:]
                                             | pltpu.roll(wvo[_half((2 * j + 1) * 128, 128), KM:], 64, 1))
            return c
        jax.lax.fori_loop(0, NT_ // 2, tail_body, 0)

        cp_mem.wait()
        memall[pl.ds(0, M), :] = jnp.concatenate([mem0[...].astype(F32), jnp.zeros((M, DP - DM), F32)], axis=1)
        cp_bx.wait()
        cp_ckv.wait()

        def bx_body(r, c):
            xt = _bf(bxraw[:, pl.ds(pl.multiple_of(r * 256, 256), 256)])
            bx[_half(r * 256, 256), :] = _u32(jnp.concatenate([xt, jnp.zeros((DP - DM, 256), BF16)], axis=0).T)
            return c
        with jax.named_scope('bx_body'):
            jax.lax.fori_loop(0, S // 256, bx_body, 0)


        def zeros(i, shape):
            return jnp.full(shape, (i >> 10).astype(F32))

        def chain_step(s):
            mem = memall[pl.ds(pl.multiple_of(s * M, M), M), :]
            zero = s >> 10
            mt = mem[:, KM:]
            mtail = jnp.concatenate([mt, pltpu.roll(mt, 64, 1)], axis=0).astype(BF16)
            t = []
            for g in range(0, NT_, 8):
                for t0 in (g, g + 4):
                    acc = zeros(s, (M, 512))
                    for k0 in range(0, KM, 128):
                        w = jnp.concatenate([wqk[t0 + j + zero, _half(k0, 128), :] for j in range(4)], axis=1)
                        yield
                        acc = acc + _dot(mem[:, k0:k0 + 128], _bf(w))
                    t += [acc[:, j * 128:(j + 1) * 128] for j in range(4)]
                w = jnp.concatenate([wqk_t[g // 2 + j + zero] for j in range(4)], axis=1)
                yield
                d = _dot(mtail, _bf(w))
                for j in range(8):
                    t[g + j] = t[g + j] + d[(j % 2) * M:(j % 2 + 1) * M, (j // 2) * 128:(j // 2 + 1) * 128]
            for _ in range(GAPS[0]):
                yield
            tq = jnp.concatenate([jnp.concatenate(t[h * PT // 2:h * PT // 2 + 4], axis=1) for h in range(H)],
                                 axis=0).astype(BF16)
            xr = _half(s * SEG, SEG)
            z8 = jnp.zeros((16 - M, DP), F32)
            keys = jnp.concatenate([
                _bf(he[xr, :]), jnp.concatenate([mem, z8], axis=0).astype(BF16),
                _bf(xo[xr, :]), jnp.concatenate([pltpu.roll(mem, DP - DM, 1), z8], axis=0).astype(BF16),
            ], axis=0)
            yield
            sc = _dot_nt(tq, keys)
            for _ in range(GAPS[1]):
                yield
            kw = SEG + 16
            ri = jax.lax.broadcasted_iota(jnp.int32, sc.shape, 0)
            ci = jax.lax.broadcasted_iota(jnp.int32, sc.shape, 1)
            lo = ((ri // M) % 2) * kw
            sc = jnp.where((ci >= lo) & (ci < lo + SEG + M), sc, NEG)
            p = jnp.exp2(sc - jnp.max(sc, axis=1, keepdims=True))
            p = (p / jnp.sum(p, axis=1, keepdims=True)).astype(BF16)
            yield
            z = _dot(p, keys)
            for _ in range(GAPS[2]):
                yield
            zt = []
            for i in range(NP):
                ze = z[2 * i * M:(2 * i + 1) * M]
                zo = z[(2 * i + 1) * M:(2 * i + 2) * M]
                zt += [ze[:, 0:128], ze[:, 128:256], ze[:, 256:384], ze[:, 384:] + zo[:, :128],
                       zo[:, 128:256], zo[:, 256:384], zo[:, 384:]]
            acc = [zeros(s, (M, 128))] * 3 + [zeros(s, (2 * M, 128))]
            for g in range(0, NT_, 8):
                for t0 in (g, g + 4):
                    zp = jnp.concatenate(zt[t0:t0 + 4], axis=1).astype(BF16).astype(F32)
                    for n in range(KM // 128):
                        w = wvo[_half((t0 + zero) * 128, 512), n * 128:(n + 1) * 128]
                        yield
                        acc[n] = acc[n] + _dot(zp, _bf(w))
                zp = jnp.concatenate([jnp.concatenate(zt[g:g + 8:2], axis=1),
                                      jnp.concatenate(zt[g + 1:g + 8:2], axis=1)], axis=0).astype(BF16)
                w = wvo_t[_half((g // 2 + zero) * 128, 512), :]
                yield
                acc[3] = acc[3] + _dot(zp, _bf(w))
            lane = jax.lax.broadcasted_iota(jnp.int32, (M, 128), 1)
            last = jnp.where(lane < 64, acc[3][:M] + pltpu.roll(acc[3][M:], 64, 1), 0.0)
            new = jnp.concatenate(acc[:3] + [last], axis=1).astype(BF16).astype(F32)
            memall[pl.ds(pl.multiple_of((s + 1) * M, M), M), :] = new
            for _ in range(GAPS[3]):
                yield

        def chain(h):
            for j in range(STEPS):
                yield from chain_step(h * STEPS + j)

        def b_head(h):
            i = h // 2
            par = h % 2
            wq_s[...] = _u32(_unpack(bwq[i], par))
            wk_s[...] = _u32(_unpack(bwk[i], par))
            wv_s[...] = _u32(_unpack(bwv[i], par))
            qs, ss, ctxs = {}, {}, {}

            def chunks(r):
                nk = (r + 1) * QB
                return [(c0, min(c0 + 256, nk)) for c0 in range(0, nk, 256)]

            def project(r):
                qp = []
                for r0 in range(r * QB, (r + 1) * QB, MBQ):
                    rows = _half(r0, MBQ)
                    acc = zeros(h, (MBQ, DH))
                    for k0, k1 in ((0, 256), (256, DM)):
                        x = _bf(bx[rows, k0:k0 + 256])[:, :k1 - k0]
                        w = _bf(wq_s[_half(k0, k1 - k0), :])
                        yield
                        acc = acc + _dot(x, w)
                    qp.append((acc * QSC).astype(BF16))
                qs[r] = jnp.concatenate(qp, axis=0)
                for w_s, dst, mb in ((wk_s, k_s, MBK), (wv_s, v_s, MBV)):
                    for r0 in range(r * QB, (r + 1) * QB, mb):
                        rows = _half(r0, mb)
                        acc = zeros(h, (mb, DH))
                        for k0 in range(0, DC, 256):
                            x = _bf(ckv[rows, k0:k0 + 256])
                            w = _bf(w_s[_half(k0, 256), :])
                            yield
                            acc = acc + _dot(x, w)
                        dst[rows, :] = _u32(acc)

            def scores(r):
                ss[r] = []
                zero = (h + r) >> 10
                for c0, c1 in chunks(r):
                    k = _bf(k_s[_half(c0 + zero, c1 - c0), :])
                    yield
                    sc = _dot_nt(qs[r], k)
                    if c1 == (r + 1) * QB:
                        ri = jax.lax.broadcasted_iota(jnp.int32, sc.shape, 0) + r * QB
                        ci = jax.lax.broadcasted_iota(jnp.int32, sc.shape, 1) + c0
                        sc = jnp.where(ci <= ri, sc, NEG)
                    ss[r].append(sc)

            def context(r):
                m = None
                for sc in ss[r]:
                    for t0 in range(0, sc.shape[1], 128):
                        m = sc[:, t0:t0 + 128] if m is None else jnp.maximum(m, sc[:, t0:t0 + 128])
                m = jnp.max(m, axis=1, keepdims=True)
                l = None
                acc = zeros(h, (QB, DH))
                for (c0, c1), sc in zip(chunks(r), ss[r]):
                    p = jnp.exp2(sc - m)
                    for t0 in range(0, p.shape[1], 128):
                        l = p[:, t0:t0 + 128] if l is None else l + p[:, t0:t0 + 128]
                    p = p.astype(BF16)
                    v = _bf(v_s[_half(c0, c1 - c0), :])
                    yield
                    acc = acc + _dot(p, v)
                ctxs[r] = (acc / jnp.sum(l, axis=1, keepdims=True)).astype(BF16)

            def output(r):
                ctx = jnp.concatenate([ctxs[r - 1], ctxs[r]], axis=0)
                cols = pl.ds((r - 1) * QB, 2 * QB)
                zero = (h + r) >> 10
                for n0 in range(0, DM, OB):
                    w = _bf(bwo[h + zero, _half(n0, OB), :])
                    yield
                    accb[n0:n0 + OB, cols] += _dot_nt(w, ctx)

            nb = S // QB
            for r in range(nb + 3):
                parts = []
                if r < nb:
                    parts.append((project(r), n_proj))
                if 0 <= r - 3 < nb and (r - 3) % 2 == 1:
                    parts.append((output(r - 3), DM // OB))
                if 0 <= r - 1 < nb:
                    parts.append((scores(r - 1), len(chunks(r - 1))))
                if 0 <= r - 2 < nb:
                    parts.append((context(r - 2), len(chunks(r - 2))))
                yield from _merge(*parts)

        n_chain = STEPS * (NT_ // 8 * 7 * 2 + 2 + sum(GAPS))
        n_head = (S // QB) * (n_proj + DM // OB // 2) + 2 * sum((r + 2) // 2 for r in range(S // QB))

        def b_body(h, c):
            i = h // 2

            @pl.when(h % 2 == 0)
            def _():
                pair_copy(bwq_h, bwq, sem_bq, i).wait()
                pair_copy(bwk_h, bwk, sem_bk, i).wait()
                pair_copy(bwv_h, bwv, sem_bv, i).wait()
                wo_copy(bwo_h, bwo, sem_bo, i).wait()
            for _ in _merge((chain(h), n_chain), (b_head(h), n_head)):
                pass
            return c
        with jax.named_scope('b_body'):
            jax.lax.fori_loop(0, H, b_body, 0)

        he[_half(S, NSEG * M), :] = _u32(memall[pl.ds(0, NSEG * M), :])
        AB = 2 * SEG
        ri = jax.lax.broadcasted_iota(jnp.int32, (AB, AB + 2 * M), 0)
        ci = jax.lax.broadcasted_iota(jnp.int32, (AB, AB + 2 * M), 1)
        amask = ((ci < AB) & ((ci // SEG) == (ri // SEG)) & (ci <= ri)) | ((ci >= AB) & (((ci - AB) // M) == (ri // SEG)))

        def a_body(h, c):
            i = h // 2
            par = h % 2
            wk = _unpack(awk[i], par)
            wv = _unpack(awv[i], par)
            RB = 512
            ps, ctxs = {}, {}

            def project(r):
                rows = _half(r * RB, RB)
                x = _bf(he[rows, :])[:, :DM]
                k_s[rows, :] = _u32(_dot(x, wk))
                v_s[rows, :] = _u32(_dot(x, wv))

            def window(ref, j):
                return _bf(jnp.concatenate([ref[_half(j * AB, AB), :], ref[_half(S + j * 2 * M, 2 * M), :]], axis=0))

            def scores(r):
                ps[r] = []
                for j in range(r * RB // AB, (r + 1) * RB // AB):
                    sc = jnp.where(amask, _dot_nt(_bf(qa[h, _half(j * AB, AB), :]), window(k_s, j)), NEG)
                    p = jnp.exp2(sc - jnp.max(sc, axis=1, keepdims=True))
                    ps[r].append((p / jnp.sum(p, axis=1, keepdims=True)).astype(BF16))

            def context(r):
                ctxs[r] = jnp.concatenate(
                    [_dot(p, window(v_s, r * RB // AB + j)).astype(BF16) for j, p in enumerate(ps[r])], axis=0)

            def output(r, c0=0, c1=RB):
                acca[:, r * RB + c0:r * RB + c1] += _dot_nt(_bf(awo[h]), ctxs[r][c0:c1])

            nr = S // RB
            project(nr)
            project(0)
            for r in range(nr):
                scores(r)
                if r > 0:
                    output(r - 1, 0, RB if r + 1 < nr else RB // 2)
                if r + 1 < nr:
                    project(r + 1)
                context(r)
            output(nr - 2, RB // 2, RB)
            output(nr - 1)
            return c
        with jax.named_scope('a_body'):
            jax.lax.fori_loop(0, H, a_body, 0)

        cps = []
        for r in range(S // 512):
            cols = pl.ds(r * 512, 512)
            rows = _half(r * 512, 512)
            ostage[rows, :] = _u32(jnp.concatenate([acca[:, cols], accb[:, cols]], axis=0).astype(BF16).T)
            cp = pltpu.make_async_copy(ostage.at[rows, :], out_h.bitcast(U32).at[0, rows, :], sem_out.at[r])
            cp.start()
            cps.append(cp)
        for cp in cps:
            cp.wait()

    def packed(*shape):
        return pltpu.VMEM(shape[:-2] + (shape[-2] // 2, shape[-1]), U32)

    scratch = [
        packed(DM, S),
        packed(S + NSEG * M, DP),
        packed(S, DP),
        pltpu.VMEM((M, DM), BF16),
        pltpu.VMEM(((NSEG + 1) * M, DP), F32),
        pltpu.VMEM((NP, DM, DH), U32),
        pltpu.VMEM((NP, DM, DH), U32),
        pltpu.VMEM((NP, DM, DH), U32),
        packed(H, DM, DH),
        packed(NT_, KM, 128),
        packed(NT_ // 2, 128, 128),
        packed(NT_ * 128, DP),
        packed(NT_ * 64, 128),
        packed(H, S, DH),
        packed(DM, S),
        packed(S, DP),
        packed(S, DC),
        pltpu.VMEM((NP, DM, DH), U32),
        pltpu.VMEM((NP, DC, DH), U32),
        pltpu.VMEM((NP, DC, DH), U32),
        packed(H, DM, DH),
        packed(DM, DH),
        packed(DC, DH),
        packed(DC, DH),
        packed(S + NSEG * M, DH),
        packed(S + NSEG * M, DH),
        pltpu.VMEM((DM, S), F32),
        pltpu.VMEM((DM, S), F32),
        packed(S, 2 * DM),
        pltpu.SemaphoreType.DMA((4,)),
    ] + [pltpu.SemaphoreType.DMA((NP,)) for _ in range(8)] + [pltpu.SemaphoreType.DMA((S // 512,))]
    return kernel, scratch


@jax.jit
def pallas_concat_heads__memory_aug_recurrent_mem_tr__compressed_kv_cla__prompt_kernel(
    A_x, A_mem0, A_Wq, A_Wk, A_Wv, A_Wo, A_seg_len, B_x, B_c_kv, B_w_q, B_w_uk, B_w_uv, B_w_o,
):
    del A_seg_len
    _, S, DM = A_x.shape
    M = A_mem0.shape[1]
    H, DH = A_Wq.shape[1], A_Wq.shape[2]
    DC = B_c_kv.shape[2]
    kernel, scratch = _make_kernel(S, DM, H, DH, M, 32, DC)
    return pl.pallas_call(
        kernel,
        out_shape=jax.ShapeDtypeStruct((1, S, 2 * DM), BF16),
        in_specs=[pl.BlockSpec(memory_space=pl.ANY)] * 12,
        out_specs=pl.BlockSpec(memory_space=pl.ANY),
        scratch_shapes=scratch,
        compiler_params=pltpu.CompilerParams(vmem_limit_bytes=124 * 1024 * 1024),
    )(A_x[0].T, A_mem0, A_Wq, A_Wk, A_Wv, A_Wo.transpose(0, 2, 1),
      B_x[0].T, B_c_kv, B_w_q, B_w_uk, B_w_uv, B_w_o.transpose(0, 2, 1))
```

```python
import jax
import jax.numpy as jnp
import jax.experimental.pallas as pl
import jax.experimental.pallas.tpu as pltpu

F32 = jnp.float32
BF16 = jnp.bfloat16
U32 = jnp.uint32
LOG2E = 1.4426950408889634
NEG = -1e30
NN = (((1,), (0,)), ((), ()))
NT = (((1,), (1,)), ((), ()))


def _dot(a, b):
    return jax.lax.dot_general(a, b, NN, preferred_element_type=F32)


def _dot_nt(a, b):
    return jax.lax.dot_general(a, b, NT, preferred_element_type=F32)


def _bf(u):
    return pltpu.bitcast(u, BF16)


def _u32(x):
    return pltpu.bitcast(x.astype(BF16), U32)


def _half(start, size):
    if isinstance(start, int):
        return pl.ds(start // 2, size // 2)
    return pl.ds(pl.multiple_of(start // 2, 8), size // 2)


def _unpack(u, parity):
    if isinstance(parity, int):
        w = (u << 16) if parity == 0 else (u & jnp.uint32(0xFFFF0000))
    else:
        w = (u >> (16 * parity).astype(U32)) << 16
    return pltpu.bitcast(w, F32).astype(BF16)


def _zeros(i, shape):
    return jnp.full(shape, (i >> 10).astype(F32))


def _softmax2(sc):
    p = jnp.exp2(sc - jnp.max(sc, axis=1, keepdims=True))
    return (p / jnp.sum(p, axis=1, keepdims=True)).astype(BF16)


def _merge(*streams):
    streams = [(g, n) for g, n in streams if n > 0]
    done = [0] * len(streams)
    order = []
    for _ in range(sum(n for _, n in streams)):
        j = min(range(len(streams)), key=lambda a: ((done[a] + 0.5) / streams[a][1], a))
        done[j] += 1
        order.append(j)
    started = set()
    for j in order:
        if j not in started:
            next(streams[j][0])
            started.add(j)
        yield
        next(streams[j][0], None)
    for g, _ in streams:
        for _ in g:
            raise AssertionError("stream longer than announced")


def _make_kernel(S, DM, H, DH, M, SEG, DC):
    NP = H // 2
    NSEG = S // SEG
    DP = 512
    KM = DM // 128 * 128
    HT = DH // 128
    PT = 6 * HT
    STEPS = NSEG // H
    QB = 128
    OB = DM // 4
    MBQ, MBK, MBV = 64, 64, 64
    GAPS = (2, 3, 2, 2)
    RB = 512
    AB = 2 * SEG
    QSC = LOG2E * DH ** -0.5

    def packed(*shape):
        return pltpu.VMEM(shape[:-2] + (shape[-2] // 2, shape[-1]), U32)

    def kernel(ax_h, mem_h, awq_h, awk_h, awv_h, awo_h, bx_h, ckv_h, bwq_h, bwk_h, bwv_h, bwo_h,
               out_h,
               ax, mem_s, awo, wqkv, wqkv_t, wo, wo_t, kx, vx, km, vm,
               bx, ckv, bwq, bwk, bwv, bwo, accb,
               sem_x, sem_aq, sem_ak, sem_av, sem_ao, sem_bq, sem_bk, sem_bv, sem_bo, sem_out):

        def pair_copy(src, dst, sem, i):
            return pltpu.make_async_copy(src.bitcast(U32).at[:, i, :], dst.at[i], sem.at[i])

        def wo_copy(src, dst, sem, i):
            return pltpu.make_async_copy(src.bitcast(U32).at[pl.ds(2 * i, 2)], dst.at[pl.ds(2 * i, 2)], sem.at[i])

        def head_weight(t):
            return _bf(jnp.concatenate(
                [jnp.concatenate([wqkv[t + j], wqkv_t[t // 2 + j // 2, _half((j % 2) * 64, 64), :]], axis=0)
                 for j in range(HT)], axis=1))

        def transposed(raw, c):
            xt = _bf(raw[:, pl.ds(c if isinstance(c, int) else pl.multiple_of(c, 256), 256)])
            return _u32(jnp.concatenate([xt, jnp.zeros((DP - DM, 256), BF16)], axis=0).T)

        def phase1(axraw, bxraw, mem0, awq, awk, awv):
            cp_ax = [pltpu.make_async_copy(ax_h.bitcast(U32).at[:, pl.ds(r * RB, RB)],
                                           axraw.at[:, pl.ds(r * RB, RB)], sem_x.at[3 + r]) for r in range(S // RB)]
            cp_mem = pltpu.make_async_copy(mem_h.at[0], mem0, sem_x.at[0])
            cp_bx = pltpu.make_async_copy(bx_h.bitcast(U32), bxraw, sem_x.at[1])
            cp_ckv = pltpu.make_async_copy(ckv_h.bitcast(U32).at[0], ckv, sem_x.at[2])

            cp_ax[0].start()
            pair_copy(awk_h, awk, sem_ak, 0).start()
            pair_copy(awv_h, awv, sem_av, 0).start()
            for cp in cp_ax[1:]:
                cp.start()
            cp_mem.start()
            for i in range(NP):
                if i > 0:
                    pair_copy(awk_h, awk, sem_ak, i).start()
                    pair_copy(awv_h, awv, sem_av, i).start()
                pair_copy(awq_h, awq, sem_aq, i).start()
                wo_copy(awo_h, awo, sem_ao, i).start()
                if i == 0:
                    cp_bx.start()
            cp_ckv.start()
            for i in range(NP):
                pair_copy(bwq_h, bwq, sem_bq, i).start()
                pair_copy(bwk_h, bwk, sem_bk, i).start()
                pair_copy(bwv_h, bwv, sem_bv, i).start()
                wo_copy(bwo_h, bwo, sem_bo, i).start()

            def keep(w, t):
                u = _u32(w)
                for j in range(HT):
                    wqkv[t + j] = u[:KM // 2, j * 128:(j + 1) * 128]
                    wqkv_t[t // 2 + j // 2, _half((j % 2) * 64, 64), :] = u[KM // 2:, j * 128:(j + 1) * 128]

            def pair(i, first):
                pair_copy(awk_h, awk, sem_ak, i).wait()
                pair_copy(awv_h, awv, sem_av, i).wait()
                ws = []
                for par in range(2):
                    wk, wv = _unpack(awk[i], par), _unpack(awv[i], par)
                    keep(wk, PT * i + (2 + par) * HT)
                    keep(wv, PT * i + (4 + par) * HT)
                    ws.append((wk, wv))
                for r in range(S // RB):
                    if first:
                        cp_ax[r].wait()
                        for c in range(r * RB, (r + 1) * RB, 256):
                            ax[_half(c, 256), :] = transposed(axraw, c)
                    rows = _half(r * RB, RB)
                    x = _bf(ax[rows, :])[:, :DM]
                    for par in range(2):
                        kx[2 * i + par, rows, :] = _u32(_dot(x, ws[par][0]))
                        vx[2 * i + par, rows, :] = _u32(_dot(x, ws[par][1]))
                    if r == 0:
                        pair_copy(awq_h, awq, sem_aq, i).wait()
                        wo_copy(awo_h, awo, sem_ao, i).wait()
                        if first:
                            cp_bx.wait()
                    if r == 1:
                        for par in range(2):
                            keep(_unpack(awq[i], par), PT * i + par * HT)
                            h = 2 * i + par
                            w = _u32(jnp.concatenate([_bf(awo[h]), jnp.zeros((DP - DM, DH), BF16)], axis=0).T)
                            wo[_half(h * DH, DH), :] = w[:, :KM]
                            wo_t[_half(h * 128, 128), :] = w[:64, KM:] | pltpu.roll(w[64:, KM:], 64, 1)
                    if r == 2:
                        c = i * (S // NP)
                        bx[_half(c, S // NP), :] = transposed(bxraw, c)
                        cols = pl.ds(c if first else pl.multiple_of(c, S // NP), S // NP)
                        accb[:, cols] = jnp.zeros((DM, S // NP), F32)

            pair(0, True)

            def pair_body(i, c):
                pair(i, False)
                return c
            jax.lax.fori_loop(1, NP, pair_body, 0)
            cp_mem.wait()
            mem_s[...] = jnp.concatenate([mem0[...].astype(F32), jnp.zeros((M, DP - DM), F32)], axis=1)
            cp_ckv.wait()

        with jax.named_scope('phase1'):
            pl.run_scoped(phase1, packed(DM, S), packed(DM, S), pltpu.VMEM((M, DM), BF16),
                          *[pltpu.VMEM((NP, DM, DH), U32)] * 3)

        def chain_step(s, held):
            mem = mem_s[...]
            zero = s >> 10
            mt = mem[:, KM:]
            mtail = jnp.concatenate([mt, pltpu.roll(mt, 64, 1)], axis=0).astype(BF16)
            t = []
            for g in range(0, NP * PT, 8):
                for t0 in (g, g + 4):
                    acc = _zeros(s, (M, 512))
                    for k0 in range(0, KM, 128):
                        w = jnp.concatenate([wqkv[t0 + j + zero, _half(k0, 128), :] for j in range(4)], axis=1)
                        yield
                        acc = acc + _dot(mem[:, k0:k0 + 128], _bf(w))
                    t += [acc[:, j * 128:(j + 1) * 128] for j in range(4)]
                w = jnp.concatenate([wqkv_t[g // 2 + j + zero] for j in range(4)], axis=1)
                yield
                d = _dot(mtail, _bf(w))
                for j in range(8):
                    t[g + j] = t[g + j] + d[(j % 2) * M:(j % 2 + 1) * M, (j // 2) * 128:(j // 2 + 1) * 128]
            for _ in range(GAPS[0]):
                yield

            def head_rows(i, which, par):
                t0 = PT * i + (2 * which + par) * HT
                return jnp.concatenate(t[t0:t0 + HT], axis=1)

            def pair_rows(i, which):
                return jnp.concatenate([head_rows(i, which, 0), head_rows(i, which, 1)], axis=0)

            def window(ref, i, which):
                xr = _half(s * SEG, SEG)
                return jnp.concatenate([_bf(ref[2 * i, xr, :]), _bf(ref[2 * i + 1, xr, :]),
                                        pair_rows(i, which).astype(BF16)], axis=0)

            now = [[head_rows(h // 2, which, h % 2) for h in range(H)] for which in (1, 2)]
            if held:
                for ref, old, new in zip((km, vm), held.pop(), now):
                    for h in range(H):
                        ref[h, _half((s - 1) * M, 2 * M), :] = _u32(jnp.concatenate([old[h], new[h]], axis=0))
            else:
                held.append(now)
            sc = []
            for i0 in range(0, NP, 2):
                ops = [((pair_rows(i, 0) * QSC).astype(BF16), window(kx, i, 1)) for i in (i0, i0 + 1)]
                yield
                sc += [_dot_nt(q, k) for q, k in ops]
            for _ in range(GAPS[1]):
                yield
            sc = jnp.concatenate(sc, axis=0)
            par = (jax.lax.broadcasted_iota(jnp.int32, sc.shape, 0) // M) % 2
            ci = jax.lax.broadcasted_iota(jnp.int32, sc.shape, 1)
            own = jnp.where(ci < 2 * SEG, ci // SEG, (ci - 2 * SEG) // M) == par
            p = _softmax2(jnp.where(own, sc, NEG))
            zt = []
            for i0 in range(0, NP, 2):
                ops = [(p[2 * M * i:2 * M * (i + 1)], window(vx, i, 2)) for i in (i0, i0 + 1)]
                yield
                for pp, v in ops:
                    o = _dot(pp, v)
                    zt += [o[par * M:(par + 1) * M, j * 128:(j + 1) * 128] for par in range(2) for j in range(HT)]
            for _ in range(GAPS[2]):
                yield
            acc = [_zeros(s, (M, 128))] * 3 + [_zeros(s, (2 * M, 128))]
            for g in range(0, H * HT, 8):
                for t0 in (g, g + 4):
                    zp = jnp.concatenate(zt[t0:t0 + 4], axis=1).astype(BF16).astype(F32)
                    for n in range(KM // 128):
                        w = wo[_half((t0 + zero) * 128, 512), n * 128:(n + 1) * 128]
                        yield
                        acc[n] = acc[n] + _dot(zp, _bf(w))
                zp = jnp.concatenate([jnp.concatenate(zt[g:g + 8:2], axis=1),
                                      jnp.concatenate(zt[g + 1:g + 8:2], axis=1)], axis=0).astype(BF16)
                w = wo_t[_half((g // 2 + zero) * 128, 512), :]
                yield
                acc[3] = acc[3] + _dot(zp, _bf(w))
            lane = jax.lax.broadcasted_iota(jnp.int32, (M, 128), 1)
            last = jnp.where(lane < 64, acc[3][:M] + pltpu.roll(acc[3][M:], 64, 1), 0.0)
            mem_s[...] = jnp.concatenate(acc[:3] + [last], axis=1).astype(BF16).astype(F32)
            for _ in range(GAPS[3]):
                yield

        def chain(h):
            held = []
            for j in range(STEPS):
                yield from chain_step(h * STEPS + j, held)

        n_chain = STEPS * ((NP * PT + H * HT) // 8 * 7 + NP + sum(GAPS))
        n_proj = 2 * (QB // MBQ) + (DC // 256) * (QB // MBK + QB // MBV)
        n_head = (S // QB) * (n_proj + DM // OB // 2) + 2 * sum((r + 2) // 2 for r in range(S // QB))

        def phase2(wq_s, wk_s, wv_s, k_s, v_s):
            def b_head(h):
                i = h // 2
                par = h % 2
                wq_s[...] = _u32(_unpack(bwq[i], par))
                wk_s[...] = _u32(_unpack(bwk[i], par))
                wv_s[...] = _u32(_unpack(bwv[i], par))
                qs, ss, ctxs = {}, {}, {}

                def chunks(r):
                    nk = (r + 1) * QB
                    return [(c0, min(c0 + 256, nk)) for c0 in range(0, nk, 256)]

                def project(r):
                    qp = []
                    for r0 in range(r * QB, (r + 1) * QB, MBQ):
                        rows = _half(r0, MBQ)
                        acc = _zeros(h, (MBQ, DH))
                        for k0, k1 in ((0, 256), (256, DM)):
                            x = _bf(bx[rows, k0:k0 + 256])[:, :k1 - k0]
                            w = _bf(wq_s[_half(k0, k1 - k0), :])
                            yield
                            acc = acc + _dot(x, w)
                        qp.append((acc * QSC).astype(BF16))
                    qs[r] = jnp.concatenate(qp, axis=0)
                    for w_s, dst, mb in ((wk_s, k_s, MBK), (wv_s, v_s, MBV)):
                        for r0 in range(r * QB, (r + 1) * QB, mb):
                            rows = _half(r0, mb)
                            acc = _zeros(h, (mb, DH))
                            for k0 in range(0, DC, 256):
                                x = _bf(ckv[rows, k0:k0 + 256])
                                w = _bf(w_s[_half(k0, 256), :])
                                yield
                                acc = acc + _dot(x, w)
                            dst[rows, :] = _u32(acc)

                def scores(r):
                    ss[r] = []
                    zero = (h + r) >> 10
                    for c0, c1 in chunks(r):
                        k = _bf(k_s[_half(c0 + zero, c1 - c0), :])
                        yield
                        sc = _dot_nt(qs[r], k)
                        if c1 == (r + 1) * QB:
                            ri = jax.lax.broadcasted_iota(jnp.int32, sc.shape, 0) + r * QB
                            ci = jax.lax.broadcasted_iota(jnp.int32, sc.shape, 1) + c0
                            sc = jnp.where(ci <= ri, sc, NEG)
                        ss[r].append(sc)

                def context(r):
                    m = None
                    for sc in ss[r]:
                        for t0 in range(0, sc.shape[1], 128):
                            m = sc[:, t0:t0 + 128] if m is None else jnp.maximum(m, sc[:, t0:t0 + 128])
                    m = jnp.max(m, axis=1, keepdims=True)
                    l = None
                    acc = _zeros(h, (QB, DH))
                    for (c0, c1), sc in zip(chunks(r), ss[r]):
                        p = jnp.exp2(sc - m)
                        for t0 in range(0, p.shape[1], 128):
                            l = p[:, t0:t0 + 128] if l is None else l + p[:, t0:t0 + 128]
                        p = p.astype(BF16)
                        v = _bf(v_s[_half(c0, c1 - c0), :])
                        yield
                        acc = acc + _dot(p, v)
                    ctxs[r] = (acc / jnp.sum(l, axis=1, keepdims=True)).astype(BF16)

                def output(r):
                    ctx = jnp.concatenate([ctxs[r - 1], ctxs[r]], axis=0)
                    cols = pl.ds((r - 1) * QB, 2 * QB)
                    zero = (h + r) >> 10
                    for n0 in range(0, DM, OB):
                        w = _bf(bwo[h + zero, _half(n0, OB), :])
                        yield
                        accb[n0:n0 + OB, cols] += _dot_nt(w, ctx)

                nb = S // QB
                for r in range(nb + 3):
                    parts = []
                    if r < nb:
                        parts.append((project(r), n_proj))
                    if 0 <= r - 3 < nb and (r - 3) % 2 == 1:
                        parts.append((output(r - 3), DM // OB))
                    if 0 <= r - 1 < nb:
                        parts.append((scores(r - 1), len(chunks(r - 1))))
                    if 0 <= r - 2 < nb:
                        parts.append((context(r - 2), len(chunks(r - 2))))
                    yield from _merge(*parts)

            def b_body(h, c):
                i = h // 2

                @pl.when(h % 2 == 0)
                def _():
                    pair_copy(bwq_h, bwq, sem_bq, i).wait()
                    pair_copy(bwk_h, bwk, sem_bk, i).wait()
                    pair_copy(bwv_h, bwv, sem_bv, i).wait()
                    wo_copy(bwo_h, bwo, sem_bo, i).wait()
                for _ in _merge((chain(h), n_chain), (b_head(h), n_head)):
                    pass
                return c
            jax.lax.fori_loop(0, H, b_body, 0)

        with jax.named_scope('phase2'):
            pl.run_scoped(phase2, packed(DM, DH), packed(DC, DH), packed(DC, DH), packed(S, DH), packed(S, DH))

        def phase3(acca, ostage):
            ri = jax.lax.broadcasted_iota(jnp.int32, (AB, AB + 2 * M), 0)
            ci = jax.lax.broadcasted_iota(jnp.int32, (AB, AB + 2 * M), 1)
            amask = (((ci < AB) & ((ci // SEG) == (ri // SEG)) & (ci <= ri))
                     | ((ci >= AB) & (((ci - AB) // M) == (ri // SEG))))

            def out_copy(r):
                rows = _half(r * RB, RB)
                return pltpu.make_async_copy(ostage.at[rows, :], out_h.bitcast(U32).at[0, rows, :], sem_out.at[r])

            def a_head(h, first, last):
                wq = head_weight(PT * (h // 2) + (h % 2) * HT)
                qs, ps, ctxs = {}, {}, {}

                def project(r):
                    qs[r] = (_dot(_bf(ax[_half(r * RB, RB), :])[:, :DM], wq) * QSC).astype(BF16)

                def window(xref, mref, j):
                    return _bf(jnp.concatenate([xref[h, _half(j * AB, AB), :],
                                                mref[h, _half(j * 2 * M, 2 * M), :]], axis=0))

                def scores(r):
                    ps[r] = []
                    for j in range(RB // AB):
                        sc = _dot_nt(qs[r][j * AB:(j + 1) * AB], window(kx, km, r * RB // AB + j))
                        ps[r].append(_softmax2(jnp.where(amask, sc, NEG)))

                def context(r):
                    ctxs[r] = jnp.concatenate(
                        [_dot(p, window(vx, vm, r * RB // AB + j)).astype(BF16) for j, p in enumerate(ps[r])],
                        axis=0)

                def output(r, c0, c1):
                    cols = slice(r * RB + c0, r * RB + c1)
                    o = _dot_nt(_bf(awo[h]), ctxs[r][c0:c1])
                    if not first:
                        o = acca[:, cols] + o
                    if not last:
                        acca[:, cols] = o
                        return
                    ostage[_half(r * RB + c0, c1 - c0), :] = _u32(
                        jnp.concatenate([o, accb[:, cols]], axis=0).astype(BF16).T)
                    if c1 == RB:
                        out_copy(r).start()

                nr = S // RB
                project(0)
                project(1)
                for r in range(nr):
                    scores(r)
                    if r > 0:
                        output(r - 1, 0, RB if r + 1 < nr else RB // 2)
                    if r + 2 < nr:
                        project(r + 2)
                    context(r)
                output(nr - 2, RB // 2, RB)
                output(nr - 1, 0, RB // 2)
                output(nr - 1, RB // 2, RB)

            a_head(0, True, False)

            def a_body(h, c):
                a_head(h, False, False)
                return c
            jax.lax.fori_loop(1, H - 1, a_body, 0)
            a_head(H - 1, False, True)
            for r in range(S // RB):
                out_copy(r).wait()

        with jax.named_scope('phase3'):
            pl.run_scoped(phase3, pltpu.VMEM((DM, S), F32), packed(S, 2 * DM))

    scratch = [
        packed(S, DP),
        pltpu.VMEM((M, DP), F32),
        packed(H, DM, DH),
        packed(NP * PT, KM, 128),
        packed(NP * PT // 2, 128, 128),
        packed(H * DH, KM),
        packed(H * DH // 2, 128),
        packed(H, S, DH),
        packed(H, S, DH),
        packed(H, NSEG * M, DH),
        packed(H, NSEG * M, DH),
        packed(S, DP),
        packed(S, DC),
        pltpu.VMEM((NP, DM, DH), U32),
        pltpu.VMEM((NP, DC, DH), U32),
        pltpu.VMEM((NP, DC, DH), U32),
        packed(H, DM, DH),
        pltpu.VMEM((DM, S), F32),
        pltpu.SemaphoreType.DMA((3 + S // RB,)),
    ] + [pltpu.SemaphoreType.DMA((NP,)) for _ in range(8)] + [pltpu.SemaphoreType.DMA((S // RB,))]
    return kernel, scratch


@jax.jit
def pallas_concat_heads__memory_aug_recurrent_mem_tr__compressed_kv_cla__prompt_kernel(
    A_x, A_mem0, A_Wq, A_Wk, A_Wv, A_Wo, A_seg_len, B_x, B_c_kv, B_w_q, B_w_uk, B_w_uv, B_w_o,
):
    del A_seg_len
    _, S, DM = A_x.shape
    M = A_mem0.shape[1]
    H, DH = A_Wq.shape[1], A_Wq.shape[2]
    DC = B_c_kv.shape[2]
    kernel, scratch = _make_kernel(S, DM, H, DH, M, 32, DC)
    return pl.pallas_call(
        kernel,
        out_shape=jax.ShapeDtypeStruct((1, S, 2 * DM), BF16),
        in_specs=[pl.BlockSpec(memory_space=pl.ANY)] * 12,
        out_specs=pl.BlockSpec(memory_space=pl.ANY),
        scratch_shapes=scratch,
        compiler_params=pltpu.CompilerParams(vmem_limit_bytes=126 * 1024 * 1024),
    )(A_x[0].T, A_mem0, A_Wq, A_Wk, A_Wv, A_Wo.transpose(0, 2, 1),
      B_x[0].T, B_c_kv, B_w_q, B_w_uk, B_w_uv, B_w_o.transpose(0, 2, 1))
```

```python
import jax
import jax.numpy as jnp
import jax.experimental.pallas as pl
import jax.experimental.pallas.tpu as pltpu

F32 = jnp.float32
BF16 = jnp.bfloat16
U32 = jnp.uint32
LOG2E = 1.4426950408889634
NEG = -1e30
NN = (((1,), (0,)), ((), ()))
NT = (((1,), (1,)), ((), ()))


def _dot(a, b):
    return jax.lax.dot_general(a, b, NN, preferred_element_type=F32)


def _dot_nt(a, b):
    return jax.lax.dot_general(a, b, NT, preferred_element_type=F32)


def _bf(u):
    return pltpu.bitcast(u, BF16)


def _u32(x):
    return pltpu.bitcast(x.astype(BF16), U32)


def _half(start, size):
    if isinstance(start, int):
        return pl.ds(start // 2, size // 2)
    return pl.ds(pl.multiple_of(start // 2, 8), size // 2)


def _unpack(u, parity):
    if isinstance(parity, int):
        w = (u << 16) if parity == 0 else (u & jnp.uint32(0xFFFF0000))
    else:
        w = (u >> (16 * parity).astype(U32)) << 16
    return pltpu.bitcast(w, F32).astype(BF16)


def _zeros(i, shape):
    return jnp.full(shape, (i >> 10).astype(F32))


def _softmax2(sc):
    p = jnp.exp2(sc - jnp.max(sc, axis=1, keepdims=True))
    return (p / jnp.sum(p, axis=1, keepdims=True)).astype(BF16)


def _order(counts):
    done = [0] * len(counts)
    live = [a for a, n in enumerate(counts) if n > 0]
    order = []
    for _ in range(sum(counts)):
        j = min(live, key=lambda a: ((done[a] + 0.5) / counts[a], a))
        done[j] += 1
        order.append(j)
    return order


def _finish(gens):
    for g in gens:
        for _ in g:
            raise AssertionError("stream longer than announced")


def _merge(*streams):
    for j in _order([n for _, n in streams]):
        for _ in range(2):
            next(streams[j][0])
            yield
    _finish([g for g, _ in streams])


def _make_kernel(S, DM, H, DH, M, SEG, DC):
    NP = H // 2
    NSEG = S // SEG
    DP = 512
    KM = DM // 128 * 128
    HT = DH // 128
    PT = 6 * HT
    STEPS = NSEG // H
    QB = 128
    OB = DM // 4
    PVR = 12
    XK, XC = 0, 0
    MBQ, MBK, MBV = 64, 64, 64
    GAPS = (2, 3, 2, 2)
    RB = 512
    AB = 2 * SEG
    QSC = LOG2E * DH ** -0.5

    def packed(*shape):
        return pltpu.VMEM(shape[:-2] + (shape[-2] // 2, shape[-1]), U32)

    def kernel(ax_h, mem_h, awq_h, awk_h, awv_h, awo_h, bx_h, ckv_h, bwq_h, bwk_h, bwv_h, bwo_h,
               out_h,
               ax, mem_s, awo, wqkv, wqkv_t, wo, wo_t, kx, vx, km, vm,
               bx, ckv, bwq, bwk, bwv, bwo, accb,
               sem_x, sem_aq, sem_ak, sem_av, sem_ao, sem_bq, sem_bk, sem_bv, sem_bo, sem_out):

        def pair_copy(src, dst, sem, i):
            return pltpu.make_async_copy(src.bitcast(U32).at[:, i, :], dst.at[i], sem.at[i])

        def wo_copy(src, dst, sem, i):
            return pltpu.make_async_copy(src.bitcast(U32).at[pl.ds(2 * i, 2)], dst.at[pl.ds(2 * i, 2)], sem.at[i])

        def head_weight(t):
            return _bf(jnp.concatenate(
                [jnp.concatenate([wqkv[t + j], wqkv_t[t // 2 + j // 2, _half((j % 2) * 64, 64), :]], axis=0)
                 for j in range(HT)], axis=1))

        def transposed(raw, c):
            xt = _bf(raw[:, pl.ds(c if isinstance(c, int) else pl.multiple_of(c, 256), 256)])
            return _u32(jnp.concatenate([xt, jnp.zeros((DP - DM, 256), BF16)], axis=0).T)

        def phase1(axraw, bxraw, mem0, awq, awk, awv):
            cp_ax = [pltpu.make_async_copy(ax_h.bitcast(U32).at[:, pl.ds(r * RB, RB)],
                                           axraw.at[:, pl.ds(r * RB, RB)], sem_x.at[3 + r]) for r in range(S // RB)]
            cp_mem = pltpu.make_async_copy(mem_h.at[0], mem0, sem_x.at[0])
            cp_bx = pltpu.make_async_copy(bx_h.bitcast(U32), bxraw, sem_x.at[1])
            cp_ckv = pltpu.make_async_copy(ckv_h.bitcast(U32).at[0], ckv, sem_x.at[2])

            cp_ax[0].start()
            pair_copy(awk_h, awk, sem_ak, 0).start()
            pair_copy(awv_h, awv, sem_av, 0).start()

            def start_more(stage):
                if stage == 0:
                    for cp in cp_ax[1:]:
                        cp.start()
                    pair_copy(awq_h, awq, sem_aq, 0).start()
                    wo_copy(awo_h, awo, sem_ao, 0).start()
                elif stage == 1:
                    cp_bx.start()
                elif stage == 2:
                    cp_mem.start()
                    for i in range(1, NP):
                        pair_copy(awk_h, awk, sem_ak, i).start()
                        pair_copy(awv_h, awv, sem_av, i).start()
                        pair_copy(awq_h, awq, sem_aq, i).start()
                        wo_copy(awo_h, awo, sem_ao, i).start()
                else:
                    cp_ckv.start()
                    for i in range(NP):
                        pair_copy(bwq_h, bwq, sem_bq, i).start()
                        pair_copy(bwk_h, bwk, sem_bk, i).start()
                        pair_copy(bwv_h, bwv, sem_bv, i).start()
                        wo_copy(bwo_h, bwo, sem_bo, i).start()

            def keep(w, t):
                u = _u32(w)
                for j in range(HT):
                    wqkv[t + j] = u[:KM // 2, j * 128:(j + 1) * 128]
                    wqkv_t[t // 2 + j // 2, _half((j % 2) * 64, 64), :] = u[KM // 2:, j * 128:(j + 1) * 128]

            def pair(i, first):
                pair_copy(awk_h, awk, sem_ak, i).wait()
                pair_copy(awv_h, awv, sem_av, i).wait()
                ws = []
                for par in range(2):
                    wk, wv = _unpack(awk[i], par), _unpack(awv[i], par)
                    keep(wk, PT * i + (2 + par) * HT)
                    keep(wv, PT * i + (4 + par) * HT)
                    ws.append((wk, wv))
                for r in range(S // RB):
                    if first:
                        cp_ax[r].wait()
                        if r < 3:
                            start_more(r)
                        for c in range(r * RB, (r + 1) * RB, 256):
                            ax[_half(c, 256), :] = transposed(axraw, c)
                    rows = _half(r * RB, RB)
                    x = _bf(ax[rows, :])[:, :DM]
                    for par in range(2):
                        kx[2 * i + par, rows, :] = _u32(_dot(x, ws[par][0]))
                        vx[2 * i + par, rows, :] = _u32(_dot(x, ws[par][1]))
                    if r == 1:
                        pair_copy(awq_h, awq, sem_aq, i).wait()
                        wo_copy(awo_h, awo, sem_ao, i).wait()
                        for par in range(2):
                            keep(_unpack(awq[i], par), PT * i + par * HT)
                            h = 2 * i + par
                            w = _u32(jnp.concatenate([_bf(awo[h]), jnp.zeros((DP - DM, DH), BF16)], axis=0).T)
                            wo[_half(h * DH, DH), :] = w[:, :KM]
                            wo_t[_half(h * 128, 128), :] = w[:64, KM:] | pltpu.roll(w[64:, KM:], 64, 1)
                    if r == 3:
                        if first:
                            cp_bx.wait()
                        c = i * (S // NP)
                        bx[_half(c, S // NP), :] = transposed(bxraw, c)
                        cols = pl.ds(c if first else pl.multiple_of(c, S // NP), S // NP)
                        accb[:, cols] = jnp.zeros((DM, S // NP), F32)

            pair(0, True)
            start_more(3)

            def pair_body(i, c):
                pair(i, False)
                return c
            jax.lax.fori_loop(1, NP, pair_body, 0)
            cp_mem.wait()
            mem_s[...] = jnp.concatenate([mem0[...].astype(F32), jnp.zeros((M, DP - DM), F32)], axis=1)
            cp_ckv.wait()

        with jax.named_scope('phase1'):
            pl.run_scoped(phase1, packed(DM, S), packed(DM, S), pltpu.VMEM((M, DM), BF16),
                          *[pltpu.VMEM((NP, DM, DH), U32)] * 3)

        def chain_step(s, held):
            mem = mem_s[...]
            zero = s >> 10
            mt = mem[:, KM:]
            mtail = jnp.concatenate([mt, pltpu.roll(mt, 64, 1)], axis=0).astype(BF16)
            t = []
            for g in range(0, NP * PT, 8):
                for t0 in (g, g + 4):
                    acc = _zeros(s, (M, 512))
                    for k0 in range(0, KM, 128):
                        w = jnp.concatenate([wqkv[t0 + j + zero, _half(k0, 128), :] for j in range(4)], axis=1)
                        yield
                        acc = acc + _dot(mem[:, k0:k0 + 128], _bf(w))
                        yield
                    t += [acc[:, j * 128:(j + 1) * 128] for j in range(4)]
                w = jnp.concatenate([wqkv_t[g // 2 + j + zero] for j in range(4)], axis=1)
                yield
                d = _dot(mtail, _bf(w))
                for j in range(8):
                    t[g + j] = t[g + j] + d[(j % 2) * M:(j % 2 + 1) * M, (j // 2) * 128:(j // 2 + 1) * 128]
                yield
            for _ in range(2 * GAPS[0]):
                yield

            def head_rows(i, which, par):
                t0 = PT * i + (2 * which + par) * HT
                return jnp.concatenate(t[t0:t0 + HT], axis=1)

            def pair_rows(i, which):
                return jnp.concatenate([head_rows(i, which, 0), head_rows(i, which, 1)], axis=0)

            def window(ref, i, which):
                xr = _half(s * SEG, SEG)
                return jnp.concatenate([_bf(ref[2 * i, xr, :]), _bf(ref[2 * i + 1, xr, :]),
                                        pair_rows(i, which).astype(BF16)], axis=0)

            now = [[head_rows(h // 2, which, h % 2) for h in range(H)] for which in (1, 2)]
            if held:
                for ref, old, new in zip((km, vm), held.pop(), now):
                    for h in range(H):
                        ref[h, _half((s - 1) * M, 2 * M), :] = _u32(jnp.concatenate([old[h], new[h]], axis=0))
            else:
                held.append(now)
            sc = []
            for i0 in range(0, NP, 2):
                ops = [((pair_rows(i, 0) * QSC).astype(BF16), window(kx, i, 1)) for i in (i0, i0 + 1)]
                yield
                sc += [_dot_nt(q, k) for q, k in ops]
                yield
            for _ in range(2 * GAPS[1]):
                yield
            sc = jnp.concatenate(sc, axis=0)
            par = (jax.lax.broadcasted_iota(jnp.int32, sc.shape, 0) // M) % 2
            ci = jax.lax.broadcasted_iota(jnp.int32, sc.shape, 1)
            own = jnp.where(ci < 2 * SEG, ci // SEG, (ci - 2 * SEG) // M) == par
            p = _softmax2(jnp.where(own, sc, NEG))
            zt = []
            for i0 in range(0, NP, 2):
                ops = [(p[2 * M * i:2 * M * (i + 1)], window(vx, i, 2)) for i in (i0, i0 + 1)]
                yield
                for pp, v in ops:
                    o = _dot(pp, v)
                    zt += [o[par * M:(par + 1) * M, j * 128:(j + 1) * 128] for par in range(2) for j in range(HT)]
                yield
            for _ in range(2 * GAPS[2]):
                yield
            acc = [_zeros(s, (M, 128))] * 3 + [_zeros(s, (2 * M, 128))]
            for g in range(0, H * HT, 8):
                for t0 in (g, g + 4):
                    zp = jnp.concatenate(zt[t0:t0 + 4], axis=1).astype(BF16).astype(F32)
                    for n in range(KM // 128):
                        w = wo[_half((t0 + zero) * 128, 512), n * 128:(n + 1) * 128]
                        yield
                        acc[n] = acc[n] + _dot(zp, _bf(w))
                        yield
                zp = jnp.concatenate([jnp.concatenate(zt[g:g + 8:2], axis=1),
                                      jnp.concatenate(zt[g + 1:g + 8:2], axis=1)], axis=0).astype(BF16)
                w = wo_t[_half((g // 2 + zero) * 128, 512), :]
                yield
                acc[3] = acc[3] + _dot(zp, _bf(w))
                yield
            lane = jax.lax.broadcasted_iota(jnp.int32, (M, 128), 1)
            last = jnp.where(lane < 64, acc[3][:M] + pltpu.roll(acc[3][M:], 64, 1), 0.0)
            mem_s[...] = jnp.concatenate(acc[:3] + [last], axis=1).astype(BF16).astype(F32)
            for _ in range(2 * GAPS[3]):
                yield

        def chain(h):
            held = []
            for j in range(STEPS):
                yield from chain_step(h * STEPS + j, held)

        n_chain = STEPS * ((NP * PT + H * HT) // 8 * 7 + NP + sum(GAPS))
        n_proj = 2 * (QB // MBQ) + (DC // 256) * (QB // MBK + QB // MBV)

        def split(r):
            return 2 if r >= PVR else 1

        def n_scores(r):
            return (r + 2) // 2

        def n_context(r):
            return (r + 1) // 2 * split(r) + (r + 1) % 2

        n_head = ((S // QB) * n_proj + (S // QB // 2) * (DM // OB) - (S // QB // 2 - 1)
                  + sum(n_scores(r) + n_context(r) for r in range(S // QB)))

        def phase2(wq_s, wk_s, wv_s, k_s, v_s):
            def b_head(h):
                i = h // 2
                par = h % 2
                wq_s[...] = _u32(_unpack(bwq[i], par))
                wk_s[...] = _u32(_unpack(bwk[i], par))
                wv_s[...] = _u32(_unpack(bwv[i], par))
                qs, ss, ctxs = {}, {}, {}

                def chunks(r):
                    nk = (r + 1) * QB
                    return [(c0, min(c0 + 256, nk)) for c0 in range(0, nk, 256)]

                def project(r):
                    qp = []
                    for r0 in range(r * QB, (r + 1) * QB, MBQ):
                        rows = _half(r0, MBQ)
                        acc = _zeros(h, (MBQ, DH))
                        for k0, k1 in ((0, 256), (256, DM)):
                            x = _bf(bx[rows, k0:k0 + 256])[:, :k1 - k0]
                            w = _bf(wq_s[_half(k0, k1 - k0), :])
                            yield
                            acc = acc + _dot(x, w)
                            if k1 == DM:
                                qp.append((acc * QSC).astype(BF16))
                                qs[r] = jnp.concatenate(qp, axis=0)
                            yield
                    for w_s, mb in ((wk_s, MBK), (wv_s, MBV)):
                        got = []
                        for r0 in range(r * QB, (r + 1) * QB, mb):
                            rows = _half(r0, mb)
                            acc = _zeros(h, (mb, DH))
                            for k0 in range(0, DC, 256):
                                x = _bf(ckv[rows, k0:k0 + 256])
                                w = _bf(w_s[_half(k0, 256), :])
                                yield
                                acc = acc + _dot(x, w)
                                if k0 + 256 == DC:
                                    got.append(acc.astype(BF16))
                                    if len(got) * mb == QB:
                                        blk = jnp.concatenate(got, axis=0)
                                        if w_s is wk_s and XK:
                                            k_s[:, r * QB:(r + 1) * QB] = _u32(blk.T)
                                        else:
                                            (k_s if w_s is wk_s else v_s)[_half(r * QB, QB), :] = _u32(blk)
                                yield

                def scores(r):
                    ss[r] = []
                    zero = (h + r) >> 10
                    for c0, c1 in chunks(r):
                        if XK:
                            k = _bf(k_s[_half(zero, DH), c0:c1])
                            yield
                            sc = _dot(qs[r], k)
                        else:
                            k = _bf(k_s[_half(c0 + zero, c1 - c0), :])
                            yield
                            sc = _dot_nt(qs[r], k)
                        if c1 == (r + 1) * QB:
                            ri = jax.lax.broadcasted_iota(jnp.int32, sc.shape, 0) + r * QB
                            ci = jax.lax.broadcasted_iota(jnp.int32, sc.shape, 1) + c0
                            sc = jnp.where(ci <= ri, sc, NEG)
                        ss[r].append(sc)
                        yield

                def context(r):
                    m = None
                    for sc in ss[r]:
                        for t0 in range(0, sc.shape[1], 128):
                            m = sc[:, t0:t0 + 128] if m is None else jnp.maximum(m, sc[:, t0:t0 + 128])
                    m = jnp.max(m, axis=1, keepdims=True)
                    l = None
                    acc = _zeros(h, (QB, DH))
                    for (c0, c1), sc in zip(chunks(r), ss[r]):
                        mb = QB // split(r) if c1 - c0 == 256 else QB
                        p = jnp.exp2(sc - m)
                        for t0 in range(0, p.shape[1], 128):
                            l = p[:, t0:t0 + 128] if l is None else l + p[:, t0:t0 + 128]
                        p = p.astype(BF16)
                        v = _bf(v_s[_half(c0, c1 - c0), :])
                        new = []
                        for r0 in range(0, QB, mb):
                            yield
                            new.append(acc[r0:r0 + mb] + _dot(p[r0:r0 + mb], v))
                            if r0 + mb == QB:
                                acc = jnp.concatenate(new, axis=0)
                                if c1 == (r + 1) * QB:
                                    ctxs[r] = (acc / jnp.sum(l, axis=1, keepdims=True)).astype(BF16)
                            yield

                def output(r):
                    ctx = jnp.concatenate([ctxs[r - 1], ctxs[r]], axis=0)
                    cols = pl.ds((r - 1) * QB, 2 * QB)
                    zero = (h + r) >> 10
                    if XC:
                        ctx = ctx.T
                    for n0 in range(0, DM, OB):
                        w = _bf(bwo[h + zero, _half(n0, OB), :])
                        yield
                        accb[n0:n0 + OB, cols] += (_dot if XC else _dot_nt)(w, ctx)
                        yield

                def both(r):
                    a, b = scores(r), context(r - 2)
                    na, nc = n_scores(r) - 1, n_context(r - 2) - 1
                    for j in _order([na, nc]):
                        for _ in range(2):
                            next((a, b)[j])
                            yield
                    for _ in range(2):
                        next(a)
                        next(b)
                        yield
                    _finish([a, b])

                nb = S // QB
                for r in range(nb + 4):
                    parts = []
                    if r < nb:
                        parts.append((project(r), n_proj))
                    if 0 <= r - 4 < nb and (r - 4) % 2 == 1:
                        parts.append((output(r - 4), DM // OB))
                    if r % 2 == 1 and 3 <= r <= nb:
                        parts.append((both(r - 1), n_scores(r - 1) + n_context(r - 3) - 1))
                    else:
                        if 0 <= r - 1 < nb:
                            parts.append((scores(r - 1), n_scores(r - 1)))
                        if 0 <= r - 3 < nb:
                            parts.append((context(r - 3), n_context(r - 3)))
                    yield from _merge(*parts)

            def b_body(h, c):
                i = h // 2

                @pl.when(h % 2 == 0)
                def _():
                    pair_copy(bwq_h, bwq, sem_bq, i).wait()
                    pair_copy(bwk_h, bwk, sem_bk, i).wait()
                    pair_copy(bwv_h, bwv, sem_bv, i).wait()
                    wo_copy(bwo_h, bwo, sem_bo, i).wait()
                for _ in _merge((chain(h), n_chain), (b_head(h), n_head)):
                    pass
                return c
            jax.lax.fori_loop(0, H, b_body, 0)

        with jax.named_scope('phase2'):
            pl.run_scoped(phase2, packed(DM, DH), packed(DC, DH), packed(DC, DH), packed(DH, S) if XK else packed(S, DH), packed(S, DH))

        def phase3(acca, ostage):
            ri = jax.lax.broadcasted_iota(jnp.int32, (AB, AB + 2 * M), 0)
            ci = jax.lax.broadcasted_iota(jnp.int32, (AB, AB + 2 * M), 1)
            amask = (((ci < AB) & ((ci // SEG) == (ri // SEG)) & (ci <= ri))
                     | ((ci >= AB) & (((ci - AB) // M) == (ri // SEG))))

            def out_copy(r):
                rows = _half(r * RB, RB)
                return pltpu.make_async_copy(ostage.at[rows, :], out_h.bitcast(U32).at[0, rows, :], sem_out.at[r])

            def a_head(h, first, last):
                wq = head_weight(PT * (h // 2) + (h % 2) * HT)
                qs, ps, ctxs = {}, {}, {}

                def project(r):
                    qs[r] = (_dot(_bf(ax[_half(r * RB, RB), :])[:, :DM], wq) * QSC).astype(BF16)

                def window(xref, mref, j):
                    return _bf(jnp.concatenate([xref[h, _half(j * AB, AB), :],
                                                mref[h, _half(j * 2 * M, 2 * M), :]], axis=0))

                def scores(r):
                    ps[r] = []
                    for j in range(RB // AB):
                        sc = _dot_nt(qs[r][j * AB:(j + 1) * AB], window(kx, km, r * RB // AB + j))
                        ps[r].append(_softmax2(jnp.where(amask, sc, NEG)))

                def context(r):
                    ctxs[r] = jnp.concatenate(
                        [_dot(p, window(vx, vm, r * RB // AB + j)).astype(BF16) for j, p in enumerate(ps[r])],
                        axis=0)

                def output(r, c0, c1):
                    cols = slice(r * RB + c0, r * RB + c1)
                    o = _dot_nt(_bf(awo[h]), ctxs[r][c0:c1])
                    if not first:
                        o = acca[:, cols] + o
                    if not last:
                        acca[:, cols] = o
                        return
                    ostage[_half(r * RB + c0, c1 - c0), :] = _u32(
                        jnp.concatenate([o, accb[:, cols]], axis=0).astype(BF16).T)
                    if c1 == RB:
                        out_copy(r).start()

                nr = S // RB
                project(0)
                project(1)
                for r in range(nr):
                    scores(r)
                    if r > 0:
                        output(r - 1, 0, RB if r + 1 < nr else RB // 2)
                    if r + 2 < nr:
                        project(r + 2)
                    context(r)
                output(nr - 2, RB // 2, RB)
                output(nr - 1, 0, RB // 2)
                output(nr - 1, RB // 2, RB)

            a_head(0, True, False)

            def a_body(h, c):
                a_head(h, False, False)
                return c
            jax.lax.fori_loop(1, H - 1, a_body, 0)
            a_head(H - 1, False, True)
            for r in range(S // RB):
                out_copy(r).wait()

        with jax.named_scope('phase3'):
            pl.run_scoped(phase3, pltpu.VMEM((DM, S), F32), packed(S, 2 * DM))

    scratch = [
        packed(S, DP),
        pltpu.VMEM((M, DP), F32),
        packed(H, DM, DH),
        packed(NP * PT, KM, 128),
        packed(NP * PT // 2, 128, 128),
        packed(H * DH, KM),
        packed(H * DH // 2, 128),
        packed(H, S, DH),
        packed(H, S, DH),
        packed(H, NSEG * M, DH),
        packed(H, NSEG * M, DH),
        packed(S, DP),
        packed(S, DC),
        pltpu.VMEM((NP, DM, DH), U32),
        pltpu.VMEM((NP, DC, DH), U32),
        pltpu.VMEM((NP, DC, DH), U32),
        packed(H, DM, DH),
        pltpu.VMEM((DM, S), F32),
        pltpu.SemaphoreType.DMA((3 + S // RB,)),
    ] + [pltpu.SemaphoreType.DMA((NP,)) for _ in range(8)] + [pltpu.SemaphoreType.DMA((S // RB,))]
    return kernel, scratch


@jax.jit
def pallas_concat_heads__memory_aug_recurrent_mem_tr__compressed_kv_cla__prompt_kernel(
    A_x, A_mem0, A_Wq, A_Wk, A_Wv, A_Wo, A_seg_len, B_x, B_c_kv, B_w_q, B_w_uk, B_w_uv, B_w_o,
):
    del A_seg_len
    _, S, DM = A_x.shape
    M = A_mem0.shape[1]
    H, DH = A_Wq.shape[1], A_Wq.shape[2]
    DC = B_c_kv.shape[2]
    kernel, scratch = _make_kernel(S, DM, H, DH, M, 32, DC)
    return pl.pallas_call(
        kernel,
        out_shape=jax.ShapeDtypeStruct((1, S, 2 * DM), BF16),
        in_specs=[pl.BlockSpec(memory_space=pl.ANY)] * 12,
        out_specs=pl.BlockSpec(memory_space=pl.ANY),
        scratch_shapes=scratch,
        compiler_params=pltpu.CompilerParams(vmem_limit_bytes=126 * 1024 * 1024),
    )(A_x[0].T, A_mem0, A_Wq, A_Wk, A_Wv, A_Wo.transpose(0, 2, 1),
      B_x[0].T, B_c_kv, B_w_q, B_w_uk, B_w_uv, B_w_o.transpose(0, 2, 1))
```

```python
import jax
import jax.numpy as jnp
import jax.experimental.pallas as pl
import jax.experimental.pallas.tpu as pltpu

F32 = jnp.float32
BF16 = jnp.bfloat16
U32 = jnp.uint32
LOG2E = 1.4426950408889634
NEG = -1e30
NN = (((1,), (0,)), ((), ()))
NT = (((1,), (1,)), ((), ()))


def _dot(a, b):
    return jax.lax.dot_general(a, b, NN, preferred_element_type=F32)


def _dot_nt(a, b):
    return jax.lax.dot_general(a, b, NT, preferred_element_type=F32)


def _bf(u):
    return pltpu.bitcast(u, BF16)


def _u32(x):
    return pltpu.bitcast(x.astype(BF16), U32)


def _half(start, size):
    if isinstance(start, int):
        return pl.ds(start // 2, size // 2)
    return pl.ds(pl.multiple_of(start // 2, 8), size // 2)


def _unpack(u, parity):
    if isinstance(parity, int):
        w = (u << 16) if parity == 0 else (u & jnp.uint32(0xFFFF0000))
    else:
        w = (u >> (16 * parity).astype(U32)) << 16
    return pltpu.bitcast(w, F32).astype(BF16)


def _zeros(i, shape):
    return jnp.full(shape, (i >> 10).astype(F32))


def _softmax2(sc):
    p = jnp.exp2(sc - jnp.max(sc, axis=1, keepdims=True))
    return (p / jnp.sum(p, axis=1, keepdims=True)).astype(BF16)


def _order(counts):
    done = [0] * len(counts)
    live = [a for a, n in enumerate(counts) if n > 0]
    order = []
    for _ in range(sum(counts)):
        j = min(live, key=lambda a: ((done[a] + 0.5) / counts[a], a))
        done[j] += 1
        order.append(j)
    return order


def _finish(gens):
    for g in gens:
        for _ in g:
            raise AssertionError("stream longer than announced")


def _merge(*streams):
    for j in _order([n for _, n in streams]):
        for _ in range(2):
            next(streams[j][0])
            yield
    _finish([g for g, _ in streams])


def _make_kernel(S, DM, H, DH, M, SEG, DC):
    NP = H // 2
    NSEG = S // SEG
    DP = 512
    KM = DM // 128 * 128
    HT = DH // 128
    PT = 6 * HT
    STEPS = NSEG // H
    QB = 128
    OB = DM // 4
    PVR = 8
    MBQ, MBK, MBV = 64, 64, 64
    GAPS = (2, 3, 2, 2)
    RB = 512
    AB = 2 * SEG
    QSC = LOG2E * DH ** -0.5

    def packed(*shape):
        return pltpu.VMEM(shape[:-2] + (shape[-2] // 2, shape[-1]), U32)

    def kernel(ax_h, mem_h, awq_h, awk_h, awv_h, awo_h, bx_h, ckv_h, bwq_h, bwk_h, bwv_h, bwo_h,
               out_h,
               ax, mem_s, awo, wqkv, wqkv_t, wo, wo_t, kx, vx, km, vm,
               bx, ckv, bwq, bwk, bwv, bwo, accb,
               sem_x, sem_aq, sem_ak, sem_av, sem_ao, sem_bq, sem_bk, sem_bv, sem_bo, sem_out):

        def pair_copy(src, dst, sem, i):
            return pltpu.make_async_copy(src.bitcast(U32).at[:, i, :], dst.at[i], sem.at[i])

        def wo_copy(src, dst, sem, i):
            return pltpu.make_async_copy(src.bitcast(U32).at[pl.ds(2 * i, 2)], dst.at[pl.ds(2 * i, 2)], sem.at[i])

        def head_weight(t):
            return _bf(jnp.concatenate(
                [jnp.concatenate([wqkv[t + j], wqkv_t[t // 2 + j // 2, _half((j % 2) * 64, 64), :]], axis=0)
                 for j in range(HT)], axis=1))

        def transposed(raw, c):
            xt = _bf(raw[:, pl.ds(c if isinstance(c, int) else pl.multiple_of(c, 256), 256)])
            return _u32(jnp.concatenate([xt, jnp.zeros((DP - DM, 256), BF16)], axis=0).T)

        def phase1(axraw, bxraw, mem0, awq, awk, awv):
            cp_ax = [pltpu.make_async_copy(ax_h.bitcast(U32).at[:, pl.ds(r * RB, RB)],
                                           axraw.at[:, pl.ds(r * RB, RB)], sem_x.at[3 + r]) for r in range(S // RB)]
            cp_mem = pltpu.make_async_copy(mem_h.at[0], mem0, sem_x.at[0])
            cp_bx = pltpu.make_async_copy(bx_h.bitcast(U32), bxraw, sem_x.at[1])
            cp_ckv = pltpu.make_async_copy(ckv_h.bitcast(U32).at[0], ckv, sem_x.at[2])

            cp_ax[0].start()
            pair_copy(awk_h, awk, sem_ak, 0).start()
            pair_copy(awv_h, awv, sem_av, 0).start()

            def start_more(stage):
                if stage == 0:
                    for cp in cp_ax[1:]:
                        cp.start()
                    pair_copy(awq_h, awq, sem_aq, 0).start()
                    wo_copy(awo_h, awo, sem_ao, 0).start()
                elif stage == 1:
                    cp_bx.start()
                elif stage == 2:
                    cp_mem.start()
                    for i in range(1, NP):
                        pair_copy(awk_h, awk, sem_ak, i).start()
                        pair_copy(awv_h, awv, sem_av, i).start()
                        pair_copy(awq_h, awq, sem_aq, i).start()
                        wo_copy(awo_h, awo, sem_ao, i).start()
                else:
                    cp_ckv.start()
                    for i in range(NP):
                        pair_copy(bwq_h, bwq, sem_bq, i).start()
                        pair_copy(bwk_h, bwk, sem_bk, i).start()
                        pair_copy(bwv_h, bwv, sem_bv, i).start()
                        wo_copy(bwo_h, bwo, sem_bo, i).start()

            def keep(w, t):
                u = _u32(w)
                for j in range(HT):
                    wqkv[t + j] = u[:KM // 2, j * 128:(j + 1) * 128]
                    wqkv_t[t // 2 + j // 2, _half((j % 2) * 64, 64), :] = u[KM // 2:, j * 128:(j + 1) * 128]

            def pair(i, first):
                pair_copy(awk_h, awk, sem_ak, i).wait()
                pair_copy(awv_h, awv, sem_av, i).wait()
                ws = []
                for par in range(2):
                    wk, wv = _unpack(awk[i], par), _unpack(awv[i], par)
                    keep(wk, PT * i + (2 + par) * HT)
                    keep(wv, PT * i + (4 + par) * HT)
                    ws.append((wk, wv))
                for r in range(S // RB):
                    if first:
                        cp_ax[r].wait()
                        if r < 3:
                            start_more(r)
                        for c in range(r * RB, (r + 1) * RB, 256):
                            ax[_half(c, 256), :] = transposed(axraw, c)
                    rows = _half(r * RB, RB)
                    x = _bf(ax[rows, :])[:, :DM]
                    for par in range(2):
                        kx[2 * i + par, rows, :] = _u32(_dot(x, ws[par][0]))
                        vx[2 * i + par, rows, :] = _u32(_dot(x, ws[par][1]))
                    if r == 1:
                        pair_copy(awq_h, awq, sem_aq, i).wait()
                        wo_copy(awo_h, awo, sem_ao, i).wait()
                        for par in range(2):
                            keep(_unpack(awq[i], par), PT * i + par * HT)
                            h = 2 * i + par
                            w = _u32(jnp.concatenate([_bf(awo[h]), jnp.zeros((DP - DM, DH), BF16)], axis=0).T)
                            wo[_half(h * DH, DH), :] = w[:, :KM]
                            wo_t[_half(h * 128, 128), :] = w[:64, KM:] | pltpu.roll(w[64:, KM:], 64, 1)
                    if r == 3:
                        if first:
                            cp_bx.wait()
                        c = i * (S // NP)
                        bx[_half(c, S // NP), :] = transposed(bxraw, c)
                        cols = pl.ds(c if first else pl.multiple_of(c, S // NP), S // NP)
                        accb[:, cols] = jnp.zeros((DM, S // NP), F32)

            pair(0, True)
            start_more(3)

            def pair_body(i, c):
                pair(i, False)
                return c
            jax.lax.fori_loop(1, NP, pair_body, 0)
            cp_mem.wait()
            mem_s[...] = jnp.concatenate([mem0[...].astype(F32), jnp.zeros((M, DP - DM), F32)], axis=1)
            cp_ckv.wait()

        with jax.named_scope('phase1'):
            pl.run_scoped(phase1, packed(DM, S), packed(DM, S), pltpu.VMEM((M, DM), BF16),
                          *[pltpu.VMEM((NP, DM, DH), U32)] * 3)

        def chain_step(s, held):
            mem = mem_s[...]
            zero = s >> 10
            mt = mem[:, KM:]
            mtail = jnp.concatenate([mt, pltpu.roll(mt, 64, 1)], axis=0).astype(BF16)
            t = []
            for g in range(0, NP * PT, 8):
                for t0 in (g, g + 4):
                    acc = _zeros(s, (M, 512))
                    for k0 in range(0, KM, 128):
                        w = jnp.concatenate([wqkv[t0 + j + zero, _half(k0, 128), :] for j in range(4)], axis=1)
                        yield
                        acc = acc + _dot(mem[:, k0:k0 + 128], _bf(w))
                        yield
                    t += [acc[:, j * 128:(j + 1) * 128] for j in range(4)]
                w = jnp.concatenate([wqkv_t[g // 2 + j + zero] for j in range(4)], axis=1)
                yield
                d = _dot(mtail, _bf(w))
                for j in range(8):
                    t[g + j] = t[g + j] + d[(j % 2) * M:(j % 2 + 1) * M, (j // 2) * 128:(j // 2 + 1) * 128]
                yield
            for _ in range(2 * GAPS[0]):
                yield

            def head_rows(i, which, par):
                t0 = PT * i + (2 * which + par) * HT
                return jnp.concatenate(t[t0:t0 + HT], axis=1)

            def pair_rows(i, which):
                return jnp.concatenate([head_rows(i, which, 0), head_rows(i, which, 1)], axis=0)

            def window(ref, i, which):
                xr = _half(s * SEG, SEG)
                return jnp.concatenate([_bf(ref[2 * i, xr, :]), _bf(ref[2 * i + 1, xr, :]),
                                        pair_rows(i, which).astype(BF16)], axis=0)

            now = [[head_rows(h // 2, which, h % 2) for h in range(H)] for which in (1, 2)]
            if held:
                for ref, old, new in zip((km, vm), held.pop(), now):
                    for h in range(H):
                        ref[h, _half((s - 1) * M, 2 * M), :] = _u32(jnp.concatenate([old[h], new[h]], axis=0))
            else:
                held.append(now)
            sc = []
            for i0 in range(0, NP, 2):
                ops = [((pair_rows(i, 0) * QSC).astype(BF16), window(kx, i, 1)) for i in (i0, i0 + 1)]
                yield
                sc += [_dot_nt(q, k) for q, k in ops]
                yield
            for _ in range(2 * GAPS[1]):
                yield
            sc = jnp.concatenate(sc, axis=0)
            par = (jax.lax.broadcasted_iota(jnp.int32, sc.shape, 0) // M) % 2
            ci = jax.lax.broadcasted_iota(jnp.int32, sc.shape, 1)
            own = jnp.where(ci < 2 * SEG, ci // SEG, (ci - 2 * SEG) // M) == par
            p = _softmax2(jnp.where(own, sc, NEG))
            zt = []
            for i0 in range(0, NP, 2):
                ops = [(p[2 * M * i:2 * M * (i + 1)], window(vx, i, 2)) for i in (i0, i0 + 1)]
                yield
                for pp, v in ops:
                    o = _dot(pp, v)
                    zt += [o[par * M:(par + 1) * M, j * 128:(j + 1) * 128] for par in range(2) for j in range(HT)]
                yield
            for _ in range(2 * GAPS[2]):
                yield
            acc = [_zeros(s, (M, 128))] * 3 + [_zeros(s, (2 * M, 128))]
            for g in range(0, H * HT, 8):
                for t0 in (g, g + 4):
                    zp = jnp.concatenate(zt[t0:t0 + 4], axis=1).astype(BF16).astype(F32)
                    for n in range(KM // 128):
                        w = wo[_half((t0 + zero) * 128, 512), n * 128:(n + 1) * 128]
                        yield
                        acc[n] = acc[n] + _dot(zp, _bf(w))
                        yield
                zp = jnp.concatenate([jnp.concatenate(zt[g:g + 8:2], axis=1),
                                      jnp.concatenate(zt[g + 1:g + 8:2], axis=1)], axis=0).astype(BF16)
                w = wo_t[_half((g // 2 + zero) * 128, 512), :]
                yield
                acc[3] = acc[3] + _dot(zp, _bf(w))
                yield
            lane = jax.lax.broadcasted_iota(jnp.int32, (M, 128), 1)
            last = jnp.where(lane < 64, acc[3][:M] + pltpu.roll(acc[3][M:], 64, 1), 0.0)
            mem_s[...] = jnp.concatenate(acc[:3] + [last], axis=1).astype(BF16).astype(F32)
            for _ in range(2 * GAPS[3]):
                yield

        def chain(h):
            held = []
            for j in range(STEPS):
                yield from chain_step(h * STEPS + j, held)

        n_chain = STEPS * ((NP * PT + H * HT) // 8 * 7 + NP + sum(GAPS))
        n_proj = 2 * (QB // MBQ) + (DC // 256) * (QB // MBK + QB // MBV)

        def split(r):
            return 2 if r >= PVR else 1

        def n_scores(r):
            return (r + 2) // 2

        def n_context(r):
            return (r + 1) // 2 * split(r) + (r + 1) % 2

        n_head = ((S // QB) * n_proj + (S // QB // 2) * (DM // OB) - (S // QB // 2 - 1)
                  + sum(n_scores(r) + n_context(r) for r in range(S // QB)))

        def phase2(wq_s, wk_s, wv_s, k_s, v_s):
            def b_head(h):
                i = h // 2
                par = h % 2
                wq_s[...] = _u32(_unpack(bwq[i], par))
                wk_s[...] = _u32(_unpack(bwk[i], par))
                wv_s[...] = _u32(_unpack(bwv[i], par))
                qs, ss, ms, ctxs = {}, {}, {}, {}

                def chunks(r):
                    nk = (r + 1) * QB
                    return [(c0, min(c0 + 256, nk)) for c0 in range(0, nk, 256)]

                def project(r):
                    qp = []
                    for r0 in range(r * QB, (r + 1) * QB, MBQ):
                        rows = _half(r0, MBQ)
                        acc = _zeros(h, (MBQ, DH))
                        for k0, k1 in ((0, 256), (256, DM)):
                            x = _bf(bx[rows, k0:k0 + 256])[:, :k1 - k0]
                            w = _bf(wq_s[_half(k0, k1 - k0), :])
                            yield
                            acc = acc + _dot(x, w)
                            if k1 == DM:
                                qp.append((acc * QSC).astype(BF16))
                                qs[r] = jnp.concatenate(qp, axis=0)
                            yield
                    for w_s, dst, mb in ((wk_s, k_s, MBK), (wv_s, v_s, MBV)):
                        got = []
                        for r0 in range(r * QB, (r + 1) * QB, mb):
                            rows = _half(r0, mb)
                            acc = _zeros(h, (mb, DH))
                            for k0 in range(0, DC, 256):
                                x = _bf(ckv[rows, k0:k0 + 256])
                                w = _bf(w_s[_half(k0, 256), :])
                                yield
                                acc = acc + _dot(x, w)
                                if k0 + 256 == DC:
                                    got.append(acc.astype(BF16))
                                    if len(got) * mb == QB:
                                        blk = jnp.concatenate(got, axis=0)
                                        dst[r][...] = _u32(blk)
                                yield

                def blocks(refs, c0, c1):
                    return _bf(jnp.concatenate([refs[j][...] for j in range(c0 // QB, c1 // QB)], axis=0))

                def scores(r):
                    ss[r] = []
                    m = None
                    for c0, c1 in chunks(r):
                        k = blocks(k_s, c0, c1)
                        yield
                        sc = _dot_nt(qs[r], k)
                        if c1 == (r + 1) * QB:
                            ri = jax.lax.broadcasted_iota(jnp.int32, sc.shape, 0) + r * QB
                            ci = jax.lax.broadcasted_iota(jnp.int32, sc.shape, 1) + c0
                            sc = jnp.where(ci <= ri, sc, NEG)
                        ss[r].append(sc)
                        for t0 in range(0, c1 - c0, 128):
                            m = sc[:, t0:t0 + 128] if m is None else jnp.maximum(m, sc[:, t0:t0 + 128])
                        if c1 == (r + 1) * QB:
                            ms[r] = jnp.max(m, axis=1, keepdims=True)
                        yield

                def context(r):
                    ls = []

                    def weights(c):
                        p = jnp.exp2(ss[r][c] - ms[r])
                        for t0 in range(0, p.shape[1], 128):
                            ls[:] = [p[:, t0:t0 + 128] + ls[0] if ls else p[:, t0:t0 + 128]]
                        return p.astype(BF16)

                    acc = _zeros(h, (QB, DH))
                    nxt = weights(0)
                    for c, (c0, c1) in enumerate(chunks(r)):
                        mb = QB // split(r) if c1 - c0 == 256 else QB
                        p = nxt
                        v = blocks(v_s, c0, c1)
                        new = []
                        for r0 in range(0, QB, mb):
                            yield
                            new.append(acc[r0:r0 + mb] + _dot(p[r0:r0 + mb], v))
                            if r0 == 0 and c1 < (r + 1) * QB:
                                nxt = weights(c + 1)
                            if r0 + mb == QB:
                                acc = jnp.concatenate(new, axis=0)
                                if c1 == (r + 1) * QB:
                                    ctxs[r] = (acc / jnp.sum(ls[0], axis=1, keepdims=True)).astype(BF16)
                            yield

                def output(r):
                    ctx = jnp.concatenate([ctxs[r - 1], ctxs[r]], axis=0)
                    cols = pl.ds((r - 1) * QB, 2 * QB)
                    for n0 in range(0, DM, OB):
                        w = _bf(bwo[h, _half(n0, OB), :])
                        yield
                        accb[n0:n0 + OB, cols] += _dot_nt(w, ctx)
                        yield

                def both(r):
                    a, b = scores(r), context(r - 2)
                    na, nc = n_scores(r) - 1, n_context(r - 2) - 1
                    for j in _order([na, nc]):
                        for _ in range(2):
                            next((a, b)[j])
                            yield
                    for _ in range(2):
                        next(a)
                        next(b)
                        yield
                    _finish([a, b])

                nb = S // QB
                for r in range(nb + 4):
                    parts = []
                    if r < nb:
                        parts.append((project(r), n_proj))
                    if 0 <= r - 4 < nb and (r - 4) % 2 == 1:
                        parts.append((output(r - 4), DM // OB))
                    if r % 2 == 1 and 3 <= r <= nb:
                        parts.append((both(r - 1), n_scores(r - 1) + n_context(r - 3) - 1))
                    else:
                        if 0 <= r - 1 < nb:
                            parts.append((scores(r - 1), n_scores(r - 1)))
                        if 0 <= r - 3 < nb:
                            parts.append((context(r - 3), n_context(r - 3)))
                    yield from _merge(*parts)

            def b_body(h, c):
                i = h // 2

                @pl.when(h % 2 == 0)
                def _():
                    pair_copy(bwq_h, bwq, sem_bq, i).wait()
                    pair_copy(bwk_h, bwk, sem_bk, i).wait()
                    pair_copy(bwv_h, bwv, sem_bv, i).wait()
                    wo_copy(bwo_h, bwo, sem_bo, i).wait()
                for _ in _merge((chain(h), n_chain), (b_head(h), n_head)):
                    pass
                return c
            jax.lax.fori_loop(0, H, b_body, 0)

        with jax.named_scope('phase2'):
            pl.run_scoped(phase2, packed(DM, DH), packed(DC, DH), packed(DC, DH), [packed(QB, DH)] * (S // QB), [packed(QB, DH)] * (S // QB))

        def phase3(acca, ostage):
            ri = jax.lax.broadcasted_iota(jnp.int32, (AB, AB + 2 * M), 0)
            ci = jax.lax.broadcasted_iota(jnp.int32, (AB, AB + 2 * M), 1)
            amask = (((ci < AB) & ((ci // SEG) == (ri // SEG)) & (ci <= ri))
                     | ((ci >= AB) & (((ci - AB) // M) == (ri // SEG))))

            def out_copy(r):
                rows = _half(r * RB, RB)
                return pltpu.make_async_copy(ostage.at[rows, :], out_h.bitcast(U32).at[0, rows, :], sem_out.at[r])

            def a_head(h, first, last):
                wq = head_weight(PT * (h // 2) + (h % 2) * HT)
                qs, ps, ctxs = {}, {}, {}

                def project(r):
                    qs[r] = (_dot(_bf(ax[_half(r * RB, RB), :])[:, :DM], wq) * QSC).astype(BF16)

                def window(xref, mref, j):
                    return _bf(jnp.concatenate([xref[h, _half(j * AB, AB), :],
                                                mref[h, _half(j * 2 * M, 2 * M), :]], axis=0))

                def scores(r):
                    ps[r] = []
                    for j in range(RB // AB):
                        sc = _dot_nt(qs[r][j * AB:(j + 1) * AB], window(kx, km, r * RB // AB + j))
                        ps[r].append(_softmax2(jnp.where(amask, sc, NEG)))

                def context(r):
                    ctxs[r] = jnp.concatenate(
                        [_dot(p, window(vx, vm, r * RB // AB + j)).astype(BF16) for j, p in enumerate(ps[r])],
                        axis=0)

                def output(r, c0, c1):
                    cols = slice(r * RB + c0, r * RB + c1)
                    o = _dot_nt(_bf(awo[h]), ctxs[r][c0:c1])
                    if not first:
                        o = acca[:, cols] + o
                    if not last:
                        acca[:, cols] = o
                        return
                    ostage[_half(r * RB + c0, c1 - c0), :] = _u32(
                        jnp.concatenate([o, accb[:, cols]], axis=0).astype(BF16).T)
                    if c1 == RB:
                        out_copy(r).start()

                nr = S // RB
                project(0)
                project(1)
                for r in range(nr):
                    scores(r)
                    if r > 0:
                        output(r - 1, 0, RB if r + 1 < nr else RB // 2)
                    if r + 2 < nr:
                        project(r + 2)
                    context(r)
                output(nr - 2, RB // 2, RB)
                output(nr - 1, 0, RB // 2)
                output(nr - 1, RB // 2, RB)

            a_head(0, True, False)

            def a_body(h, c):
                a_head(h, False, False)
                return c
            jax.lax.fori_loop(1, H - 1, a_body, 0)
            a_head(H - 1, False, True)
            for r in range(S // RB):
                out_copy(r).wait()

        with jax.named_scope('phase3'):
            pl.run_scoped(phase3, pltpu.VMEM((DM, S), F32), packed(S, 2 * DM))

    scratch = [
        packed(S, DP),
        pltpu.VMEM((M, DP), F32),
        packed(H, DM, DH),
        packed(NP * PT, KM, 128),
        packed(NP * PT // 2, 128, 128),
        packed(H * DH, KM),
        packed(H * DH // 2, 128),
        packed(H, S, DH),
        packed(H, S, DH),
        packed(H, NSEG * M, DH),
        packed(H, NSEG * M, DH),
        packed(S, DP),
        packed(S, DC),
        pltpu.VMEM((NP, DM, DH), U32),
        pltpu.VMEM((NP, DC, DH), U32),
        pltpu.VMEM((NP, DC, DH), U32),
        packed(H, DM, DH),
        pltpu.VMEM((DM, S), F32),
        pltpu.SemaphoreType.DMA((3 + S // RB,)),
    ] + [pltpu.SemaphoreType.DMA((NP,)) for _ in range(8)] + [pltpu.SemaphoreType.DMA((S // RB,))]
    return kernel, scratch


@jax.jit
def pallas_concat_heads__memory_aug_recurrent_mem_tr__compressed_kv_cla__prompt_kernel(
    A_x, A_mem0, A_Wq, A_Wk, A_Wv, A_Wo, A_seg_len, B_x, B_c_kv, B_w_q, B_w_uk, B_w_uv, B_w_o,
):
    del A_seg_len
    _, S, DM = A_x.shape
    M = A_mem0.shape[1]
    H, DH = A_Wq.shape[1], A_Wq.shape[2]
    DC = B_c_kv.shape[2]
    kernel, scratch = _make_kernel(S, DM, H, DH, M, 32, DC)
    return pl.pallas_call(
        kernel,
        out_shape=jax.ShapeDtypeStruct((1, S, 2 * DM), BF16),
        in_specs=[pl.BlockSpec(memory_space=pl.ANY)] * 12,
        out_specs=pl.BlockSpec(memory_space=pl.ANY),
        scratch_shapes=scratch,
        compiler_params=pltpu.CompilerParams(vmem_limit_bytes=126 * 1024 * 1024),
    )(A_x[0].T, A_mem0, A_Wq, A_Wk, A_Wv, A_Wo.transpose(0, 2, 1),
      B_x[0].T, B_c_kv, B_w_q, B_w_uk, B_w_uv, B_w_o.transpose(0, 2, 1))
```

```python
import jax
import jax.numpy as jnp
import jax.experimental.pallas as pl
import jax.experimental.pallas.tpu as pltpu

F32 = jnp.float32
BF16 = jnp.bfloat16
U32 = jnp.uint32
LOG2E = 1.4426950408889634
NEG = -1e30
NN = (((1,), (0,)), ((), ()))
NT = (((1,), (1,)), ((), ()))


def _dot(a, b):
    return jax.lax.dot_general(a, b, NN, preferred_element_type=F32)


def _dot_nt(a, b):
    return jax.lax.dot_general(a, b, NT, preferred_element_type=F32)


def _bf(u):
    return pltpu.bitcast(u, BF16)


def _u32(x):
    return pltpu.bitcast(x.astype(BF16), U32)


def _half(start, size):
    if isinstance(start, int):
        return pl.ds(start // 2, size // 2)
    return pl.ds(pl.multiple_of(start // 2, 8), size // 2)


def _unpack(u, parity):
    if isinstance(parity, int):
        w = (u << 16) if parity == 0 else (u & jnp.uint32(0xFFFF0000))
    else:
        w = (u >> (16 * parity).astype(U32)) << 16
    return pltpu.bitcast(w, F32).astype(BF16)


def _zeros(i, shape):
    return jnp.full(shape, (i >> 10).astype(F32))


def _softmax2(sc):
    p = jnp.exp2(sc - jnp.max(sc, axis=1, keepdims=True))
    return (p / jnp.sum(p, axis=1, keepdims=True)).astype(BF16)


def _order(counts):
    done = [0] * len(counts)
    live = [a for a, n in enumerate(counts) if n > 0]
    order = []
    for _ in range(sum(counts)):
        j = min(live, key=lambda a: ((done[a] + 0.5) / counts[a], a))
        done[j] += 1
        order.append(j)
    return order


def _finish(gens):
    for g in gens:
        for _ in g:
            raise AssertionError("stream longer than announced")


def _merge(*streams):
    for j in _order([n for _, n in streams]):
        for _ in range(2):
            next(streams[j][0])
            yield
    _finish([g for g, _ in streams])


def _make_kernel(S, DM, H, DH, M, SEG, DC):
    NP = H // 2
    NSEG = S // SEG
    DP = 512
    KM = DM // 128 * 128
    HT = DH // 128
    PT = 6 * HT
    STEPS = NSEG // H
    QB = 128
    OB = DM // 4
    PVR = 8
    MBQ, MBK, MBV = 64, 64, 64
    GAPS = (2, 3, 2, 2)
    RB = 512
    OUT = 256
    AB = 2 * SEG
    QSC = LOG2E * DH ** -0.5

    def packed(*shape):
        return pltpu.VMEM(shape[:-2] + (shape[-2] // 2, shape[-1]), U32)

    def kernel(ax_h, mem_h, awq_h, awk_h, awv_h, awo_h, bx_h, ckv_h, bwq_h, bwk_h, bwv_h, bwo_h,
               out_h,
               ax, mem_s, awo, wqkv, wqkv_t, wo, wo_t, kx, vx, km, vm,
               bx, ckv, bwq, bwk, bwv, bwo, accb,
               sem_x, sem_aq, sem_ak, sem_av, sem_ao, sem_bq, sem_bk, sem_bv, sem_bo, sem_out):

        def pair_copy(src, dst, sem, i):
            return pltpu.make_async_copy(src.bitcast(U32).at[:, i, :], dst.at[i], sem.at[i])

        def wo_copy(src, dst, sem, i):
            return pltpu.make_async_copy(src.bitcast(U32).at[pl.ds(2 * i, 2)], dst.at[pl.ds(2 * i, 2)], sem.at[i])

        def head_weight(t):
            return _bf(jnp.concatenate(
                [jnp.concatenate([wqkv[t + j], wqkv_t[t // 2 + j // 2, _half((j % 2) * 64, 64), :]], axis=0)
                 for j in range(HT)], axis=1))

        def transposed(raw, c, n):
            xt = _bf(raw[:, pl.ds(pl.multiple_of(c, n), n)])
            return _u32(jnp.concatenate([xt, jnp.zeros((DP - DM, n), BF16)], axis=0).T)

        def phase1(axraw, bxraw, mem0, awq, awk, awv):
            def cp_ax(r):
                cols = pl.ds(r * RB if isinstance(r, int) else pl.multiple_of(r * RB, RB), RB)
                return pltpu.make_async_copy(ax_h.bitcast(U32).at[:, cols], axraw.at[:, cols], sem_x.at[3 + r])

            cp_mem = pltpu.make_async_copy(mem_h.at[0], mem0, sem_x.at[0])
            cp_bx = pltpu.make_async_copy(bx_h.bitcast(U32), bxraw, sem_x.at[1])
            cp_ckv = pltpu.make_async_copy(ckv_h.bitcast(U32).at[0], ckv, sem_x.at[2])

            def a_weights(i):
                pair_copy(awk_h, awk, sem_ak, i).start()
                pair_copy(awv_h, awv, sem_av, i).start()
                pair_copy(awq_h, awq, sem_aq, i).start()
                wo_copy(awo_h, awo, sem_ao, i).start()

            def b_weights(i):
                pair_copy(bwq_h, bwq, sem_bq, i).start()
                pair_copy(bwk_h, bwk, sem_bk, i).start()
                pair_copy(bwv_h, bwv, sem_bv, i).start()
                wo_copy(bwo_h, bwo, sem_bo, i).start()

            for r in range(S // RB):
                cp_ax(r).start()
            a_weights(0)
            cp_bx.start()
            cp_mem.start()

            def keep(w, t):
                u = _u32(w)
                for j in range(HT):
                    wqkv[t + j] = u[:KM // 2, j * 128:(j + 1) * 128]
                    wqkv_t[t // 2 + j // 2, _half((j % 2) * 64, 64), :] = u[KM // 2:, j * 128:(j + 1) * 128]

            def x_body(r, c):
                cp_ax(r).wait()
                for j in range(0, RB, 256):
                    ax[_half(r * RB + j, 256), :] = transposed(axraw, r * RB + j, 256)
                return c
            jax.lax.fori_loop(0, S // RB, x_body, 0)
            cp_bx.wait()
            pl.loop(1, NP)(a_weights)
            cp_ckv.start()
            pl.loop(0, NP)(b_weights)

            def kv_body(h, c):
                i = h // 2
                par = h % 2

                @pl.when(par == 0)
                def _():
                    pair_copy(awk_h, awk, sem_ak, i).wait()
                    pair_copy(awv_h, awv, sem_av, i).wait()
                    pair_copy(awq_h, awq, sem_aq, i).wait()
                    wo_copy(awo_h, awo, sem_ao, i).wait()
                wk, wv = _unpack(awk[i], par), _unpack(awv[i], par)
                for r in range(S // RB):
                    rows = _half(r * RB, RB)
                    x = _bf(ax[rows, :])[:, :DM]
                    kx[h, rows, :] = _u32(_dot(x, wk))
                    vx[h, rows, :] = _u32(_dot(x, wv))
                keep(_unpack(awq[i], par), PT * i + par * HT)
                keep(wk, PT * i + (2 + par) * HT)
                keep(wv, PT * i + (4 + par) * HT)
                w = _u32(jnp.concatenate([_bf(awo[h]), jnp.zeros((DP - DM, DH), BF16)], axis=0).T)
                wo[_half(h * DH, DH), :] = w[:, :KM]
                wo_t[_half(h * 128, 128), :] = w[:64, KM:] | pltpu.roll(w[64:, KM:], 64, 1)
                n = S // H
                bx[_half(h * n, n), :] = transposed(bxraw, h * n, n)
                accb[:, pl.ds(pl.multiple_of(h * n, n), n)] = jnp.zeros((DM, n), F32)
                return c
            jax.lax.fori_loop(0, H, kv_body, 0)
            cp_mem.wait()
            mem_s[...] = jnp.concatenate([mem0[...].astype(F32), jnp.zeros((M, DP - DM), F32)], axis=1)
            cp_ckv.wait()

        with jax.named_scope('phase1'):
            pl.run_scoped(phase1, packed(DM, S), packed(DM, S), pltpu.VMEM((M, DM), BF16),
                          *[pltpu.VMEM((NP, DM, DH), U32)] * 3)

        def chain_step(s, held):
            mem = mem_s[...]
            zero = s >> 10
            mt = mem[:, KM:]
            mtail = jnp.concatenate([mt, pltpu.roll(mt, 64, 1)], axis=0).astype(BF16)
            t = []
            for g in range(0, NP * PT, 8):
                for t0 in (g, g + 4):
                    acc = _zeros(s, (M, 512))
                    for k0 in range(0, KM, 128):
                        w = jnp.concatenate([wqkv[t0 + j + zero, _half(k0, 128), :] for j in range(4)], axis=1)
                        yield
                        acc = acc + _dot(mem[:, k0:k0 + 128], _bf(w))
                        yield
                    t += [acc[:, j * 128:(j + 1) * 128] for j in range(4)]
                w = jnp.concatenate([wqkv_t[g // 2 + j + zero] for j in range(4)], axis=1)
                yield
                d = _dot(mtail, _bf(w))
                for j in range(8):
                    t[g + j] = t[g + j] + d[(j % 2) * M:(j % 2 + 1) * M, (j // 2) * 128:(j // 2 + 1) * 128]
                yield
            for _ in range(2 * GAPS[0]):
                yield

            def head_rows(i, which, par):
                t0 = PT * i + (2 * which + par) * HT
                return jnp.concatenate(t[t0:t0 + HT], axis=1)

            def pair_rows(i, which):
                return jnp.concatenate([head_rows(i, which, 0), head_rows(i, which, 1)], axis=0)

            def window(ref, i, which):
                xr = _half(s * SEG, SEG)
                return jnp.concatenate([_bf(ref[2 * i, xr, :]), _bf(ref[2 * i + 1, xr, :]),
                                        pair_rows(i, which).astype(BF16)], axis=0)

            now = [[head_rows(h // 2, which, h % 2) for h in range(H)] for which in (1, 2)]
            if held:
                for ref, old, new in zip((km, vm), held.pop(), now):
                    for h in range(H):
                        ref[h, _half((s - 1) * M, 2 * M), :] = _u32(jnp.concatenate([old[h], new[h]], axis=0))
            else:
                held.append(now)
            sc = []
            for i0 in range(0, NP, 2):
                ops = [((pair_rows(i, 0) * QSC).astype(BF16), window(kx, i, 1)) for i in (i0, i0 + 1)]
                yield
                sc += [_dot_nt(q, k) for q, k in ops]
                yield
            for _ in range(2 * GAPS[1]):
                yield
            sc = jnp.concatenate(sc, axis=0)
            par = (jax.lax.broadcasted_iota(jnp.int32, sc.shape, 0) // M) % 2
            ci = jax.lax.broadcasted_iota(jnp.int32, sc.shape, 1)
            own = jnp.where(ci < 2 * SEG, ci // SEG, (ci - 2 * SEG) // M) == par
            p = _softmax2(jnp.where(own, sc, NEG))
            zt = []
            for i0 in range(0, NP, 2):
                ops = [(p[2 * M * i:2 * M * (i + 1)], window(vx, i, 2)) for i in (i0, i0 + 1)]
                yield
                for pp, v in ops:
                    o = _dot(pp, v)
                    zt += [o[par * M:(par + 1) * M, j * 128:(j + 1) * 128] for par in range(2) for j in range(HT)]
                yield
            for _ in range(2 * GAPS[2]):
                yield
            acc = [_zeros(s, (M, 128))] * 3 + [_zeros(s, (2 * M, 128))]
            for g in range(0, H * HT, 8):
                for t0 in (g, g + 4):
                    zp = jnp.concatenate(zt[t0:t0 + 4], axis=1).astype(BF16).astype(F32)
                    for n in range(KM // 128):
                        w = wo[_half((t0 + zero) * 128, 512), n * 128:(n + 1) * 128]
                        yield
                        acc[n] = acc[n] + _dot(zp, _bf(w))
                        yield
                zp = jnp.concatenate([jnp.concatenate(zt[g:g + 8:2], axis=1),
                                      jnp.concatenate(zt[g + 1:g + 8:2], axis=1)], axis=0).astype(BF16)
                w = wo_t[_half((g // 2 + zero) * 128, 512), :]
                yield
                acc[3] = acc[3] + _dot(zp, _bf(w))
                yield
            lane = jax.lax.broadcasted_iota(jnp.int32, (M, 128), 1)
            last = jnp.where(lane < 64, acc[3][:M] + pltpu.roll(acc[3][M:], 64, 1), 0.0)
            mem_s[...] = jnp.concatenate(acc[:3] + [last], axis=1).astype(BF16).astype(F32)
            for _ in range(2 * GAPS[3]):
                yield

        def chain(h):
            held = []
            for j in range(STEPS):
                yield from chain_step(h * STEPS + j, held)

        n_chain = STEPS * ((NP * PT + H * HT) // 8 * 7 + NP + sum(GAPS))
        n_proj = 2 * (QB // MBQ) + (DC // 256) * (QB // MBK + QB // MBV)

        def split(r):
            return 2 if r >= PVR else 1

        def n_scores(r):
            return (r + 2) // 2

        def n_context(r):
            return (r + 1) // 2 * split(r) + (r + 1) % 2

        n_head = ((S // QB) * n_proj + (S // QB // 2) * (DM // OB) - (S // QB // 2 - 1)
                  + sum(n_scores(r) + n_context(r) for r in range(S // QB)))

        def phase2(wq_s, wk_s, wv_s, k_s, v_s):
            def b_head(h):
                i = h // 2
                par = h % 2
                wq_s[...] = _u32(_unpack(bwq[i], par))
                wk_s[...] = _u32(_unpack(bwk[i], par))
                wv_s[...] = _u32(_unpack(bwv[i], par))
                qs, ss, ms, ctxs = {}, {}, {}, {}

                def chunks(r):
                    nk = (r + 1) * QB
                    return [(c0, min(c0 + 256, nk)) for c0 in range(0, nk, 256)]

                def project(r):
                    qp = []
                    for r0 in range(r * QB, (r + 1) * QB, MBQ):
                        rows = _half(r0, MBQ)
                        acc = _zeros(h, (MBQ, DH))
                        for k0, k1 in ((0, 256), (256, DM)):
                            x = _bf(bx[rows, k0:k0 + 256])[:, :k1 - k0]
                            w = _bf(wq_s[_half(k0, k1 - k0), :])
                            yield
                            acc = acc + _dot(x, w)
                            if k1 == DM:
                                qp.append((acc * QSC).astype(BF16))
                                qs[r] = jnp.concatenate(qp, axis=0)
                            yield
                    for w_s, dst, mb in ((wk_s, k_s, MBK), (wv_s, v_s, MBV)):
                        got = []
                        for r0 in range(r * QB, (r + 1) * QB, mb):
                            rows = _half(r0, mb)
                            acc = _zeros(h, (mb, DH))
                            for k0 in range(0, DC, 256):
                                x = _bf(ckv[rows, k0:k0 + 256])
                                w = _bf(w_s[_half(k0, 256), :])
                                yield
                                acc = acc + _dot(x, w)
                                if k0 + 256 == DC:
                                    got.append(acc.astype(BF16))
                                    if len(got) * mb == QB:
                                        blk = jnp.concatenate(got, axis=0)
                                        dst[r][...] = _u32(blk)
                                yield

                def blocks(refs, c0, c1):
                    return _bf(jnp.concatenate([refs[j][...] for j in range(c0 // QB, c1 // QB)], axis=0))

                def scores(r):
                    ss[r] = []
                    m = None
                    for c0, c1 in chunks(r):
                        k = blocks(k_s, c0, c1)
                        yield
                        sc = _dot_nt(qs[r], k)
                        if c1 == (r + 1) * QB:
                            ri = jax.lax.broadcasted_iota(jnp.int32, sc.shape, 0) + r * QB
                            ci = jax.lax.broadcasted_iota(jnp.int32, sc.shape, 1) + c0
                            sc = jnp.where(ci <= ri, sc, NEG)
                        ss[r].append(sc)
                        for t0 in range(0, c1 - c0, 128):
                            m = sc[:, t0:t0 + 128] if m is None else jnp.maximum(m, sc[:, t0:t0 + 128])
                        if c1 == (r + 1) * QB:
                            ms[r] = jnp.max(m, axis=1, keepdims=True)
                        yield

                def context(r):
                    ls = []

                    def weights(c):
                        p = jnp.exp2(ss[r][c] - ms[r])
                        for t0 in range(0, p.shape[1], 128):
                            ls[:] = [p[:, t0:t0 + 128] + ls[0] if ls else p[:, t0:t0 + 128]]
                        return p.astype(BF16)

                    acc = _zeros(h, (QB, DH))
                    nxt = weights(0)
                    for c, (c0, c1) in enumerate(chunks(r)):
                        mb = QB // split(r) if c1 - c0 == 256 else QB
                        p = nxt
                        v = blocks(v_s, c0, c1)
                        new = []
                        for r0 in range(0, QB, mb):
                            yield
                            new.append(acc[r0:r0 + mb] + _dot(p[r0:r0 + mb], v))
                            if r0 == 0 and c1 < (r + 1) * QB:
                                nxt = weights(c + 1)
                            if r0 + mb == QB:
                                acc = jnp.concatenate(new, axis=0)
                                if c1 == (r + 1) * QB:
                                    ctxs[r] = (acc / jnp.sum(ls[0], axis=1, keepdims=True)).astype(BF16)
                            yield

                def output(r):
                    ctx = jnp.concatenate([ctxs[r - 1], ctxs[r]], axis=0)
                    cols = pl.ds((r - 1) * QB, 2 * QB)
                    for n0 in range(0, DM, OB):
                        w = _bf(bwo[h, _half(n0, OB), :])
                        yield
                        accb[n0:n0 + OB, cols] += _dot_nt(w, ctx)
                        yield

                def both(r):
                    a, b = scores(r), context(r - 2)
                    na, nc = n_scores(r) - 1, n_context(r - 2) - 1
                    for j in _order([na, nc]):
                        for _ in range(2):
                            next((a, b)[j])
                            yield
                    for _ in range(2):
                        next(a)
                        next(b)
                        yield
                    _finish([a, b])

                nb = S // QB
                for r in range(nb + 4):
                    parts = []
                    if r < nb:
                        parts.append((project(r), n_proj))
                    if 0 <= r - 4 < nb and (r - 4) % 2 == 1:
                        parts.append((output(r - 4), DM // OB))
                    if r % 2 == 1 and 3 <= r <= nb:
                        parts.append((both(r - 1), n_scores(r - 1) + n_context(r - 3) - 1))
                    else:
                        if 0 <= r - 1 < nb:
                            parts.append((scores(r - 1), n_scores(r - 1)))
                        if 0 <= r - 3 < nb:
                            parts.append((context(r - 3), n_context(r - 3)))
                    yield from _merge(*parts)

            def b_body(h, c):
                i = h // 2

                @pl.when(h % 2 == 0)
                def _():
                    pair_copy(bwq_h, bwq, sem_bq, i).wait()
                    pair_copy(bwk_h, bwk, sem_bk, i).wait()
                    pair_copy(bwv_h, bwv, sem_bv, i).wait()
                    wo_copy(bwo_h, bwo, sem_bo, i).wait()
                for _ in _merge((chain(h), n_chain), (b_head(h), n_head)):
                    pass
                return c
            jax.lax.fori_loop(0, H, b_body, 0)

        with jax.named_scope('phase2'):
            pl.run_scoped(phase2, packed(DM, DH), packed(DC, DH), packed(DC, DH), [packed(QB, DH)] * (S // QB), [packed(QB, DH)] * (S // QB))

        def phase3(acca, ostage):
            ri = jax.lax.broadcasted_iota(jnp.int32, (AB, AB + 2 * M), 0)
            ci = jax.lax.broadcasted_iota(jnp.int32, (AB, AB + 2 * M), 1)
            amask = (((ci < AB) & ((ci // SEG) == (ri // SEG)) & (ci <= ri))
                     | ((ci >= AB) & (((ci - AB) // M) == (ri // SEG))))

            def out_copy(r):
                rows = _half(r * OUT, OUT)
                return pltpu.make_async_copy(ostage.at[rows, :], out_h.bitcast(U32).at[0, rows, :], sem_out.at[r])

            def a_head(h):
                wq = head_weight(PT * (h // 2) + (h % 2) * HT)
                qs, ps, ctxs = {}, {}, {}

                def project(r):
                    qs[r] = (_dot(_bf(ax[_half(r * RB, RB), :])[:, :DM], wq) * QSC).astype(BF16)

                def window(xref, mref, j):
                    return _bf(jnp.concatenate([xref[h, _half(j * AB, AB), :],
                                                mref[h, _half(j * 2 * M, 2 * M), :]], axis=0))

                def scores(r):
                    ps[r] = []
                    for j in range(RB // AB):
                        sc = _dot_nt(qs[r][j * AB:(j + 1) * AB], window(kx, km, r * RB // AB + j))
                        ps[r].append(_softmax2(jnp.where(amask, sc, NEG)))

                def context(r):
                    ctxs[r] = jnp.concatenate(
                        [_dot(p, window(vx, vm, r * RB // AB + j)).astype(BF16) for j, p in enumerate(ps[r])],
                        axis=0)

                def output(r, c0, c1):
                    cols = slice(r * RB + c0, r * RB + c1)
                    acca[:, cols] = jnp.where(h > 0, acca[:, cols], 0.0) + _dot_nt(_bf(awo[h]), ctxs[r][c0:c1])

                nr = S // RB
                project(0)
                project(1)
                for r in range(nr):
                    scores(r)
                    if r > 0:
                        output(r - 1, 0, RB if r + 1 < nr else RB // 2)
                    if r + 2 < nr:
                        project(r + 2)
                    context(r)
                output(nr - 2, RB // 2, RB)
                output(nr - 1, 0, RB // 2)
                output(nr - 1, RB // 2, RB)

            pl.loop(0, H)(a_head)

            @pl.loop(0, S // OUT)
            def _(r):
                cols = pl.ds(pl.multiple_of(r * OUT, OUT), OUT)
                ostage[_half(r * OUT, OUT), :] = _u32(
                    jnp.concatenate([acca[:, cols], accb[:, cols]], axis=0).astype(BF16).T)
                out_copy(r).start()

            @pl.loop(0, S // OUT)
            def _(r):
                out_copy(r).wait()

        with jax.named_scope('phase3'):
            pl.run_scoped(phase3, pltpu.VMEM((DM, S), F32), packed(S, 2 * DM))

    scratch = [
        packed(S, DP),
        pltpu.VMEM((M, DP), F32),
        packed(H, DM, DH),
        packed(NP * PT, KM, 128),
        packed(NP * PT // 2, 128, 128),
        packed(H * DH, KM),
        packed(H * DH // 2, 128),
        packed(H, S, DH),
        packed(H, S, DH),
        packed(H, NSEG * M, DH),
        packed(H, NSEG * M, DH),
        packed(S, DP),
        packed(S, DC),
        pltpu.VMEM((NP, DM, DH), U32),
        pltpu.VMEM((NP, DC, DH), U32),
        pltpu.VMEM((NP, DC, DH), U32),
        packed(H, DM, DH),
        pltpu.VMEM((DM, S), F32),
        pltpu.SemaphoreType.DMA((3 + S // RB,)),
    ] + [pltpu.SemaphoreType.DMA((NP,)) for _ in range(8)] + [pltpu.SemaphoreType.DMA((S // OUT,))]
    return kernel, scratch


@jax.jit
def pallas_concat_heads__memory_aug_recurrent_mem_tr__compressed_kv_cla__prompt_kernel(
    A_x, A_mem0, A_Wq, A_Wk, A_Wv, A_Wo, A_seg_len, B_x, B_c_kv, B_w_q, B_w_uk, B_w_uv, B_w_o,
):
    del A_seg_len
    _, S, DM = A_x.shape
    M = A_mem0.shape[1]
    H, DH = A_Wq.shape[1], A_Wq.shape[2]
    DC = B_c_kv.shape[2]
    kernel, scratch = _make_kernel(S, DM, H, DH, M, 32, DC)
    return pl.pallas_call(
        kernel,
        out_shape=jax.ShapeDtypeStruct((1, S, 2 * DM), BF16),
        in_specs=[pl.BlockSpec(memory_space=pl.ANY)] * 12,
        out_specs=pl.BlockSpec(memory_space=pl.ANY),
        scratch_shapes=scratch,
        compiler_params=pltpu.CompilerParams(vmem_limit_bytes=126 * 1024 * 1024),
    )(A_x[0].T, A_mem0, A_Wq, A_Wk, A_Wv, A_Wo.transpose(0, 2, 1),
      B_x[0].T, B_c_kv, B_w_q, B_w_uk, B_w_uv, B_w_o.transpose(0, 2, 1))
```

```python
import jax
import jax.numpy as jnp
import jax.experimental.pallas as pl
import jax.experimental.pallas.tpu as pltpu

F32 = jnp.float32
BF16 = jnp.bfloat16
U32 = jnp.uint32
LOG2E = 1.4426950408889634
NEG = -1e30
NN = (((1,), (0,)), ((), ()))
NT = (((1,), (1,)), ((), ()))


def _dot(a, b):
    return jax.lax.dot_general(a, b, NN, preferred_element_type=F32)


def _dot_nt(a, b):
    return jax.lax.dot_general(a, b, NT, preferred_element_type=F32)


def _bf(u):
    return pltpu.bitcast(u, BF16)


def _u32(x):
    return pltpu.bitcast(x.astype(BF16), U32)


def _half(start, size):
    if isinstance(start, int):
        return pl.ds(start // 2, size // 2)
    return pl.ds(pl.multiple_of(start // 2, 8), size // 2)


def _unpack(u, parity):
    if isinstance(parity, int):
        w = (u << 16) if parity == 0 else (u & jnp.uint32(0xFFFF0000))
    else:
        w = (u >> (16 * parity).astype(U32)) << 16
    return pltpu.bitcast(w, F32).astype(BF16)


def _zeros(i, shape):
    return jnp.full(shape, (i >> 10).astype(F32))


def _softmax2(sc):
    p = jnp.exp2(sc - jnp.max(sc, axis=1, keepdims=True))
    return (p / jnp.sum(p, axis=1, keepdims=True)).astype(BF16)


def _order(counts):
    done = [0] * len(counts)
    live = [a for a, n in enumerate(counts) if n > 0]
    order = []
    for _ in range(sum(counts)):
        j = min(live, key=lambda a: ((done[a] + 0.5) / counts[a], a))
        done[j] += 1
        order.append(j)
    return order


def _finish(gens):
    for g in gens:
        for _ in g:
            raise AssertionError("stream longer than announced")


def _merge(*streams):
    for j in _order([n for _, n in streams]):
        for _ in range(2):
            next(streams[j][0])
            yield
    _finish([g for g, _ in streams])


def _make_kernel(S, DM, H, DH, M, SEG, DC):
    NP = H // 2
    NSEG = S // SEG
    DP = 512
    KM = DM // 128 * 128
    HT = DH // 128
    PT = 6 * HT
    STEPS = NSEG // H
    QB = 128
    OB = DM // 4
    PVR = 8
    MBQ, MBK, MBV = 64, 64, 64
    GAPS = (2, 3, 2, 2)
    RB = 512
    OUT = 256
    XC = S // H
    AB = 2 * SEG
    QSC = LOG2E * DH ** -0.5

    def packed(*shape):
        return pltpu.VMEM(shape[:-2] + (shape[-2] // 2, shape[-1]), U32)

    def kernel(ax_h, mem_h, awq_h, awk_h, awv_h, awo_h, bx_h, ckv_h, bwq_h, bwk_h, bwv_h, bwo_h,
               out_h,
               ax, mem_s, awo, wqkv, wqkv_t, wo, wo_t, kx, vx, km, vm,
               bx, ckv, bwq, bwk, bwv, bwo, accb,
               sem_x, sem_aq, sem_ak, sem_av, sem_ao, sem_bq, sem_bk, sem_bv, sem_bo, sem_out):

        def pair_copy(src, dst, sem, i):
            return pltpu.make_async_copy(src.bitcast(U32).at[:, i, :], dst.at[i], sem.at[i])

        def wo_copy(src, dst, sem, i):
            return pltpu.make_async_copy(src.bitcast(U32).at[pl.ds(2 * i, 2)], dst.at[pl.ds(2 * i, 2)], sem.at[i])

        def head_weight(t):
            return _bf(jnp.concatenate(
                [jnp.concatenate([wqkv[t + j], wqkv_t[t // 2 + j // 2, _half((j % 2) * 64, 64), :]], axis=0)
                 for j in range(HT)], axis=1))

        def transposed(raw, c, n):
            xt = _bf(raw[:, pl.ds(c if isinstance(c, int) else pl.multiple_of(c, n), n)])
            return _u32(jnp.concatenate([xt, jnp.zeros((DP - DM, n), BF16)], axis=0).T)

        def phase1(xraw, mem0, awq, awk, awv):
            def cp_ax(r):
                cols = pl.ds(r * RB if isinstance(r, int) else pl.multiple_of(r * RB, RB), RB)
                return pltpu.make_async_copy(ax_h.bitcast(U32).at[:, cols], xraw.at[:, cols], sem_x.at[3 + r])

            cp_mem = pltpu.make_async_copy(mem_h.at[0], mem0, sem_x.at[0])
            cp_bx = pltpu.make_async_copy(bx_h.bitcast(U32), xraw.at[:, pl.ds(S, S)], sem_x.at[1])
            cp_ckv = pltpu.make_async_copy(ckv_h.bitcast(U32).at[0], ckv, sem_x.at[2])

            def a_weights(i):
                pair_copy(awk_h, awk, sem_ak, i).start()
                pair_copy(awv_h, awv, sem_av, i).start()
                pair_copy(awq_h, awq, sem_aq, i).start()
                wo_copy(awo_h, awo, sem_ao, i).start()

            def b_weights(i):
                pair_copy(bwq_h, bwq, sem_bq, i).start()
                pair_copy(bwk_h, bwk, sem_bk, i).start()
                pair_copy(bwv_h, bwv, sem_bv, i).start()
                wo_copy(bwo_h, bwo, sem_bo, i).start()

            for r in range(S // RB):
                cp_ax(r).start()
            a_weights(0)

            def keep(w, t):
                u = _u32(w)
                for j in range(HT):
                    wqkv[t + j] = u[:KM // 2, j * 128:(j + 1) * 128]
                    wqkv_t[t // 2 + j // 2, _half((j % 2) * 64, 64), :] = u[KM // 2:, j * 128:(j + 1) * 128]

            def keep_kv(h):
                i = h // 2
                keep(_unpack(awk[i], h % 2), PT * i + (2 + h % 2) * HT)
                keep(_unpack(awv[i], h % 2), PT * i + (4 + h % 2) * HT)

            def keep_bx(j):
                bx[_half(j * XC, XC), :] = transposed(xraw, S + (j - 1) * XC, XC)

            @pl.loop(0, S // RB)
            def _(r):
                cp_ax(r).wait()
                for j in range(0, RB, 256):
                    ax[_half(r * RB + j, 256), :] = transposed(xraw, r * RB + j, 256)
            cp_bx.start()
            cp_mem.start()
            pl.loop(1, NP)(a_weights)
            cp_ckv.start()
            pl.loop(0, NP)(b_weights)
            pair_copy(awk_h, awk, sem_ak, 0).wait()
            pair_copy(awv_h, awv, sem_av, 0).wait()
            keep_kv(0)

            @pl.loop(0, H)
            def _(h):
                i = h // 2
                par = h % 2

                @pl.when(par == 0)
                def _():
                    pair_copy(awq_h, awq, sem_aq, i).wait()
                    wo_copy(awo_h, awo, sem_ao, i).wait()

                @pl.when((par == 1) & (i + 1 < NP))
                def _():
                    pair_copy(awk_h, awk, sem_ak, i + 1).wait()
                    pair_copy(awv_h, awv, sem_av, i + 1).wait()

                @pl.when(h == 1)
                def _():
                    cp_bx.wait()
                wk, wv = head_weight(PT * i + (2 + par) * HT), head_weight(PT * i + (4 + par) * HT)
                for r in range(S // RB):
                    rows = _half(r * RB, RB)
                    x = _bf(ax[rows, :])[:, :DM]
                    kx[h, rows, :] = _u32(_dot(x, wk))
                    vx[h, rows, :] = _u32(_dot(x, wv))
                    if r == 0:
                        w = _u32(jnp.concatenate([_bf(awo[h]), jnp.zeros((DP - DM, DH), BF16)], axis=0).T)
                        wo[_half(h * DH, DH), :] = w[:, :KM]
                        wo_t[_half(h * 128, 128), :] = w[:64, KM:] | pltpu.roll(w[64:, KM:], 64, 1)
                        keep_bx(h)
                    if r == 1:
                        keep(_unpack(awq[i], par), PT * i + par * HT)
                        accb[:, pl.ds(pl.multiple_of(h * XC, XC), XC)] = jnp.zeros((DM, XC), F32)
                    if r == 2:
                        keep_kv(jnp.minimum(h + 1, H - 1))
            keep_bx(H)
            cp_mem.wait()
            mem_s[...] = jnp.concatenate([mem0[...].astype(F32), jnp.zeros((M, DP - DM), F32)], axis=1)
            cp_ckv.wait()

        with jax.named_scope('phase1'):
            pl.run_scoped(phase1, packed(DM, 2 * S), pltpu.VMEM((M, DM), BF16),
                          *[pltpu.VMEM((NP, DM, DH), U32)] * 3)

        def chain_step(s, held):
            mem = mem_s[...]
            zero = s >> 10
            mt = mem[:, KM:]
            mtail = jnp.concatenate([mt, pltpu.roll(mt, 64, 1)], axis=0).astype(BF16)
            t = []
            for g in range(0, NP * PT, 8):
                for t0 in (g, g + 4):
                    acc = _zeros(s, (M, 512))
                    for k0 in range(0, KM, 128):
                        w = jnp.concatenate([wqkv[t0 + j + zero, _half(k0, 128), :] for j in range(4)], axis=1)
                        yield
                        acc = acc + _dot(mem[:, k0:k0 + 128], _bf(w))
                        yield
                    t += [acc[:, j * 128:(j + 1) * 128] for j in range(4)]
                w = jnp.concatenate([wqkv_t[g // 2 + j + zero] for j in range(4)], axis=1)
                yield
                d = _dot(mtail, _bf(w))
                for j in range(8):
                    t[g + j] = t[g + j] + d[(j % 2) * M:(j % 2 + 1) * M, (j // 2) * 128:(j // 2 + 1) * 128]
                yield
            for _ in range(2 * GAPS[0]):
                yield

            def head_rows(i, which, par):
                t0 = PT * i + (2 * which + par) * HT
                return jnp.concatenate(t[t0:t0 + HT], axis=1)

            def pair_rows(i, which):
                return jnp.concatenate([head_rows(i, which, 0), head_rows(i, which, 1)], axis=0)

            def window(ref, i, which):
                xr = _half(s * SEG, SEG)
                return jnp.concatenate([_bf(ref[2 * i, xr, :]), _bf(ref[2 * i + 1, xr, :]),
                                        pair_rows(i, which).astype(BF16)], axis=0)

            now = [[head_rows(h // 2, which, h % 2) for h in range(H)] for which in (1, 2)]
            if held:
                for ref, old, new in zip((km, vm), held.pop(), now):
                    for h in range(H):
                        ref[h, _half((s - 1) * M, 2 * M), :] = _u32(jnp.concatenate([old[h], new[h]], axis=0))
            else:
                held.append(now)
            sc = []
            for i0 in range(0, NP, 2):
                ops = [((pair_rows(i, 0) * QSC).astype(BF16), window(kx, i, 1)) for i in (i0, i0 + 1)]
                yield
                sc += [_dot_nt(q, k) for q, k in ops]
                yield
            for _ in range(2 * GAPS[1]):
                yield
            sc = jnp.concatenate(sc, axis=0)
            par = (jax.lax.broadcasted_iota(jnp.int32, sc.shape, 0) // M) % 2
            ci = jax.lax.broadcasted_iota(jnp.int32, sc.shape, 1)
            own = jnp.where(ci < 2 * SEG, ci // SEG, (ci - 2 * SEG) // M) == par
            p = _softmax2(jnp.where(own, sc, NEG))
            zt = []
            for i0 in range(0, NP, 2):
                ops = [(p[2 * M * i:2 * M * (i + 1)], window(vx, i, 2)) for i in (i0, i0 + 1)]
                yield
                for pp, v in ops:
                    o = _dot(pp, v)
                    zt += [o[par * M:(par + 1) * M, j * 128:(j + 1) * 128] for par in range(2) for j in range(HT)]
                yield
            for _ in range(2 * GAPS[2]):
                yield
            acc = [_zeros(s, (M, 128))] * 3 + [_zeros(s, (2 * M, 128))]
            for g in range(0, H * HT, 8):
                for t0 in (g, g + 4):
                    zp = jnp.concatenate(zt[t0:t0 + 4], axis=1).astype(BF16).astype(F32)
                    for n in range(KM // 128):
                        w = wo[_half((t0 + zero) * 128, 512), n * 128:(n + 1) * 128]
                        yield
                        acc[n] = acc[n] + _dot(zp, _bf(w))
                        yield
                zp = jnp.concatenate([jnp.concatenate(zt[g:g + 8:2], axis=1),
                                      jnp.concatenate(zt[g + 1:g + 8:2], axis=1)], axis=0).astype(BF16)
                w = wo_t[_half((g // 2 + zero) * 128, 512), :]
                yield
                acc[3] = acc[3] + _dot(zp, _bf(w))
                yield
            lane = jax.lax.broadcasted_iota(jnp.int32, (M, 128), 1)
            last = jnp.where(lane < 64, acc[3][:M] + pltpu.roll(acc[3][M:], 64, 1), 0.0)
            mem_s[...] = jnp.concatenate(acc[:3] + [last], axis=1).astype(BF16).astype(F32)
            for _ in range(2 * GAPS[3]):
                yield

        def chain(h):
            held = []
            for j in range(STEPS):
                yield from chain_step(h * STEPS + j, held)

        n_chain = STEPS * ((NP * PT + H * HT) // 8 * 7 + NP + sum(GAPS))
        n_proj = 2 * (QB // MBQ) + (DC // 256) * (QB // MBK + QB // MBV)

        def split(r):
            return 2 if r >= PVR else 1

        def n_scores(r):
            return (r + 2) // 2

        def n_context(r):
            return (r + 1) // 2 * split(r) + (r + 1) % 2

        n_head = ((S // QB) * n_proj + (S // QB // 2) * (DM // OB) - (S // QB // 2 - 1)
                  + sum(n_scores(r) + n_context(r) for r in range(S // QB)))

        def phase2(wq_s, wk_s, wv_s, k_s, v_s):
            def b_head(h):
                i = h // 2
                par = h % 2
                wq_s[...] = _u32(_unpack(bwq[i], par))
                wk_s[...] = _u32(_unpack(bwk[i], par))
                wv_s[...] = _u32(_unpack(bwv[i], par))
                qs, ss, ms, ctxs = {}, {}, {}, {}

                def chunks(r):
                    nk = (r + 1) * QB
                    return [(c0, min(c0 + 256, nk)) for c0 in range(0, nk, 256)]

                def project(r):
                    qp = []
                    for r0 in range(r * QB, (r + 1) * QB, MBQ):
                        acc = _zeros(h, (MBQ, DH))
                        for k0, k1 in ((0, 256), (256, DM)):
                            x = _bf(bx[_half(XC + r0, MBQ), k0:k0 + 256])[:, :k1 - k0]
                            w = _bf(wq_s[_half(k0, k1 - k0), :])
                            yield
                            acc = acc + _dot(x, w)
                            if k1 == DM:
                                qp.append((acc * QSC).astype(BF16))
                                qs[r] = jnp.concatenate(qp, axis=0)
                            yield
                    for w_s, dst, mb in ((wk_s, k_s, MBK), (wv_s, v_s, MBV)):
                        got = []
                        for r0 in range(r * QB, (r + 1) * QB, mb):
                            rows = _half(r0, mb)
                            acc = _zeros(h, (mb, DH))
                            for k0 in range(0, DC, 256):
                                x = _bf(ckv[rows, k0:k0 + 256])
                                w = _bf(w_s[_half(k0, 256), :])
                                yield
                                acc = acc + _dot(x, w)
                                if k0 + 256 == DC:
                                    got.append(acc.astype(BF16))
                                    if len(got) * mb == QB:
                                        blk = jnp.concatenate(got, axis=0)
                                        dst[r][...] = _u32(blk)
                                yield

                def blocks(refs, c0, c1):
                    return _bf(jnp.concatenate([refs[j][...] for j in range(c0 // QB, c1 // QB)], axis=0))

                def scores(r):
                    ss[r] = []
                    m = None
                    for c0, c1 in chunks(r):
                        k = blocks(k_s, c0, c1)
                        yield
                        sc = _dot_nt(qs[r], k)
                        if c1 == (r + 1) * QB:
                            ri = jax.lax.broadcasted_iota(jnp.int32, sc.shape, 0) + r * QB
                            ci = jax.lax.broadcasted_iota(jnp.int32, sc.shape, 1) + c0
                            sc = jnp.where(ci <= ri, sc, NEG)
                        ss[r].append(sc)
                        for t0 in range(0, c1 - c0, 128):
                            m = sc[:, t0:t0 + 128] if m is None else jnp.maximum(m, sc[:, t0:t0 + 128])
                        if c1 == (r + 1) * QB:
                            ms[r] = jnp.max(m, axis=1, keepdims=True)
                        yield

                def context(r):
                    ls = []

                    def weights(c):
                        p = jnp.exp2(ss[r][c] - ms[r])
                        for t0 in range(0, p.shape[1], 128):
                            ls[:] = [p[:, t0:t0 + 128] + ls[0] if ls else p[:, t0:t0 + 128]]
                        return p.astype(BF16)

                    acc = _zeros(h, (QB, DH))
                    nxt = weights(0)
                    for c, (c0, c1) in enumerate(chunks(r)):
                        mb = QB // split(r) if c1 - c0 == 256 else QB
                        p = nxt
                        v = blocks(v_s, c0, c1)
                        new = []
                        for r0 in range(0, QB, mb):
                            yield
                            new.append(acc[r0:r0 + mb] + _dot(p[r0:r0 + mb], v))
                            if r0 == 0 and c1 < (r + 1) * QB:
                                nxt = weights(c + 1)
                            if r0 + mb == QB:
                                acc = jnp.concatenate(new, axis=0)
                                if c1 == (r + 1) * QB:
                                    ctxs[r] = (acc / jnp.sum(ls[0], axis=1, keepdims=True)).astype(BF16)
                            yield

                def output(r):
                    ctx = jnp.concatenate([ctxs[r - 1], ctxs[r]], axis=0)
                    cols = pl.ds((r - 1) * QB, 2 * QB)
                    for n0 in range(0, DM, OB):
                        w = _bf(bwo[h, _half(n0, OB), :])
                        yield
                        accb[n0:n0 + OB, cols] += _dot_nt(w, ctx)
                        yield

                def both(r):
                    a, b = scores(r), context(r - 2)
                    na, nc = n_scores(r) - 1, n_context(r - 2) - 1
                    for j in _order([na, nc]):
                        for _ in range(2):
                            next((a, b)[j])
                            yield
                    for _ in range(2):
                        next(a)
                        next(b)
                        yield
                    _finish([a, b])

                nb = S // QB
                for r in range(nb + 4):
                    parts = []
                    if r < nb:
                        parts.append((project(r), n_proj))
                    if 0 <= r - 4 < nb and (r - 4) % 2 == 1:
                        parts.append((output(r - 4), DM // OB))
                    if r % 2 == 1 and 3 <= r <= nb:
                        parts.append((both(r - 1), n_scores(r - 1) + n_context(r - 3) - 1))
                    else:
                        if 0 <= r - 1 < nb:
                            parts.append((scores(r - 1), n_scores(r - 1)))
                        if 0 <= r - 3 < nb:
                            parts.append((context(r - 3), n_context(r - 3)))
                    yield from _merge(*parts)

            def b_body(h, c):
                i = h // 2

                @pl.when(h % 2 == 0)
                def _():
                    pair_copy(bwq_h, bwq, sem_bq, i).wait()
                    pair_copy(bwk_h, bwk, sem_bk, i).wait()
                    pair_copy(bwv_h, bwv, sem_bv, i).wait()
                    wo_copy(bwo_h, bwo, sem_bo, i).wait()
                for _ in _merge((chain(h), n_chain), (b_head(h), n_head)):
                    pass
                return c
            jax.lax.fori_loop(0, H, b_body, 0)

        with jax.named_scope('phase2'):
            pl.run_scoped(phase2, packed(DM, DH), packed(DC, DH), packed(DC, DH), [packed(QB, DH)] * (S // QB), [packed(QB, DH)] * (S // QB))

        def phase3(acca, ostage, q0):
            ri = jax.lax.broadcasted_iota(jnp.int32, (AB, AB + 2 * M), 0)
            ci = jax.lax.broadcasted_iota(jnp.int32, (AB, AB + 2 * M), 1)
            amask = (((ci < AB) & ((ci // SEG) == (ri // SEG)) & (ci <= ri))
                     | ((ci >= AB) & (((ci - AB) // M) == (ri // SEG))))

            def out_copy(r):
                rows = _half(r * OUT, OUT)
                return pltpu.make_async_copy(ostage.at[rows, :], out_h.bitcast(U32).at[0, rows, :], sem_out.at[r])

            def query_weight(h):
                return head_weight(PT * (h // 2) + (h % 2) * HT)

            def query(wq, r):
                return (_dot(_bf(ax[_half(r * RB, RB), :])[:, :DM], wq) * QSC).astype(BF16)

            def a_head(h):
                wq = query_weight(h)
                qs, ps, ctxs = {0: _bf(q0[...])}, {}, {}

                def project(r):
                    qs[r] = query(wq, r)

                def window(xref, mref, j):
                    return _bf(jnp.concatenate([xref[h, _half(j * AB, AB), :],
                                                mref[h, _half(j * 2 * M, 2 * M), :]], axis=0))

                def scores(r):
                    ps[r] = []
                    for j in range(RB // AB):
                        sc = _dot_nt(qs[r][j * AB:(j + 1) * AB], window(kx, km, r * RB // AB + j))
                        ps[r].append(_softmax2(jnp.where(amask, sc, NEG)))

                def context(r):
                    ctxs[r] = jnp.concatenate(
                        [_dot(p, window(vx, vm, r * RB // AB + j)).astype(BF16) for j, p in enumerate(ps[r])],
                        axis=0)

                def output(r, c0, c1):
                    cols = slice(r * RB + c0, r * RB + c1)
                    acca[:, cols] = jnp.where(h > 0, acca[:, cols], 0.0) + _dot_nt(_bf(awo[h]), ctxs[r][c0:c1])

                nr = S // RB
                project(1)
                for r in range(nr):
                    scores(r)
                    if r > 0:
                        output(r - 1, 0, RB)
                    if r + 2 < nr:
                        project(r + 2)
                    context(r)
                q0[...] = _u32(query(query_weight(jnp.minimum(h + 1, H - 1)), 0))
                output(nr - 1, 0, RB)

            q0[...] = _u32(query(query_weight(0), 0))
            pl.loop(0, H)(a_head)

            @pl.loop(0, S // OUT)
            def _(r):
                cols = pl.ds(pl.multiple_of(r * OUT, OUT), OUT)
                ostage[_half(r * OUT, OUT), :] = _u32(
                    jnp.concatenate([acca[:, cols], accb[:, cols]], axis=0).astype(BF16).T)
                out_copy(r).start()

            @pl.loop(0, S // OUT)
            def _(r):
                out_copy(r).wait()

        with jax.named_scope('phase3'):
            pl.run_scoped(phase3, pltpu.VMEM((DM, S), F32), packed(S, 2 * DM), packed(RB, DH))

    scratch = [
        packed(S, DP),
        pltpu.VMEM((M, DP), F32),
        packed(H, DM, DH),
        packed(NP * PT, KM, 128),
        packed(NP * PT // 2, 128, 128),
        packed(H * DH, KM),
        packed(H * DH // 2, 128),
        packed(H, S, DH),
        packed(H, S, DH),
        packed(H, NSEG * M, DH),
        packed(H, NSEG * M, DH),
        packed(XC + S, DP),
        packed(S, DC),
        pltpu.VMEM((NP, DM, DH), U32),
        pltpu.VMEM((NP, DC, DH), U32),
        pltpu.VMEM((NP, DC, DH), U32),
        packed(H, DM, DH),
        pltpu.VMEM((DM, S), F32),
        pltpu.SemaphoreType.DMA((3 + S // RB,)),
    ] + [pltpu.SemaphoreType.DMA((NP,)) for _ in range(8)] + [pltpu.SemaphoreType.DMA((S // OUT,))]
    return kernel, scratch


@jax.jit
def pallas_concat_heads__memory_aug_recurrent_mem_tr__compressed_kv_cla__prompt_kernel(
    A_x, A_mem0, A_Wq, A_Wk, A_Wv, A_Wo, A_seg_len, B_x, B_c_kv, B_w_q, B_w_uk, B_w_uv, B_w_o,
):
    del A_seg_len
    _, S, DM = A_x.shape
    M = A_mem0.shape[1]
    H, DH = A_Wq.shape[1], A_Wq.shape[2]
    DC = B_c_kv.shape[2]
    kernel, scratch = _make_kernel(S, DM, H, DH, M, 32, DC)
    return pl.pallas_call(
        kernel,
        out_shape=jax.ShapeDtypeStruct((1, S, 2 * DM), BF16),
        in_specs=[pl.BlockSpec(memory_space=pl.ANY)] * 12,
        out_specs=pl.BlockSpec(memory_space=pl.ANY),
        scratch_shapes=scratch,
        compiler_params=pltpu.CompilerParams(vmem_limit_bytes=126 * 1024 * 1024),
    )(A_x[0].T, A_mem0, A_Wq, A_Wk, A_Wv, A_Wo.transpose(0, 2, 1),
      B_x[0].T, B_c_kv, B_w_q, B_w_uk, B_w_uv, B_w_o.transpose(0, 2, 1))
```

```python
import jax
import jax.numpy as jnp
import jax.experimental.pallas as pl
import jax.experimental.pallas.tpu as pltpu

F32 = jnp.float32
BF16 = jnp.bfloat16
U32 = jnp.uint32
LOG2E = 1.4426950408889634
NEG = -1e30
NN = (((1,), (0,)), ((), ()))
NT = (((1,), (1,)), ((), ()))


def _dot(a, b):
    return jax.lax.dot_general(a, b, NN, preferred_element_type=F32)


def _dot_nt(a, b):
    return jax.lax.dot_general(a, b, NT, preferred_element_type=F32)


def _bf(u):
    return pltpu.bitcast(u, BF16)


def _u32(x):
    return pltpu.bitcast(x.astype(BF16), U32)


def _half(start, size):
    if isinstance(start, int):
        return pl.ds(start // 2, size // 2)
    return pl.ds(pl.multiple_of(start // 2, 8), size // 2)


def _unpack(u, parity):
    if isinstance(parity, int):
        w = (u << 16) if parity == 0 else (u & jnp.uint32(0xFFFF0000))
    else:
        w = (u >> (16 * parity).astype(U32)) << 16
    return pltpu.bitcast(w, F32)


def _lhs_terms(x):
    r, k = x.shape[0] // 2, x.shape[1] // 2
    x11, x12, x21, x22 = x[:r, :k], x[:r, k:], x[r:, :k], x[r:, k:]
    return [x11 + x22, x22, x21 + x22, x11, x11 + x12, x12 - x22, x21 - x11]


def _rhs_terms(w, k):
    n, k2 = w.shape[1] // 2, w.shape[0] - k
    w11, w12, w21, w22 = w[:k, :n], w[:k, n:], w[k:, :n], w[k:, n:]

    def full(a):
        return a if k2 == k else jnp.concatenate([a, jnp.zeros((k - k2, n), a.dtype)], axis=0)
    return [w11 + full(w22), full(w21) - w11, w11, w12 - full(w22), w22, w21 + w22, w11 + w12]


def _block_product(product):
    c = {}
    for n, (first, second) in enumerate((("+11", "+22"), ("+11", "+21"), ("+21", "-22"), ("+12", "+22"),
                                         ("+12", "-11"), ("+11", None), ("+22", None))):
        multiply = product(n)
        yield
        p = multiply()
        for sign, *key in filter(None, (first, second)):
            key = "".join(key)
            c[key] = p if key not in c else c[key] + p if sign == "+" else c[key] - p
        if n < 6:
            yield
    return (jnp.concatenate([c["11"], c["12"]], axis=1).astype(F32),
            jnp.concatenate([c["21"], c["22"]], axis=1).astype(F32))


def _run(gen):
    try:
        while True:
            next(gen)
    except StopIteration as stop:
        return stop.value


def _zeros(i, shape):
    return jnp.full(shape, (i >> 10).astype(F32))


def _softmax2(sc):
    p = jnp.exp2(sc - jnp.max(sc, axis=1, keepdims=True))
    return (p / jnp.sum(p, axis=1, keepdims=True)).astype(BF16)


def _order(counts):
    done = [0] * len(counts)
    live = [a for a, n in enumerate(counts) if n > 0]
    order = []
    for _ in range(sum(counts)):
        j = min(live, key=lambda a: ((done[a] + 0.5) / counts[a], a))
        done[j] += 1
        order.append(j)
    return order


def _finish(gens):
    for g in gens:
        for _ in g:
            raise AssertionError("stream longer than announced")


def _merge(*streams):
    for j in _order([n for _, n in streams]):
        for _ in range(2):
            next(streams[j][0])
            yield
    _finish([g for g, _ in streams])


def _make_kernel(S, DM, H, DH, M, SEG, DC):
    NP = H // 2
    NSEG = S // SEG
    DP = 512
    KM = DM // 128 * 128
    HT = DH // 128
    PT = 6 * HT
    STEPS = NSEG // H
    QB = 128
    OB = DM // 4
    PVR = 8
    MBK, MBV = 64, 64
    GAPS = (2, 3, 2, 2)
    RB = 512
    OUT = 256
    XC = S // H
    GB = 2 * QB
    NG = S // GB
    AB = 2 * SEG
    QSC = LOG2E * DH ** -0.5

    def packed(*shape):
        return pltpu.VMEM(shape[:-2] + (shape[-2] // 2, shape[-1]), U32)

    def kernel(ax_h, mem_h, awq_h, awk_h, awv_h, awo_h, bx_h, ckv_h, bwq_h, bwk_h, bwv_h, bwo_h,
               out_h,
               ax, mem_s, awo, wqkv, wqkv_t, wo, wo_t, kx, vx, km, vm,
               bx, ckv, bwq, bwk, bwv, bwo, accb,
               sem_x, sem_aq, sem_ak, sem_av, sem_ao, sem_bq, sem_bk, sem_bv, sem_bo, sem_out):

        def pair_copy(src, dst, sem, i):
            return pltpu.make_async_copy(src.bitcast(U32).at[:, i, :], dst.at[i], sem.at[i])

        def wo_copy(src, dst, sem, i):
            return pltpu.make_async_copy(src.bitcast(U32).at[pl.ds(2 * i, 2)], dst.at[pl.ds(2 * i, 2)], sem.at[i])

        def head_weight(t):
            return _bf(jnp.concatenate(
                [jnp.concatenate([wqkv[t + j], wqkv_t[t // 2 + j // 2, _half((j % 2) * 64, 64), :]], axis=0)
                 for j in range(HT)], axis=1))

        def transposed(raw, c, n):
            xt = _bf(raw[:, pl.ds(c if isinstance(c, int) else pl.multiple_of(c, n), n)])
            return jnp.concatenate([xt, jnp.zeros((DP - DM, n), BF16)], axis=0).T

        def keep_terms(dst, g, x):
            for n, term in enumerate(_lhs_terms(x.astype(F32))):
                dst[n, _half(g * QB, QB), :] = _u32(term)

        def project_rows(src, g, terms):
            def product(n):
                x = _bf(src[n, _half(g * QB, QB), :])[:, :terms[n].shape[0]]
                return lambda: _dot(x, terms[n])
            return jnp.concatenate(_run(_block_product(product)), axis=0)

        def weight_terms(t):
            return [w.astype(BF16) for w in _rhs_terms(head_weight(t).astype(F32), DP // 2)]

        def phase1(xraw, craw, mem0, awq, awk, awv):
            def cp_ax(r):
                cols = pl.ds(r * RB if isinstance(r, int) else pl.multiple_of(r * RB, RB), RB)
                return pltpu.make_async_copy(ax_h.bitcast(U32).at[:, cols], xraw.at[:, cols], sem_x.at[3 + r])

            cp_mem = pltpu.make_async_copy(mem_h.at[0], mem0, sem_x.at[0])
            cp_bx = pltpu.make_async_copy(bx_h.bitcast(U32), xraw.at[:, pl.ds(S, S)], sem_x.at[1])
            cp_ckv = pltpu.make_async_copy(ckv_h.bitcast(U32).at[0], craw, sem_x.at[2])

            def a_weights(i):
                pair_copy(awk_h, awk, sem_ak, i).start()
                pair_copy(awv_h, awv, sem_av, i).start()
                pair_copy(awq_h, awq, sem_aq, i).start()
                wo_copy(awo_h, awo, sem_ao, i).start()

            def b_weights(i):
                pair_copy(bwq_h, bwq, sem_bq, i).start()
                pair_copy(bwk_h, bwk, sem_bk, i).start()
                pair_copy(bwv_h, bwv, sem_bv, i).start()
                wo_copy(bwo_h, bwo, sem_bo, i).start()

            for r in range(S // RB):
                cp_ax(r).start()
            a_weights(0)

            def keep(w, t):
                u = _u32(w)
                for j in range(HT):
                    wqkv[t + j] = u[:KM // 2, j * 128:(j + 1) * 128]
                    wqkv_t[t // 2 + j // 2, _half((j % 2) * 64, 64), :] = u[KM // 2:, j * 128:(j + 1) * 128]

            def keep_kv(h):
                i = h // 2
                keep(_unpack(awk[i], h % 2), PT * i + (2 + h % 2) * HT)
                keep(_unpack(awv[i], h % 2), PT * i + (4 + h % 2) * HT)

            @pl.loop(0, S // RB)
            def _(r):
                cp_ax(r).wait()
                for j in range(RB // GB):
                    g = r * (RB // GB) + j
                    keep_terms(ax, g, transposed(xraw, g * GB, GB))
            cp_bx.start()
            cp_mem.start()
            pl.loop(1, NP)(a_weights)
            cp_ckv.start()
            pl.loop(0, NP)(b_weights)
            pair_copy(awk_h, awk, sem_ak, 0).wait()
            pair_copy(awv_h, awv, sem_av, 0).wait()
            keep_kv(0)

            @pl.loop(0, H)
            def _(h):
                i = h // 2
                par = h % 2

                @pl.when(par == 0)
                def _():
                    pair_copy(awq_h, awq, sem_aq, i).wait()
                    wo_copy(awo_h, awo, sem_ao, i).wait()

                @pl.when((par == 1) & (i + 1 < NP))
                def _():
                    pair_copy(awk_h, awk, sem_ak, i + 1).wait()
                    pair_copy(awv_h, awv, sem_av, i + 1).wait()

                @pl.when(h == 1)
                def _():
                    cp_bx.wait()

                @pl.when(h == H - NG)
                def _():
                    cp_ckv.wait()

                @pl.when(h >= H - NG)
                def _():
                    g = h - (H - NG)
                    keep_terms(ckv, g, _bf(craw[_half(g * GB, GB), :]))
                wk, wv = weight_terms(PT * i + (2 + par) * HT), weight_terms(PT * i + (4 + par) * HT)
                for g in range(NG):
                    kx[h, _half(g * GB, GB), :] = _u32(project_rows(ax, g, wk))
                    vx[h, _half(g * GB, GB), :] = _u32(project_rows(ax, g, wv))
                    if g == 0:
                        w = _u32(jnp.concatenate([_bf(awo[h]), jnp.zeros((DP - DM, DH), BF16)], axis=0).T)
                        wo[_half(h * DH, DH), :] = w[:, :KM]
                        wo_t[_half(h * 128, 128), :] = w[:64, KM:] | pltpu.roll(w[64:, KM:], 64, 1)
                    if g == 1:
                        src = jnp.where(h == 0, NG - 1, NG + (h - 1) % NG)
                        keep_terms(bx, (h + NG - 1) % NG, transposed(xraw, src * GB, GB))
                    if g == 3:
                        keep(_unpack(awq[i], par), PT * i + par * HT)
                        accb[:, pl.ds(pl.multiple_of(h * XC, XC), XC)] = jnp.zeros((DM, XC), F32)
                    if g == 5:
                        keep_kv(jnp.minimum(h + 1, H - 1))
            cp_mem.wait()
            mem_s[...] = jnp.concatenate([mem0[...].astype(F32), jnp.zeros((M, DP - DM), F32)], axis=1)

        with jax.named_scope('phase1'):
            pl.run_scoped(phase1, packed(DM, 2 * S), packed(S, DC), pltpu.VMEM((M, DM), BF16),
                          *[pltpu.VMEM((NP, DM, DH), U32)] * 3)

        def chain_step(s, held):
            mem = mem_s[...]
            zero = s >> 10
            mt = mem[:, KM:]
            mtail = jnp.concatenate([mt, pltpu.roll(mt, 64, 1)], axis=0).astype(BF16)
            t = []
            for g in range(0, NP * PT, 8):
                for t0 in (g, g + 4):
                    acc = _zeros(s, (M, 512))
                    for k0 in range(0, KM, 128):
                        w = jnp.concatenate([wqkv[t0 + j + zero, _half(k0, 128), :] for j in range(4)], axis=1)
                        yield
                        acc = acc + _dot(mem[:, k0:k0 + 128], _bf(w))
                        yield
                    t += [acc[:, j * 128:(j + 1) * 128] for j in range(4)]
                w = jnp.concatenate([wqkv_t[g // 2 + j + zero] for j in range(4)], axis=1)
                yield
                d = _dot(mtail, _bf(w))
                for j in range(8):
                    t[g + j] = t[g + j] + d[(j % 2) * M:(j % 2 + 1) * M, (j // 2) * 128:(j // 2 + 1) * 128]
                yield
            for _ in range(2 * GAPS[0]):
                yield

            def head_rows(i, which, par):
                t0 = PT * i + (2 * which + par) * HT
                return jnp.concatenate(t[t0:t0 + HT], axis=1)

            def pair_rows(i, which):
                return jnp.concatenate([head_rows(i, which, 0), head_rows(i, which, 1)], axis=0)

            def window(ref, i, which):
                xr = _half(s * SEG, SEG)
                return jnp.concatenate([_bf(ref[2 * i, xr, :]), _bf(ref[2 * i + 1, xr, :]),
                                        pair_rows(i, which).astype(BF16)], axis=0)

            now = [[head_rows(h // 2, which, h % 2) for h in range(H)] for which in (1, 2)]
            if held:
                for ref, old, new in zip((km, vm), held.pop(), now):
                    for h in range(H):
                        ref[h, _half((s - 1) * M, 2 * M), :] = _u32(jnp.concatenate([old[h], new[h]], axis=0))
            else:
                held.append(now)
            sc = []
            for i0 in range(0, NP, 2):
                ops = [((pair_rows(i, 0) * QSC).astype(BF16), window(kx, i, 1)) for i in (i0, i0 + 1)]
                yield
                sc += [_dot_nt(q, k) for q, k in ops]
                yield
            for _ in range(2 * GAPS[1]):
                yield
            sc = jnp.concatenate(sc, axis=0)
            par = (jax.lax.broadcasted_iota(jnp.int32, sc.shape, 0) // M) % 2
            ci = jax.lax.broadcasted_iota(jnp.int32, sc.shape, 1)
            own = jnp.where(ci < 2 * SEG, ci // SEG, (ci - 2 * SEG) // M) == par
            p = _softmax2(jnp.where(own, sc, NEG))
            zt = []
            for i0 in range(0, NP, 2):
                ops = [(p[2 * M * i:2 * M * (i + 1)], window(vx, i, 2)) for i in (i0, i0 + 1)]
                yield
                for pp, v in ops:
                    o = _dot(pp, v)
                    zt += [o[par * M:(par + 1) * M, j * 128:(j + 1) * 128] for par in range(2) for j in range(HT)]
                yield
            for _ in range(2 * GAPS[2]):
                yield
            acc = [_zeros(s, (M, 128))] * 3 + [_zeros(s, (2 * M, 128))]
            for g in range(0, H * HT, 8):
                for t0 in (g, g + 4):
                    zp = jnp.concatenate(zt[t0:t0 + 4], axis=1).astype(BF16).astype(F32)
                    for n in range(KM // 128):
                        w = wo[_half((t0 + zero) * 128, 512), n * 128:(n + 1) * 128]
                        yield
                        acc[n] = acc[n] + _dot(zp, _bf(w))
                        yield
                zp = jnp.concatenate([jnp.concatenate(zt[g:g + 8:2], axis=1),
                                      jnp.concatenate(zt[g + 1:g + 8:2], axis=1)], axis=0).astype(BF16)
                w = wo_t[_half((g // 2 + zero) * 128, 512), :]
                yield
                acc[3] = acc[3] + _dot(zp, _bf(w))
                yield
            lane = jax.lax.broadcasted_iota(jnp.int32, (M, 128), 1)
            last = jnp.where(lane < 64, acc[3][:M] + pltpu.roll(acc[3][M:], 64, 1), 0.0)
            mem_s[...] = jnp.concatenate(acc[:3] + [last], axis=1).astype(BF16).astype(F32)
            for _ in range(2 * GAPS[3]):
                yield

        def chain(h):
            held = []
            for j in range(STEPS):
                yield from chain_step(h * STEPS + j, held)

        n_chain = STEPS * ((NP * PT + H * HT) // 8 * 7 + NP + sum(GAPS))
        n_qk, n_v = 7 * (1 + QB // MBK), 7 * (QB // MBV)

        def split(r):
            return 2 if r >= PVR else 1

        def n_scores(r):
            return (r + 2) // 2

        def n_context(r):
            return (r + 1) // 2 * split(r) + (r + 1) % 2

        n_head = (NG * (n_qk + n_v) + (S // QB // 2) * (DM // OB) - (S // QB // 2 - 1)
                  + sum(n_scores(r) + n_context(r) for r in range(S // QB)))

        def phase2(wq_s, wk_s, wv_s, k_s, v_s):
            def b_head(h):
                i = h // 2
                par = h % 2
                for w_s, raw in ((wq_s, bwq), (wk_s, bwk), (wv_s, bwv)):
                    for n, term in enumerate(_rhs_terms(_unpack(raw[i], par), 2 * w_s.shape[1])):
                        w_s[n, _half(0, term.shape[0]), :] = _u32(term)
                qs, ss, ms, ctxs = {}, {}, {}, {}

                def chunks(r):
                    nk = (r + 1) * QB
                    return [(c0, min(c0 + 256, nk)) for c0 in range(0, nk, 256)]

                def project(g, src, w_s, depth, mb, together):
                    parts = []
                    for r0 in range(g * QB, (g + 1) * QB, mb * together):
                        def product(n):
                            k = depth - 2 * w_s.shape[1] if n in (4, 5) else 2 * w_s.shape[1]
                            xs = [_bf(src[n, _half(r0 + j * mb, mb), :])[:, :k] for j in range(together)]
                            w = _bf(w_s[n, _half(0, k), :])
                            return lambda: jnp.concatenate([_dot(x, w) for x in xs], axis=0)
                        if parts:
                            yield
                        parts.append((yield from _block_product(product)))
                    return [jnp.concatenate(half, axis=0) for half in zip(*parts)]

                def project_qk(g):
                    top, bottom = yield from project(g, bx, wq_s, DM, QB // 2, 2)
                    qs[2 * g], qs[2 * g + 1] = (top * QSC).astype(BF16), (bottom * QSC).astype(BF16)
                    yield
                    top, bottom = yield from project(g, ckv, wk_s, DC, MBK, 1)
                    k_s[2 * g][...], k_s[2 * g + 1][...] = _u32(top), _u32(bottom)
                    yield

                def project_v(g):
                    top, bottom = yield from project(g, ckv, wv_s, DC, MBV, 1)
                    v_s[2 * g][...], v_s[2 * g + 1][...] = _u32(top), _u32(bottom)
                    yield

                def blocks(refs, c0, c1):
                    return _bf(jnp.concatenate([refs[j][...] for j in range(c0 // QB, c1 // QB)], axis=0))

                def scores(r):
                    ss[r] = []
                    m = None
                    for c0, c1 in chunks(r):
                        k = blocks(k_s, c0, c1)
                        yield
                        sc = _dot_nt(qs[r], k)
                        if c1 == (r + 1) * QB:
                            ri = jax.lax.broadcasted_iota(jnp.int32, sc.shape, 0) + r * QB
                            ci = jax.lax.broadcasted_iota(jnp.int32, sc.shape, 1) + c0
                            sc = jnp.where(ci <= ri, sc, NEG)
                        ss[r].append(sc)
                        for t0 in range(0, c1 - c0, 128):
                            m = sc[:, t0:t0 + 128] if m is None else jnp.maximum(m, sc[:, t0:t0 + 128])
                        if c1 == (r + 1) * QB:
                            ms[r] = jnp.max(m, axis=1, keepdims=True)
                        yield

                def context(r):
                    ls = []

                    def weights(c):
                        p = jnp.exp2(ss[r][c] - ms[r])
                        for t0 in range(0, p.shape[1], 128):
                            ls[:] = [p[:, t0:t0 + 128] + ls[0] if ls else p[:, t0:t0 + 128]]
                        return p.astype(BF16)

                    acc = _zeros(h, (QB, DH))
                    nxt = weights(0)
                    for c, (c0, c1) in enumerate(chunks(r)):
                        mb = QB // split(r) if c1 - c0 == 256 else QB
                        p = nxt
                        v = blocks(v_s, c0, c1)
                        new = []
                        for r0 in range(0, QB, mb):
                            yield
                            new.append(acc[r0:r0 + mb] + _dot(p[r0:r0 + mb], v))
                            if r0 == 0 and c1 < (r + 1) * QB:
                                nxt = weights(c + 1)
                            if r0 + mb == QB:
                                acc = jnp.concatenate(new, axis=0)
                                if c1 == (r + 1) * QB:
                                    ctxs[r] = (acc / jnp.sum(ls[0], axis=1, keepdims=True)).astype(BF16)
                            yield

                def output(r):
                    ctx = jnp.concatenate([ctxs[r - 1], ctxs[r]], axis=0)
                    cols = pl.ds((r - 1) * QB, 2 * QB)
                    for n0 in range(0, DM, OB):
                        w = _bf(bwo[h, _half(n0, OB), :])
                        yield
                        accb[n0:n0 + OB, cols] += _dot_nt(w, ctx)
                        yield

                def both(r):
                    a, b = scores(r), context(r - 2)
                    na, nc = n_scores(r) - 1, n_context(r - 2) - 1
                    for j in _order([na, nc]):
                        for _ in range(2):
                            next((a, b)[j])
                            yield
                    for _ in range(2):
                        next(a)
                        next(b)
                        yield
                    _finish([a, b])

                nb = S // QB
                for r in range(nb + 4):
                    parts = []
                    if r < nb:
                        parts.append((project_v(r // 2), n_v) if r % 2 else (project_qk(r // 2), n_qk))
                    if 0 <= r - 4 < nb and (r - 4) % 2 == 1:
                        parts.append((output(r - 4), DM // OB))
                    if r % 2 == 1 and 3 <= r <= nb:
                        parts.append((both(r - 1), n_scores(r - 1) + n_context(r - 3) - 1))
                    else:
                        if 0 <= r - 1 < nb:
                            parts.append((scores(r - 1), n_scores(r - 1)))
                        if 0 <= r - 3 < nb:
                            parts.append((context(r - 3), n_context(r - 3)))
                    yield from _merge(*parts)

            def b_body(h, c):
                i = h // 2

                @pl.when(h % 2 == 0)
                def _():
                    pair_copy(bwq_h, bwq, sem_bq, i).wait()
                    pair_copy(bwk_h, bwk, sem_bk, i).wait()
                    pair_copy(bwv_h, bwv, sem_bv, i).wait()
                    wo_copy(bwo_h, bwo, sem_bo, i).wait()
                for _ in _merge((chain(h), n_chain), (b_head(h), n_head)):
                    pass
                return c
            jax.lax.fori_loop(0, H, b_body, 0)

        with jax.named_scope('phase2'):
            pl.run_scoped(phase2, packed(7, DP // 2, DH // 2), packed(7, DC // 2, DH // 2), packed(7, DC // 2, DH // 2), [packed(QB, DH)] * (S // QB), [packed(QB, DH)] * (S // QB))

        def phase3(acca, ostage, q0):
            ri = jax.lax.broadcasted_iota(jnp.int32, (AB, AB + 2 * M), 0)
            ci = jax.lax.broadcasted_iota(jnp.int32, (AB, AB + 2 * M), 1)
            amask = (((ci < AB) & ((ci // SEG) == (ri // SEG)) & (ci <= ri))
                     | ((ci >= AB) & (((ci - AB) // M) == (ri // SEG))))

            def out_copy(r):
                rows = _half(r * OUT, OUT)
                return pltpu.make_async_copy(ostage.at[rows, :], out_h.bitcast(U32).at[0, rows, :], sem_out.at[r])

            def query_weight(h):
                return weight_terms(PT * (h // 2) + (h % 2) * HT)

            def query(wq, r):
                groups = range(r * RB // GB, (r + 1) * RB // GB)
                return (jnp.concatenate([project_rows(ax, g, wq) for g in groups], axis=0) * QSC).astype(BF16)

            def a_head(h):
                wq = query_weight(h)
                qs, ps, ctxs = {0: _bf(q0[...])}, {}, {}

                def project(r):
                    qs[r] = query(wq, r)

                def window(xref, mref, j):
                    return _bf(jnp.concatenate([xref[h, _half(j * AB, AB), :],
                                                mref[h, _half(j * 2 * M, 2 * M), :]], axis=0))

                def scores(r):
                    ps[r] = []
                    for j in range(RB // AB):
                        sc = _dot_nt(qs[r][j * AB:(j + 1) * AB], window(kx, km, r * RB // AB + j))
                        ps[r].append(_softmax2(jnp.where(amask, sc, NEG)))

                def context(r):
                    ctxs[r] = jnp.concatenate(
                        [_dot(p, window(vx, vm, r * RB // AB + j)).astype(BF16) for j, p in enumerate(ps[r])],
                        axis=0)

                def output(r, c0, c1):
                    cols = slice(r * RB + c0, r * RB + c1)
                    acca[:, cols] = jnp.where(h > 0, acca[:, cols], 0.0) + _dot_nt(_bf(awo[h]), ctxs[r][c0:c1])

                nr = S // RB
                project(1)
                for r in range(nr):
                    scores(r)
                    if r > 0:
                        output(r - 1, 0, RB)
                    if r + 2 < nr:
                        project(r + 2)
                    context(r)
                q0[...] = _u32(query(query_weight(jnp.minimum(h + 1, H - 1)), 0))
                output(nr - 1, 0, RB)

            q0[...] = _u32(query(query_weight(0), 0))
            pl.loop(0, H)(a_head)

            @pl.loop(0, S // OUT)
            def _(r):
                cols = pl.ds(pl.multiple_of(r * OUT, OUT), OUT)
                ostage[_half(r * OUT, OUT), :] = _u32(
                    jnp.concatenate([acca[:, cols], accb[:, cols]], axis=0).astype(BF16).T)
                out_copy(r).start()

            @pl.loop(0, S // OUT)
            def _(r):
                out_copy(r).wait()

        with jax.named_scope('phase3'):
            pl.run_scoped(phase3, pltpu.VMEM((DM, S), F32), packed(S, 2 * DM), packed(RB, DH))

    scratch = [
        packed(7, S // 2, DP // 2),
        pltpu.VMEM((M, DP), F32),
        packed(H, DM, DH),
        packed(NP * PT, KM, 128),
        packed(NP * PT // 2, 128, 128),
        packed(H * DH, KM),
        packed(H * DH // 2, 128),
        packed(H, S, DH),
        packed(H, S, DH),
        packed(H, NSEG * M, DH),
        packed(H, NSEG * M, DH),
        packed(7, S // 2, DP // 2),
        packed(7, S // 2, DC // 2),
        pltpu.VMEM((NP, DM, DH), U32),
        pltpu.VMEM((NP, DC, DH), U32),
        pltpu.VMEM((NP, DC, DH), U32),
        packed(H, DM, DH),
        pltpu.VMEM((DM, S), F32),
        pltpu.SemaphoreType.DMA((3 + S // RB,)),
    ] + [pltpu.SemaphoreType.DMA((NP,)) for _ in range(8)] + [pltpu.SemaphoreType.DMA((S // OUT,))]
    return kernel, scratch


@jax.jit
def pallas_concat_heads__memory_aug_recurrent_mem_tr__compressed_kv_cla__prompt_kernel(
    A_x, A_mem0, A_Wq, A_Wk, A_Wv, A_Wo, A_seg_len, B_x, B_c_kv, B_w_q, B_w_uk, B_w_uv, B_w_o,
):
    del A_seg_len
    _, S, DM = A_x.shape
    M = A_mem0.shape[1]
    H, DH = A_Wq.shape[1], A_Wq.shape[2]
    DC = B_c_kv.shape[2]
    kernel, scratch = _make_kernel(S, DM, H, DH, M, 32, DC)
    return pl.pallas_call(
        kernel,
        out_shape=jax.ShapeDtypeStruct((1, S, 2 * DM), BF16),
        in_specs=[pl.BlockSpec(memory_space=pl.ANY)] * 12,
        out_specs=pl.BlockSpec(memory_space=pl.ANY),
        scratch_shapes=scratch,
        compiler_params=pltpu.CompilerParams(vmem_limit_bytes=126 * 1024 * 1024),
    )(A_x[0].T, A_mem0, A_Wq, A_Wk, A_Wv, A_Wo.transpose(0, 2, 1),
      B_x[0].T, B_c_kv, B_w_q, B_w_uk, B_w_uv, B_w_o.transpose(0, 2, 1))
```

```python
import jax
import jax.numpy as jnp
import jax.experimental.pallas as pl
import jax.experimental.pallas.tpu as pltpu

F32 = jnp.float32
BF16 = jnp.bfloat16
U32 = jnp.uint32
LOG2E = 1.4426950408889634
NEG = -1e30
NN = (((1,), (0,)), ((), ()))
NT = (((1,), (1,)), ((), ()))


def _dot(a, b):
    return jax.lax.dot_general(a, b, NN, preferred_element_type=F32)


def _dot_nt(a, b):
    return jax.lax.dot_general(a, b, NT, preferred_element_type=F32)


def _bf(u):
    return pltpu.bitcast(u, BF16)


def _u32(x):
    return pltpu.bitcast(x.astype(BF16), U32)


def _half(start, size):
    if isinstance(start, int):
        return pl.ds(start // 2, size // 2)
    return pl.ds(pl.multiple_of(start // 2, 8), size // 2)


def _unpack(u, parity):
    if isinstance(parity, int):
        w = (u << 16) if parity == 0 else (u & jnp.uint32(0xFFFF0000))
    else:
        w = (u >> (16 * parity).astype(U32)) << 16
    return pltpu.bitcast(w, F32)


def _lhs_terms(x):
    r, k = x.shape[0] // 2, x.shape[1] // 2
    x11, x12, x21, x22 = x[:r, :k], x[:r, k:], x[r:, :k], x[r:, k:]
    return [x11 + x22, x22, x21 + x22, x11, x11 + x12, x12 - x22, x21 - x11]


def _rhs_terms(w, k):
    n, k2 = w.shape[1] // 2, w.shape[0] - k
    w11, w12, w21, w22 = w[:k, :n], w[:k, n:], w[k:, :n], w[k:, n:]

    def full(a):
        return a if k2 == k else jnp.concatenate([a, jnp.zeros((k - k2, n), a.dtype)], axis=0)
    return [w11 + full(w22), full(w21) - w11, w11, w12 - full(w22), w22, w21 + w22, w11 + w12]


_STRASSEN = (
    ((1, 0, 0), (1, 1, 1)), ((1, 0, 0), (1, 1, 0)), ((1, 1, 0), (-1, 1, 1)), ((1, 0, 1), (1, 1, 1)),
    ((1, 0, 1), (-1, 0, 0)), ((1, 0, 0),), ((1, 1, 1),))


def _block_product(product, finish, start=None):
    c = {}
    for n, uses in enumerate(_STRASSEN):
        multiply = product(n)
        yield
        p = multiply()
        for sign, a, b in uses:
            if start and (a, b) not in c:
                c[a, b] = start(a, b)
            c[a, b] = p if (a, b) not in c else c[a, b] + p if sign > 0 else c[a, b] - p
            if all((a, b) != use[1:] for later in _STRASSEN[n + 1:] for use in later):
                finish(a, b, c[a, b])
        yield


def _rhs_terms_t(wt):
    n, k = wt.shape[0] // 2, wt.shape[1] // 2
    w11, w12, w21, w22 = wt[:n, :k], wt[n:, :k], wt[:n, k:], wt[n:, k:]
    return [w11 + w22, w21 - w11, w11, w12 - w22, w22, w21 + w22, w11 + w12]


def _zeros(i, shape):
    return jnp.full(shape, (i >> 10).astype(F32))


def _softmax2(sc):
    p = jnp.exp2(sc - jnp.max(sc, axis=1, keepdims=True))
    return (p / jnp.sum(p, axis=1, keepdims=True)).astype(BF16)


def _order(counts):
    done = [0] * len(counts)
    live = [a for a, n in enumerate(counts) if n > 0]
    order = []
    for _ in range(sum(counts)):
        j = min(live, key=lambda a: ((done[a] + 0.5) / counts[a], a))
        done[j] += 1
        order.append(j)
    return order


def _finish(gens):
    for g in gens:
        for _ in g:
            raise AssertionError("stream longer than announced")


def _merge(*streams):
    for j in _order([n for _, n in streams]):
        for _ in range(2):
            next(streams[j][0])
            yield
    _finish([g for g, _ in streams])


def _make_kernel(S, DM, H, DH, M, SEG, DC):
    NP = H // 2
    NSEG = S // SEG
    DP = 512
    KM = DM // 128 * 128
    HT = DH // 128
    PT = 6 * HT
    STEPS = NSEG // H
    QB = 128
    PVR = 4
    MBK, MBV = 64, 64
    GAPS = (1, 2, 1, 2)
    RB = 512
    OUT = 256
    XC = S // H
    GB = 2 * QB
    NG = S // GB
    AB = 2 * SEG
    QSC = LOG2E * DH ** -0.5

    def packed(*shape):
        return pltpu.VMEM(shape[:-2] + (shape[-2] // 2, shape[-1]), U32)

    def kernel(ax_h, mem_h, awq_h, awk_h, awv_h, awo_h, bx_h, ckv_h, bwq_h, bwk_h, bwv_h, bwo_h,
               out_h,
               ax, mem_s, awo, wqkv, wqkv_t, wo, wo_t, kx, vx, km, vm,
               bx, ckv, bwq, bwk, bwv, bwo, accb,
               sem_x, sem_aq, sem_ak, sem_av, sem_ao, sem_bq, sem_bk, sem_bv, sem_bo, sem_out):

        def pair_copy(src, dst, sem, i):
            return pltpu.make_async_copy(src.bitcast(U32).at[:, i, :], dst.at[i], sem.at[i])

        def wo_copy(src, dst, sem, i):
            return pltpu.make_async_copy(src.bitcast(U32).at[pl.ds(2 * i, 2)], dst.at[pl.ds(2 * i, 2)], sem.at[i])

        def head_weight(t):
            return _bf(jnp.concatenate(
                [jnp.concatenate([wqkv[t + j], wqkv_t[t // 2 + j // 2, _half((j % 2) * 64, 64), :]], axis=0)
                 for j in range(HT)], axis=1))

        def transposed(raw, c, n):
            xt = _bf(raw[:, pl.ds(c if isinstance(c, int) else pl.multiple_of(c, n), n)])
            return jnp.concatenate([xt, jnp.zeros((DP - DM, n), BF16)], axis=0).T

        def keep_terms(dst, g, x):
            for n, term in enumerate(_lhs_terms(x.astype(F32))):
                dst[n, _half(g * QB, QB), :] = _u32(term)

        def project_rows(g, terms, finish):
            def product(n):
                x = _bf(ax[n, _half(g * QB, QB), :])[:, :terms[n].shape[0]]
                return lambda: _dot(x, terms[n])
            for _ in _block_product(product, finish):
                pass

        def store_blocks(top, bottom, row):
            def finish(a, b, c):
                (top, bottom)[a][_half(row, c.shape[0]), b * 128:(b + 1) * 128] = _u32(c)
            return finish

        def query_blocks(blocks):
            def finish(a, b, c):
                blocks[a, b] = (c * QSC).astype(BF16)
            return finish

        def add_output(acc, col, wt, ctx, parts, keep=None):
            half = DM // 2

            def product(n):
                ws = [wt(n, r, half // parts) for r in range(0, half, half // parts)]
                return lambda: jnp.concatenate(
                    [jnp.concatenate([_dot_nt(w, c[n]) for w in ws], axis=0) for c in ctx], axis=1)

            def where(a, b, j):
                return slice(a * half, (a + 1) * half), slice(col + j * GB + b * QB, col + j * GB + (b + 1) * QB)

            def start(a, b):
                old = jnp.concatenate([acc[where(a, b, j)] for j in range(2)], axis=1)
                return old if keep is None else jnp.where(keep, old, 0.0)

            def finish(a, b, c):
                for j in range(2):
                    acc[where(a, b, j)] = c[:, j * QB:(j + 1) * QB]
            return _block_product(product, finish, start)

        def context_terms(ctx):
            return [t.astype(BF16) for t in _rhs_terms_t(ctx)]

        def weight_terms(t):
            return [w.astype(BF16) for w in _rhs_terms(head_weight(t).astype(F32), DP // 2)]

        def phase1(xraw, craw, mem0, awq, awk, awv):
            def cp_ax(r):
                cols = pl.ds(r * RB if isinstance(r, int) else pl.multiple_of(r * RB, RB), RB)
                return pltpu.make_async_copy(ax_h.bitcast(U32).at[:, cols], xraw.at[:, cols], sem_x.at[3 + r])

            cp_mem = pltpu.make_async_copy(mem_h.at[0], mem0, sem_x.at[0])
            cp_bx = pltpu.make_async_copy(bx_h.bitcast(U32), xraw.at[:, pl.ds(S, S)], sem_x.at[1])
            cp_ckv = pltpu.make_async_copy(ckv_h.bitcast(U32).at[0], craw, sem_x.at[2])

            def a_weights(i):
                pair_copy(awk_h, awk, sem_ak, i).start()
                pair_copy(awv_h, awv, sem_av, i).start()
                pair_copy(awq_h, awq, sem_aq, i).start()
                wo_copy(awo_h, awo, sem_ao, i).start()

            def b_weights(i):
                pair_copy(bwq_h, bwq, sem_bq, i).start()
                pair_copy(bwk_h, bwk, sem_bk, i).start()
                pair_copy(bwv_h, bwv, sem_bv, i).start()
                wo_copy(bwo_h, bwo, sem_bo, i).start()

            for r in range(S // RB):
                cp_ax(r).start()
            a_weights(0)

            def keep(w, t):
                u = _u32(w)
                for j in range(HT):
                    wqkv[t + j] = u[:KM // 2, j * 128:(j + 1) * 128]
                    wqkv_t[t // 2 + j // 2, _half((j % 2) * 64, 64), :] = u[KM // 2:, j * 128:(j + 1) * 128]

            def keep_kv(h):
                i = h // 2
                keep(_unpack(awk[i], h % 2), PT * i + (2 + h % 2) * HT)
                keep(_unpack(awv[i], h % 2), PT * i + (4 + h % 2) * HT)

            @pl.loop(0, S // RB)
            def _(r):
                cp_ax(r).wait()
                for j in range(RB // GB):
                    g = r * (RB // GB) + j
                    keep_terms(ax, g, transposed(xraw, g * GB, GB))
            cp_bx.start()
            cp_mem.start()
            pl.loop(1, NP)(a_weights)
            cp_ckv.start()
            pl.loop(0, NP)(b_weights)
            pair_copy(awk_h, awk, sem_ak, 0).wait()
            pair_copy(awv_h, awv, sem_av, 0).wait()
            keep_kv(0)

            @pl.loop(0, H)
            def _(h):
                i = h // 2
                par = h % 2

                @pl.when(par == 0)
                def _():
                    pair_copy(awq_h, awq, sem_aq, i).wait()
                    wo_copy(awo_h, awo, sem_ao, i).wait()

                @pl.when((par == 1) & (i + 1 < NP))
                def _():
                    pair_copy(awk_h, awk, sem_ak, i + 1).wait()
                    pair_copy(awv_h, awv, sem_av, i + 1).wait()

                @pl.when(h == 1)
                def _():
                    cp_bx.wait()

                @pl.when(h == H - NG)
                def _():
                    cp_ckv.wait()

                @pl.when(h >= H - NG)
                def _():
                    g = h - (H - NG)
                    keep_terms(ckv, g, _bf(craw[_half(g * GB, GB), :]))
                wk, wv = weight_terms(PT * i + (2 + par) * HT), weight_terms(PT * i + (4 + par) * HT)
                for g in range(NG):
                    for dst, terms in ((kx, wk), (vx, wv)):
                        halves = [dst.at[h, _half(g * GB + a * QB, QB)] for a in range(2)]
                        project_rows(g, terms, store_blocks(*halves, 0))
                    if g == 0:
                        w = _u32(jnp.concatenate([_bf(awo[h]), jnp.zeros((DP - DM, DH), BF16)], axis=0).T)
                        wo[_half(h * DH, DH), :] = w[:, :KM]
                        wo_t[_half(h * 128, 128), :] = w[:64, KM:] | pltpu.roll(w[64:, KM:], 64, 1)
                    if g == 1:
                        src = jnp.where(h == 0, NG - 1, NG + (h - 1) % NG)
                        keep_terms(bx, (h + NG - 1) % NG, transposed(xraw, src * GB, GB))
                    if g == 3:
                        keep(_unpack(awq[i], par), PT * i + par * HT)
                        accb[:, pl.ds(pl.multiple_of(h * XC, XC), XC)] = jnp.zeros((DM, XC), F32)
                    if g == 5:
                        keep_kv(jnp.minimum(h + 1, H - 1))
            cp_mem.wait()
            mem_s[...] = jnp.concatenate([mem0[...].astype(F32), jnp.zeros((M, DP - DM), F32)], axis=1)

        with jax.named_scope('phase1'):
            pl.run_scoped(phase1, packed(DM, 2 * S), packed(S, DC), pltpu.VMEM((M, DM), BF16),
                          *[pltpu.VMEM((NP, DM, DH), U32)] * 3)

        def chain_step(s, held):
            mem = mem_s[...]
            zero = s >> 10
            mt = mem[:, KM:]
            mtail = jnp.concatenate([mt, pltpu.roll(mt, 64, 1)], axis=0).astype(BF16)
            t = []
            for g in range(0, NP * PT, 8):
                for t0 in (g, g + 4):
                    acc = _zeros(s, (M, 512))
                    for k0 in range(0, KM, 128):
                        w = jnp.concatenate([wqkv[t0 + j + zero, _half(k0, 128), :] for j in range(4)], axis=1)
                        yield
                        acc = acc + _dot(mem[:, k0:k0 + 128], _bf(w))
                        yield
                    t += [acc[:, j * 128:(j + 1) * 128] for j in range(4)]
                w = jnp.concatenate([wqkv_t[g // 2 + j + zero] for j in range(4)], axis=1)
                yield
                d = _dot(mtail, _bf(w))
                for j in range(8):
                    t[g + j] = t[g + j] + d[(j % 2) * M:(j % 2 + 1) * M, (j // 2) * 128:(j // 2 + 1) * 128]
                yield
            for _ in range(2 * GAPS[0]):
                yield

            def head_rows(i, which, par):
                t0 = PT * i + (2 * which + par) * HT
                return jnp.concatenate(t[t0:t0 + HT], axis=1)

            def pair_rows(i, which):
                return jnp.concatenate([head_rows(i, which, 0), head_rows(i, which, 1)], axis=0)

            def window(ref, i, which):
                xr = _half(s * SEG, SEG)
                return jnp.concatenate([_bf(ref[2 * i, xr, :]), _bf(ref[2 * i + 1, xr, :]),
                                        pair_rows(i, which).astype(BF16)], axis=0)

            now = [[head_rows(h // 2, which, h % 2) for h in range(H)] for which in (1, 2)]
            if held:
                for ref, old, new in zip((km, vm), held.pop(), now):
                    for h in range(H):
                        ref[h, _half((s - 1) * M, 2 * M), :] = _u32(jnp.concatenate([old[h], new[h]], axis=0))
            else:
                held.append(now)
            sc = []
            for i0 in range(0, NP, 2):
                ops = [((pair_rows(i, 0) * QSC).astype(BF16), window(kx, i, 1)) for i in (i0, i0 + 1)]
                yield
                sc += [_dot_nt(q, k) for q, k in ops]
                yield
            for _ in range(2 * GAPS[1]):
                yield
            sc = jnp.concatenate(sc, axis=0)
            par = (jax.lax.broadcasted_iota(jnp.int32, sc.shape, 0) // M) % 2
            ci = jax.lax.broadcasted_iota(jnp.int32, sc.shape, 1)
            own = jnp.where(ci < 2 * SEG, ci // SEG, (ci - 2 * SEG) // M) == par
            p = _softmax2(jnp.where(own, sc, NEG))
            zt = []
            for i0 in range(0, NP, 2):
                ops = [(p[2 * M * i:2 * M * (i + 1)], window(vx, i, 2)) for i in (i0, i0 + 1)]
                yield
                for pp, v in ops:
                    o = _dot(pp, v)
                    zt += [o[par * M:(par + 1) * M, j * 128:(j + 1) * 128] for par in range(2) for j in range(HT)]
                yield
            for _ in range(2 * GAPS[2]):
                yield
            acc = [_zeros(s, (M, 128))] * 3 + [_zeros(s, (2 * M, 128))]
            for g in range(0, H * HT, 8):
                for t0 in (g, g + 4):
                    zp = jnp.concatenate(zt[t0:t0 + 4], axis=1).astype(BF16).astype(F32)
                    for n in range(KM // 128):
                        w = wo[_half((t0 + zero) * 128, 512), n * 128:(n + 1) * 128]
                        yield
                        acc[n] = acc[n] + _dot(zp, _bf(w))
                        yield
                zp = jnp.concatenate([jnp.concatenate(zt[g:g + 8:2], axis=1),
                                      jnp.concatenate(zt[g + 1:g + 8:2], axis=1)], axis=0).astype(BF16)
                w = wo_t[_half((g // 2 + zero) * 128, 512), :]
                yield
                acc[3] = acc[3] + _dot(zp, _bf(w))
                yield
            lane = jax.lax.broadcasted_iota(jnp.int32, (M, 128), 1)
            last = jnp.where(lane < 64, acc[3][:M] + pltpu.roll(acc[3][M:], 64, 1), 0.0)
            mem_s[...] = jnp.concatenate(acc[:3] + [last], axis=1).astype(BF16).astype(F32)
            for _ in range(2 * GAPS[3]):
                yield

        def chain(h):
            held = []
            for j in range(STEPS):
                yield from chain_step(h * STEPS + j, held)

        n_chain = STEPS * ((NP * PT + H * HT) // 8 * 7 + NP + sum(GAPS))
        n_qk, n_v = 7 * (1 + QB // MBK), 7 * (QB // MBV)

        def split(r):
            return 2 if r >= PVR else 1

        def n_scores(r):
            return (r + 2) // 2

        def n_context(r):
            return (r + 1) // 2 * split(r) + (r + 1) % 2

        n_head = (NG * (n_qk + n_v) + (NG // 2) * 7 - (S // QB // 2 - 1)
                  + sum(n_scores(r) + n_context(r) for r in range(S // QB)))

        def phase2(wq_s, wk_s, wv_s, wo_s, k_s, v_s):
            def b_head(h):
                i = h // 2
                par = h % 2
                for w_s, raw in ((wq_s, bwq), (wk_s, bwk), (wv_s, bwv)):
                    for n, term in enumerate(_rhs_terms(_unpack(raw[i], par), 2 * w_s.shape[1])):
                        w_s[n, _half(0, term.shape[0]), :] = _u32(term)
                for n, term in enumerate(_lhs_terms(_bf(bwo[h]).astype(F32))):
                    wo_s[n] = _u32(term)
                qs, ss, ms, ctxs = {}, {}, {}, {}

                def chunks(r):
                    nk = (r + 1) * QB
                    return [(c0, min(c0 + 256, nk)) for c0 in range(0, nk, 256)]

                def project(g, r0, src, w_s, depth, mb, together, finish):
                    def product(n):
                        k = depth - 2 * w_s.shape[1] if n in (4, 5) else 2 * w_s.shape[1]
                        xs = [_bf(src[n, _half(g * QB + r0 + j * mb, mb), :])[:, :k] for j in range(together)]
                        w = _bf(w_s[n, _half(0, k), :])
                        return lambda: jnp.concatenate([_dot(x, w) for x in xs], axis=0)
                    return _block_product(product, finish)

                def project_qk(g):
                    q = {}
                    yield from project(g, 0, bx, wq_s, DM, QB // 2, 2, query_blocks(q))
                    for a in range(2):
                        qs[2 * g + a] = jnp.concatenate([q[a, 0], q[a, 1]], axis=1)
                    for r0 in range(0, QB, MBK):
                        yield from project(g, r0, ckv, wk_s, DC, MBK, 1, store_blocks(*k_s[2 * g:2 * g + 2], r0))

                def project_v(g):
                    for r0 in range(0, QB, MBV):
                        yield from project(g, r0, ckv, wv_s, DC, MBV, 1, store_blocks(*v_s[2 * g:2 * g + 2], r0))

                def blocks(refs, c0, c1):
                    return _bf(jnp.concatenate([refs[j][...] for j in range(c0 // QB, c1 // QB)], axis=0))

                def scores(r):
                    ss[r] = []
                    m = None
                    for c0, c1 in chunks(r):
                        k = blocks(k_s, c0, c1)
                        yield
                        sc = _dot_nt(qs[r], k)
                        if c1 == (r + 1) * QB:
                            ri = jax.lax.broadcasted_iota(jnp.int32, sc.shape, 0) + r * QB
                            ci = jax.lax.broadcasted_iota(jnp.int32, sc.shape, 1) + c0
                            sc = jnp.where(ci <= ri, sc, NEG)
                        ss[r].append(sc)
                        for t0 in range(0, c1 - c0, 128):
                            m = sc[:, t0:t0 + 128] if m is None else jnp.maximum(m, sc[:, t0:t0 + 128])
                        if c1 == (r + 1) * QB:
                            ms[r] = jnp.max(m, axis=1, keepdims=True)
                        yield

                def context(r):
                    ls = []

                    def weights(c):
                        p = jnp.exp2(ss[r][c] - ms[r])
                        for t0 in range(0, p.shape[1], 128):
                            ls[:] = [p[:, t0:t0 + 128] + ls[0] if ls else p[:, t0:t0 + 128]]
                        return p.astype(BF16)

                    acc = _zeros(h, (QB, DH))
                    nxt = weights(0)
                    for c, (c0, c1) in enumerate(chunks(r)):
                        mb = QB // split(r) if c1 - c0 == 256 else QB
                        p = nxt
                        v = blocks(v_s, c0, c1)
                        new = []
                        for r0 in range(0, QB, mb):
                            yield
                            new.append(acc[r0:r0 + mb] + _dot(p[r0:r0 + mb], v))
                            if r0 == 0 and c1 < (r + 1) * QB:
                                nxt = weights(c + 1)
                            if r0 + mb == QB:
                                acc = jnp.concatenate(new, axis=0)
                                if c1 == (r + 1) * QB:
                                    ctxs[r] = acc / jnp.sum(ls[0], axis=1, keepdims=True)
                                    if r % 2:
                                        ctxs[r] = context_terms(jnp.concatenate([ctxs[r - 1], ctxs[r]], axis=0))
                            yield

                def output(r):
                    yield from add_output(accb, (r - 3) * QB, lambda n, r0, m: _bf(wo_s[n, _half(r0, m), :]),
                                          (ctxs[r - 2], ctxs[r]), 2)

                def both(r):
                    a, b = scores(r), context(r - 2)
                    na, nc = n_scores(r) - 1, n_context(r - 2) - 1
                    for j in _order([na, nc]):
                        for _ in range(2):
                            next((a, b)[j])
                            yield
                    for _ in range(2):
                        next(a)
                        next(b)
                        yield
                    _finish([a, b])

                nb = S // QB
                for r in range(nb + 4):
                    parts = []
                    if r < nb:
                        parts.append((project_v(r // 2), n_v) if r % 2 else (project_qk(r // 2), n_qk))
                    if 0 <= r - 4 < nb and (r - 4) % 4 == 3:
                        parts.append((output(r - 4), 7))
                    if r % 2 == 1 and 3 <= r <= nb:
                        parts.append((both(r - 1), n_scores(r - 1) + n_context(r - 3) - 1))
                    else:
                        if 0 <= r - 1 < nb:
                            parts.append((scores(r - 1), n_scores(r - 1)))
                        if 0 <= r - 3 < nb:
                            parts.append((context(r - 3), n_context(r - 3)))
                    yield from _merge(*parts)

            def b_body(h, c):
                i = h // 2

                @pl.when(h % 2 == 0)
                def _():
                    pair_copy(bwq_h, bwq, sem_bq, i).wait()
                    pair_copy(bwk_h, bwk, sem_bk, i).wait()
                    pair_copy(bwv_h, bwv, sem_bv, i).wait()
                    wo_copy(bwo_h, bwo, sem_bo, i).wait()
                for _ in _merge((chain(h), n_chain), (b_head(h), n_head)):
                    pass
                return c
            jax.lax.fori_loop(0, H, b_body, 0)

        with jax.named_scope('phase2'):
            pl.run_scoped(phase2, packed(7, DP // 2, DH // 2), packed(7, DC // 2, DH // 2), packed(7, DC // 2, DH // 2),
                          packed(7, DM // 2, DH // 2), [packed(QB, DH)] * (S // QB), [packed(QB, DH)] * (S // QB))

        def phase3(acca, ostage, q0):
            ri = jax.lax.broadcasted_iota(jnp.int32, (AB, AB + 2 * M), 0)
            ci = jax.lax.broadcasted_iota(jnp.int32, (AB, AB + 2 * M), 1)
            amask = (((ci < AB) & ((ci // SEG) == (ri // SEG)) & (ci <= ri))
                     | ((ci >= AB) & (((ci - AB) // M) == (ri // SEG))))

            def out_copy(r):
                rows = _half(r * OUT, OUT)
                return pltpu.make_async_copy(ostage.at[rows, :], out_h.bitcast(U32).at[0, rows, :], sem_out.at[r])

            def query_weight(h):
                return weight_terms(PT * (h // 2) + (h % 2) * HT)

            def query(wq, r):
                rows = []
                for g in range(r * RB // GB, (r + 1) * RB // GB):
                    q = {}
                    project_rows(g, wq, query_blocks(q))
                    rows += [jnp.concatenate([q[a, 0], q[a, 1]], axis=1) for a in range(2)]
                return jnp.concatenate(rows, axis=0)

            def a_head(h):
                wq = query_weight(h)
                wt = [t.astype(BF16) for t in _lhs_terms(_bf(awo[h]).astype(F32))]
                qs, ps, ctxs = {0: _bf(q0[...])}, {}, {}

                def project(r):
                    qs[r] = query(wq, r)

                def window(xref, mref, j):
                    return _bf(jnp.concatenate([xref[h, _half(j * AB, AB), :],
                                                mref[h, _half(j * 2 * M, 2 * M), :]], axis=0))

                def scores(r):
                    ps[r] = []
                    for j in range(RB // AB):
                        sc = _dot_nt(qs[r][j * AB:(j + 1) * AB], window(kx, km, r * RB // AB + j))
                        ps[r].append(_softmax2(jnp.where(amask, sc, NEG)))

                def context(r):
                    ctx = jnp.concatenate(
                        [_dot(p, window(vx, vm, r * RB // AB + j)) for j, p in enumerate(ps[r])], axis=0)
                    ctxs[r] = [context_terms(ctx[:GB]), context_terms(ctx[GB:])]

                def output(r):
                    for _ in add_output(acca, r * RB, lambda n, r0, m: wt[n], ctxs[r], 1, h > 0):
                        pass

                nr = S // RB
                project(1)
                for r in range(nr):
                    scores(r)
                    if r > 0:
                        output(r - 1)
                    if r + 2 < nr:
                        project(r + 2)
                    context(r)
                q0[...] = _u32(query(query_weight(jnp.minimum(h + 1, H - 1)), 0))
                output(nr - 1)

            q0[...] = _u32(query(query_weight(0), 0))
            pl.loop(0, H)(a_head)

            @pl.loop(0, S // OUT)
            def _(r):
                cols = pl.ds(pl.multiple_of(r * OUT, OUT), OUT)
                ostage[_half(r * OUT, OUT), :] = _u32(
                    jnp.concatenate([acca[:, cols], accb[:, cols]], axis=0).astype(BF16).T)
                out_copy(r).start()

            @pl.loop(0, S // OUT)
            def _(r):
                out_copy(r).wait()

        with jax.named_scope('phase3'):
            pl.run_scoped(phase3, pltpu.VMEM((DM, S), F32), packed(S, 2 * DM), packed(RB, DH))

    scratch = [
        packed(7, S // 2, DP // 2),
        pltpu.VMEM((M, DP), F32),
        packed(H, DM, DH),
        packed(NP * PT, KM, 128),
        packed(NP * PT // 2, 128, 128),
        packed(H * DH, KM),
        packed(H * DH // 2, 128),
        packed(H, S, DH),
        packed(H, S, DH),
        packed(H, NSEG * M, DH),
        packed(H, NSEG * M, DH),
        packed(7, S // 2, DP // 2),
        packed(7, S // 2, DC // 2),
        pltpu.VMEM((NP, DM, DH), U32),
        pltpu.VMEM((NP, DC, DH), U32),
        pltpu.VMEM((NP, DC, DH), U32),
        packed(H, DM, DH),
        pltpu.VMEM((DM, S), F32),
        pltpu.SemaphoreType.DMA((3 + S // RB,)),
    ] + [pltpu.SemaphoreType.DMA((NP,)) for _ in range(8)] + [pltpu.SemaphoreType.DMA((S // OUT,))]
    return kernel, scratch


@jax.jit
def pallas_concat_heads__memory_aug_recurrent_mem_tr__compressed_kv_cla__prompt_kernel(
    A_x, A_mem0, A_Wq, A_Wk, A_Wv, A_Wo, A_seg_len, B_x, B_c_kv, B_w_q, B_w_uk, B_w_uv, B_w_o,
):
    del A_seg_len
    _, S, DM = A_x.shape
    M = A_mem0.shape[1]
    H, DH = A_Wq.shape[1], A_Wq.shape[2]
    DC = B_c_kv.shape[2]
    kernel, scratch = _make_kernel(S, DM, H, DH, M, 32, DC)
    return pl.pallas_call(
        kernel,
        out_shape=jax.ShapeDtypeStruct((1, S, 2 * DM), BF16),
        in_specs=[pl.BlockSpec(memory_space=pl.ANY)] * 12,
        out_specs=pl.BlockSpec(memory_space=pl.ANY),
        scratch_shapes=scratch,
        compiler_params=pltpu.CompilerParams(vmem_limit_bytes=126 * 1024 * 1024),
    )(A_x[0].T, A_mem0, A_Wq, A_Wk, A_Wv, A_Wo.transpose(0, 2, 1),
      B_x[0].T, B_c_kv, B_w_q, B_w_uk, B_w_uv, B_w_o.transpose(0, 2, 1))
```

```python
import jax
import jax.numpy as jnp
import jax.experimental.pallas as pl
import jax.experimental.pallas.tpu as pltpu

F32 = jnp.float32
BF16 = jnp.bfloat16
U32 = jnp.uint32
LOG2E = 1.4426950408889634
NEG = -1e30
NN = (((1,), (0,)), ((), ()))
NT = (((1,), (1,)), ((), ()))


def _dot(a, b):
    return jax.lax.dot_general(a, b, NN, preferred_element_type=F32)


def _dot_nt(a, b):
    return jax.lax.dot_general(a, b, NT, preferred_element_type=F32)


def _bf(u):
    return pltpu.bitcast(u, BF16)


def _u32(x):
    return pltpu.bitcast(x.astype(BF16), U32)


def _half(start, size):
    if isinstance(start, int):
        return pl.ds(start // 2, size // 2)
    return pl.ds(pl.multiple_of(start // 2, 8), size // 2)


def _unpack(u, parity):
    if isinstance(parity, int):
        w = (u << 16) if parity == 0 else (u & jnp.uint32(0xFFFF0000))
    else:
        w = (u >> (16 * parity).astype(U32)) << 16
    return pltpu.bitcast(w, F32)


def _lhs_terms(x):
    r, k = x.shape[0] // 2, x.shape[1] // 2
    x11, x12, x21, x22 = x[:r, :k], x[:r, k:], x[r:, :k], x[r:, k:]
    return [x11 + x22, x22, x21 + x22, x11, x11 + x12, x12 - x22, x21 - x11]


def _rhs_terms(w, k):
    n, k2 = w.shape[1] // 2, w.shape[0] - k
    w11, w12, w21, w22 = w[:k, :n], w[:k, n:], w[k:, :n], w[k:, n:]

    def full(a):
        return a if k2 == k else jnp.concatenate([a, jnp.zeros((k - k2, n), a.dtype)], axis=0)
    return [w11 + full(w22), full(w21) - w11, w11, w12 - full(w22), w22, w21 + w22, w11 + w12]


_STRASSEN = (
    ((1, 0, 0), (1, 1, 1)), ((1, 0, 0), (1, 1, 0)), ((1, 1, 0), (-1, 1, 1)), ((1, 0, 1), (1, 1, 1)),
    ((1, 0, 1), (-1, 0, 0)), ((1, 0, 0),), ((1, 1, 1),))


def _block_product(product, finish, start=None):
    c = {}
    for n, uses in enumerate(_STRASSEN):
        multiply = product(n)
        yield
        p = multiply()
        for sign, a, b in uses:
            if start and (a, b) not in c:
                c[a, b] = start(a, b)
            c[a, b] = p if (a, b) not in c else c[a, b] + p if sign > 0 else c[a, b] - p
            if all((a, b) != use[1:] for later in _STRASSEN[n + 1:] for use in later):
                finish(a, b, c[a, b])
        yield


def _rhs_terms_t(wt):
    n, k = wt.shape[0] // 2, wt.shape[1] // 2
    w11, w12, w21, w22 = wt[:n, :k], wt[n:, :k], wt[:n, k:], wt[n:, k:]
    return [w11 + w22, w21 - w11, w11, w12 - w22, w22, w21 + w22, w11 + w12]


def _zeros(i, shape):
    return jnp.full(shape, (i >> 10).astype(F32))


def _softmax2(sc):
    p = jnp.exp2(sc - jnp.max(sc, axis=1, keepdims=True))
    return (p / jnp.sum(p, axis=1, keepdims=True)).astype(BF16)


def _order(counts):
    done = [0] * len(counts)
    live = [a for a, n in enumerate(counts) if n > 0]
    order = []
    for _ in range(sum(counts)):
        j = min(live, key=lambda a: ((done[a] + 0.5) / counts[a], a))
        done[j] += 1
        order.append(j)
    return order


def _finish(gens):
    for g in gens:
        for _ in g:
            raise AssertionError("stream longer than announced")


def _merge(*streams):
    for j in _order([n for _, n in streams]):
        for _ in range(2):
            next(streams[j][0])
            yield
    _finish([g for g, _ in streams])


def _make_kernel(S, DM, H, DH, M, SEG, DC):
    NP = H // 2
    NSEG = S // SEG
    DP = 512
    KM = DM // 128 * 128
    HT = DH // 128
    PT = 6 * HT
    STEPS = NSEG // H
    QB = 128
    PVR = 4
    MBK, MBV = 64, 64
    GAPS = (1, 2, 1, 2)
    RB = 512
    XC = S // H
    GB = 2 * QB
    NG = S // GB
    G1, G3 = 2, 2
    AB = 2 * SEG
    QSC = LOG2E * DH ** -0.5

    def packed(*shape):
        return pltpu.VMEM(shape[:-2] + (shape[-2] // 2, shape[-1]), U32)

    def kernel(ax_h, mem_h, awq_h, awk_h, awv_h, awo_h, bx_h, ckv_h, bwq_h, bwk_h, bwv_h, bwo_h,
               out_h,
               ax, mem_s, awo, wqkv, wqkv_t, wo, wo_t, kx, vx, km, vm,
               bx, ckv, bwq, bwk, bwv, bwo, accb,
               sem_x, sem_aq, sem_ak, sem_av, sem_ao, sem_bq, sem_bk, sem_bv, sem_bo, sem_l, sem_r):

        def pair_copy(src, dst, sem, i):
            return pltpu.make_async_copy(src.bitcast(U32).at[:, i, :], dst.at[i], sem.at[i])

        def wo_copy(src, dst, sem, i):
            return pltpu.make_async_copy(src.bitcast(U32).at[pl.ds(2 * i, 2)], dst.at[pl.ds(2 * i, 2)], sem.at[i])

        def head_weight(t):
            return _bf(jnp.concatenate(
                [jnp.concatenate([wqkv[t + j], wqkv_t[t // 2 + j // 2, _half((j % 2) * 64, 64), :]], axis=0)
                 for j in range(HT)], axis=1))

        def transposed(raw, c, n):
            xt = _bf(raw[:, pl.ds(c if isinstance(c, int) else pl.multiple_of(c, n), n)])
            return jnp.concatenate([xt, jnp.zeros((DP - DM, n), BF16)], axis=0).T

        def keep_terms(dst, g, x):
            for n, term in enumerate(_lhs_terms(x.astype(F32))):
                dst[n, _half(g * QB, QB), :] = _u32(term)

        def project_rows(g, terms, finish):
            def product(n):
                x = _bf(ax[n, _half(g * QB, len(finish) * QB), :])[:, :terms[n].shape[0]]
                return lambda: _dot(x, terms[n])

            def finish_all(a, b, c):
                for j, fin in enumerate(finish):
                    fin(a, b, c[j * QB:(j + 1) * QB])
            for _ in _block_product(product, finish_all):
                pass

        def store_blocks(top, bottom, row):
            def finish(a, b, c):
                (top, bottom)[a][_half(row, c.shape[0]), b * 128:(b + 1) * 128] = _u32(c)
            return finish

        def query_blocks(blocks):
            def finish(a, b, c):
                blocks[a, b] = (c * QSC).astype(BF16)
            return finish

        def add_output(acc, col, wt, ctx, parts, keep=None):
            half = DM // 2

            def product(n):
                ws = [wt(n, r, half // parts) for r in range(0, half, half // parts)]
                return lambda: jnp.concatenate(
                    [jnp.concatenate([_dot_nt(w, c[n]) for w in ws], axis=0) for c in ctx], axis=1)

            def where(a, b, j):
                return slice(a * half, (a + 1) * half), slice(col + j * GB + b * QB, col + j * GB + (b + 1) * QB)

            def start(a, b):
                old = jnp.concatenate([acc[where(a, b, j)] for j in range(2)], axis=1)
                return old if keep is None else jnp.where(keep, old, 0.0)

            def finish(a, b, c):
                for j in range(2):
                    acc[where(a, b, j)] = c[:, j * QB:(j + 1) * QB]
            return _block_product(product, finish, start)

        def context_terms(ctx):
            return [t.astype(BF16) for t in _rhs_terms_t(ctx)]

        def weight_terms(t):
            return [w.astype(BF16) for w in _rhs_terms(head_weight(t).astype(F32), DP // 2)]

        def phase1(xraw, craw, mem0, awq, awk, awv):
            def cp_ax(r):
                cols = pl.ds(r * RB if isinstance(r, int) else pl.multiple_of(r * RB, RB), RB)
                return pltpu.make_async_copy(ax_h.bitcast(U32).at[:, cols], xraw.at[:, cols], sem_x.at[3 + r])

            cp_mem = pltpu.make_async_copy(mem_h.at[0], mem0, sem_x.at[0])
            cp_bx = pltpu.make_async_copy(bx_h.bitcast(U32), xraw.at[:, pl.ds(S, S)], sem_x.at[1])
            cp_ckv = pltpu.make_async_copy(ckv_h.bitcast(U32).at[0], craw, sem_x.at[2])

            def a_weights(i):
                pair_copy(awk_h, awk, sem_ak, i).start()
                pair_copy(awv_h, awv, sem_av, i).start()
                pair_copy(awq_h, awq, sem_aq, i).start()
                wo_copy(awo_h, awo, sem_ao, i).start()

            def b_weights(i):
                pair_copy(bwq_h, bwq, sem_bq, i).start()
                pair_copy(bwk_h, bwk, sem_bk, i).start()
                pair_copy(bwv_h, bwv, sem_bv, i).start()
                wo_copy(bwo_h, bwo, sem_bo, i).start()

            for r in range(S // RB):
                cp_ax(r).start()
            pair_copy(awk_h, awk, sem_ak, 0).start()
            pair_copy(awv_h, awv, sem_av, 0).start()

            def keep(w, t):
                u = _u32(w)
                for j in range(HT):
                    wqkv[t + j] = u[:KM // 2, j * 128:(j + 1) * 128]
                    wqkv_t[t // 2 + j // 2, _half((j % 2) * 64, 64), :] = u[KM // 2:, j * 128:(j + 1) * 128]

            def keep_kv(h):
                i = h // 2
                keep(_unpack(awk[i], h % 2), PT * i + (2 + h % 2) * HT)
                keep(_unpack(awv[i], h % 2), PT * i + (4 + h % 2) * HT)

            @pl.loop(0, S // RB)
            def _(r):
                cp_ax(r).wait()
                for j in range(RB // GB):
                    g = r * (RB // GB) + j
                    keep_terms(ax, g, transposed(xraw, g * GB, GB))
            pair_copy(awq_h, awq, sem_aq, 0).start()
            wo_copy(awo_h, awo, sem_ao, 0).start()
            pair_copy(awk_h, awk, sem_ak, 0).wait()
            pair_copy(awv_h, awv, sem_av, 0).wait()
            keep_kv(0)
            cp_bx.start()
            cp_mem.start()
            pl.loop(1, NP)(a_weights)
            cp_ckv.start()
            pl.loop(0, NP)(b_weights)

            @pl.loop(0, H)
            def _(h):
                i = h // 2
                par = h % 2

                @pl.when(par == 0)
                def _():
                    pair_copy(awq_h, awq, sem_aq, i).wait()
                    wo_copy(awo_h, awo, sem_ao, i).wait()

                @pl.when((par == 1) & (i + 1 < NP))
                def _():
                    pair_copy(awk_h, awk, sem_ak, i + 1).wait()
                    pair_copy(awv_h, awv, sem_av, i + 1).wait()

                @pl.when(h == 1)
                def _():
                    cp_bx.wait()

                @pl.when(h == H - NG)
                def _():
                    cp_ckv.wait()

                @pl.when(h >= H - NG)
                def _():
                    g = h - (H - NG)
                    keep_terms(ckv, g, _bf(craw[_half(g * GB, GB), :]))
                wk, wv = weight_terms(PT * i + (2 + par) * HT), weight_terms(PT * i + (4 + par) * HT)
                for g in range(0, NG, G1):
                    for dst, terms in ((kx, wk), (vx, wv)):
                        project_rows(g, terms, [
                            store_blocks(*[dst.at[h, _half(j * GB + a * QB, QB)] for a in range(2)], 0)
                            for j in range(g, g + G1)])
                    if g == 0:
                        w = _u32(jnp.concatenate([_bf(awo[h]), jnp.zeros((DP - DM, DH), BF16)], axis=0).T)
                        wo[_half(h * DH, DH), :] = w[:, :KM]
                        wo_t[_half(h * 128, 128), :] = w[:64, KM:] | pltpu.roll(w[64:, KM:], 64, 1)
                    if g == 2:
                        src = jnp.where(h == 0, NG - 1, NG + (h - 1) % NG)
                        keep_terms(bx, (h + NG - 1) % NG, transposed(xraw, src * GB, GB))
                    if g == 2:
                        keep(_unpack(awq[i], par), PT * i + par * HT)
                        accb[:, pl.ds(pl.multiple_of(h * XC, XC), XC)] = jnp.zeros((DM, XC), F32)
                    if g == 4:
                        keep_kv(jnp.minimum(h + 1, H - 1))
            cp_mem.wait()
            mem_s[...] = jnp.concatenate([mem0[...].astype(F32), jnp.zeros((M, DP - DM), F32)], axis=1)

        with jax.named_scope('phase1'):
            pl.run_scoped(phase1, packed(DM, 2 * S), packed(S, DC), pltpu.VMEM((M, DM), BF16),
                          *[pltpu.VMEM((NP, DM, DH), U32)] * 3)

        def chain_step(s, held):
            mem = mem_s[...]
            zero = s >> 10
            mt = mem[:, KM:]
            mtail = jnp.concatenate([mt, pltpu.roll(mt, 64, 1)], axis=0).astype(BF16)
            t = []
            for g in range(0, NP * PT, 8):
                for t0 in (g, g + 4):
                    acc = _zeros(s, (M, 512))
                    for k0 in range(0, KM, 128):
                        w = jnp.concatenate([wqkv[t0 + j + zero, _half(k0, 128), :] for j in range(4)], axis=1)
                        yield
                        acc = acc + _dot(mem[:, k0:k0 + 128], _bf(w))
                        yield
                    t += [acc[:, j * 128:(j + 1) * 128] for j in range(4)]
                w = jnp.concatenate([wqkv_t[g // 2 + j + zero] for j in range(4)], axis=1)
                yield
                d = _dot(mtail, _bf(w))
                for j in range(8):
                    t[g + j] = t[g + j] + d[(j % 2) * M:(j % 2 + 1) * M, (j // 2) * 128:(j // 2 + 1) * 128]
                yield
            for _ in range(2 * GAPS[0]):
                yield

            def head_rows(i, which, par):
                t0 = PT * i + (2 * which + par) * HT
                return jnp.concatenate(t[t0:t0 + HT], axis=1)

            def pair_rows(i, which):
                return jnp.concatenate([head_rows(i, which, 0), head_rows(i, which, 1)], axis=0)

            def window(ref, i, which):
                xr = _half(s * SEG, SEG)
                return jnp.concatenate([_bf(ref[2 * i, xr, :]), _bf(ref[2 * i + 1, xr, :]),
                                        pair_rows(i, which).astype(BF16)], axis=0)

            now = [[head_rows(h // 2, which, h % 2) for h in range(H)] for which in (1, 2)]
            if held:
                for ref, old, new in zip((km, vm), held.pop(), now):
                    for h in range(H):
                        ref[h, _half((s - 1) * M, 2 * M), :] = _u32(jnp.concatenate([old[h], new[h]], axis=0))
            else:
                held.append(now)
            sc = []
            for i0 in range(0, NP, 2):
                ops = [((pair_rows(i, 0) * QSC).astype(BF16), window(kx, i, 1)) for i in (i0, i0 + 1)]
                yield
                sc += [_dot_nt(q, k) for q, k in ops]
                yield
            for _ in range(2 * GAPS[1]):
                yield
            sc = jnp.concatenate(sc, axis=0)
            par = (jax.lax.broadcasted_iota(jnp.int32, sc.shape, 0) // M) % 2
            ci = jax.lax.broadcasted_iota(jnp.int32, sc.shape, 1)
            own = jnp.where(ci < 2 * SEG, ci // SEG, (ci - 2 * SEG) // M) == par
            p = _softmax2(jnp.where(own, sc, NEG))
            zt = []
            for i0 in range(0, NP, 2):
                ops = [(p[2 * M * i:2 * M * (i + 1)], window(vx, i, 2)) for i in (i0, i0 + 1)]
                yield
                for pp, v in ops:
                    o = _dot(pp, v)
                    zt += [o[par * M:(par + 1) * M, j * 128:(j + 1) * 128] for par in range(2) for j in range(HT)]
                yield
            for _ in range(2 * GAPS[2]):
                yield
            acc = [_zeros(s, (M, 128))] * 3 + [_zeros(s, (2 * M, 128))]
            for g in range(0, H * HT, 8):
                for t0 in (g, g + 4):
                    zp = jnp.concatenate(zt[t0:t0 + 4], axis=1).astype(BF16).astype(F32)
                    for n in range(KM // 128):
                        w = wo[_half((t0 + zero) * 128, 512), n * 128:(n + 1) * 128]
                        yield
                        acc[n] = acc[n] + _dot(zp, _bf(w))
                        yield
                zp = jnp.concatenate([jnp.concatenate(zt[g:g + 8:2], axis=1),
                                      jnp.concatenate(zt[g + 1:g + 8:2], axis=1)], axis=0).astype(BF16)
                w = wo_t[_half((g // 2 + zero) * 128, 512), :]
                yield
                acc[3] = acc[3] + _dot(zp, _bf(w))
                yield
            lane = jax.lax.broadcasted_iota(jnp.int32, (M, 128), 1)
            last = jnp.where(lane < 64, acc[3][:M] + pltpu.roll(acc[3][M:], 64, 1), 0.0)
            mem_s[...] = jnp.concatenate(acc[:3] + [last], axis=1).astype(BF16).astype(F32)
            for _ in range(2 * GAPS[3]):
                yield

        def chain(h):
            held = []
            for j in range(STEPS):
                yield from chain_step(h * STEPS + j, held)

        n_chain = STEPS * ((NP * PT + H * HT) // 8 * 7 + NP + sum(GAPS))
        n_qk, n_v = 7 * (1 + QB // MBK), 7 * (QB // MBV)

        def split(r):
            return 2 if r >= PVR else 1

        def n_scores(r):
            return (r + 2) // 2

        def n_context(r):
            return (r + 1) // 2 * split(r) + (r + 1) % 2

        n_head = (NG * (n_qk + n_v) + (NG // 2) * 7 - (S // QB // 2 - 1)
                  + sum(n_scores(r) + n_context(r) for r in range(S // QB)))

        def phase2(wq_s, wk_s, wv_s, wo_s, k_s, v_s):
            def b_head(h):
                i = h // 2
                par = h % 2
                for w_s, raw in ((wq_s, bwq), (wk_s, bwk), (wv_s, bwv)):
                    for n, term in enumerate(_rhs_terms(_unpack(raw[i], par), 2 * w_s.shape[1])):
                        w_s[n, _half(0, term.shape[0]), :] = _u32(term)
                for n, term in enumerate(_lhs_terms(_bf(bwo[h]).astype(F32))):
                    wo_s[n] = _u32(term)
                qs, ss, ms, ctxs = {}, {}, {}, {}

                def chunks(r):
                    nk = (r + 1) * QB
                    return [(c0, min(c0 + 256, nk)) for c0 in range(0, nk, 256)]

                def project(g, r0, src, w_s, depth, mb, together, finish):
                    def product(n):
                        k = depth - 2 * w_s.shape[1] if n in (4, 5) else 2 * w_s.shape[1]
                        xs = [_bf(src[n, _half(g * QB + r0 + j * mb, mb), :])[:, :k] for j in range(together)]
                        w = _bf(w_s[n, _half(0, k), :])
                        return lambda: jnp.concatenate([_dot(x, w) for x in xs], axis=0)
                    return _block_product(product, finish)

                def project_qk(g):
                    q = {}
                    yield from project(g, 0, bx, wq_s, DM, QB // 2, 2, query_blocks(q))
                    for a in range(2):
                        qs[2 * g + a] = jnp.concatenate([q[a, 0], q[a, 1]], axis=1)
                    for r0 in range(0, QB, MBK):
                        yield from project(g, r0, ckv, wk_s, DC, MBK, 1, store_blocks(*k_s[2 * g:2 * g + 2], r0))

                def project_v(g):
                    for r0 in range(0, QB, MBV):
                        yield from project(g, r0, ckv, wv_s, DC, MBV, 1, store_blocks(*v_s[2 * g:2 * g + 2], r0))

                def blocks(refs, c0, c1):
                    return _bf(jnp.concatenate([refs[j][...] for j in range(c0 // QB, c1 // QB)], axis=0))

                def scores(r):
                    ss[r] = []
                    m = None
                    for c0, c1 in chunks(r):
                        k = blocks(k_s, c0, c1)
                        yield
                        sc = _dot_nt(qs[r], k)
                        if c1 == (r + 1) * QB:
                            ri = jax.lax.broadcasted_iota(jnp.int32, sc.shape, 0) + r * QB
                            ci = jax.lax.broadcasted_iota(jnp.int32, sc.shape, 1) + c0
                            sc = jnp.where(ci <= ri, sc, NEG)
                        ss[r].append(sc)
                        for t0 in range(0, c1 - c0, 128):
                            m = sc[:, t0:t0 + 128] if m is None else jnp.maximum(m, sc[:, t0:t0 + 128])
                        if c1 == (r + 1) * QB:
                            ms[r] = jnp.max(m, axis=1, keepdims=True)
                        yield

                def context(r):
                    ls = []

                    def weights(c):
                        p = jnp.exp2(ss[r][c] - ms[r])
                        for t0 in range(0, p.shape[1], 128):
                            ls[:] = [p[:, t0:t0 + 128] + ls[0] if ls else p[:, t0:t0 + 128]]
                        return p.astype(BF16)

                    acc = _zeros(h, (QB, DH))
                    nxt = weights(0)
                    for c, (c0, c1) in enumerate(chunks(r)):
                        mb = QB // split(r) if c1 - c0 == 256 else QB
                        p = nxt
                        v = blocks(v_s, c0, c1)
                        new = []
                        for r0 in range(0, QB, mb):
                            yield
                            new.append(acc[r0:r0 + mb] + _dot(p[r0:r0 + mb], v))
                            if r0 == 0 and c1 < (r + 1) * QB:
                                nxt = weights(c + 1)
                            if r0 + mb == QB:
                                acc = jnp.concatenate(new, axis=0)
                                if c1 == (r + 1) * QB:
                                    ctxs[r] = acc / jnp.sum(ls[0], axis=1, keepdims=True)
                                    if r % 2:
                                        ctxs[r] = context_terms(jnp.concatenate([ctxs[r - 1], ctxs[r]], axis=0))
                            yield

                def output(r):
                    yield from add_output(accb, (r - 3) * QB, lambda n, r0, m: _bf(wo_s[n, _half(r0, m), :]),
                                          (ctxs[r - 2], ctxs[r]), 2)

                def both(r):
                    a, b = scores(r), context(r - 2)
                    na, nc = n_scores(r) - 1, n_context(r - 2) - 1
                    for j in _order([na, nc]):
                        for _ in range(2):
                            next((a, b)[j])
                            yield
                    for _ in range(2):
                        next(a)
                        next(b)
                        yield
                    _finish([a, b])

                nb = S // QB
                for r in range(nb + 4):
                    parts = []
                    if r < nb:
                        parts.append((project_v(r // 2), n_v) if r % 2 else (project_qk(r // 2), n_qk))
                    if 0 <= r - 4 < nb and (r - 4) % 4 == 3:
                        parts.append((output(r - 4), 7))
                    if r % 2 == 1 and 3 <= r <= nb:
                        parts.append((both(r - 1), n_scores(r - 1) + n_context(r - 3) - 1))
                    else:
                        if 0 <= r - 1 < nb:
                            parts.append((scores(r - 1), n_scores(r - 1)))
                        if 0 <= r - 3 < nb:
                            parts.append((context(r - 3), n_context(r - 3)))
                    yield from _merge(*parts)

            def b_body(h, c):
                i = h // 2

                @pl.when(h % 2 == 0)
                def _():
                    pair_copy(bwq_h, bwq, sem_bq, i).wait()
                    pair_copy(bwk_h, bwk, sem_bk, i).wait()
                    pair_copy(bwv_h, bwv, sem_bv, i).wait()
                    wo_copy(bwo_h, bwo, sem_bo, i).wait()
                for _ in _merge((chain(h), n_chain), (b_head(h), n_head)):
                    pass
                return c
            jax.lax.fori_loop(0, H, b_body, 0)

        with jax.named_scope('phase2'):
            pl.run_scoped(phase2, packed(7, DP // 2, DH // 2), packed(7, DC // 2, DH // 2), packed(7, DC // 2, DH // 2),
                          packed(7, DM // 2, DH // 2), [packed(QB, DH)] * (S // QB), [packed(QB, DH)] * (S // QB))

        def phase3(acca, ostage, q0):
            ri = jax.lax.broadcasted_iota(jnp.int32, (AB, AB + 2 * M), 0)
            ci = jax.lax.broadcasted_iota(jnp.int32, (AB, AB + 2 * M), 1)
            amask = (((ci < AB) & ((ci // SEG) == (ri // SEG)) & (ci <= ri))
                     | ((ci >= AB) & (((ci - AB) // M) == (ri // SEG))))

            def out_copy(row, n, cols, sem):
                rows = _half(row, n)
                return pltpu.make_async_copy(ostage.at[rows, cols], out_h.bitcast(U32).at[0, rows, cols], sem)

            def left_copy(r):
                return out_copy(r * GB, GB, pl.ds(0, DP), sem_l.at[r])

            def right_copy(h):
                return out_copy(h * XC, XC, pl.ds(DP, 2 * DM - DP), sem_r.at[h])

            def query_weight(h):
                return weight_terms(PT * (h // 2) + (h % 2) * HT)

            def query(wq, r):
                qs = [{} for _ in range(RB // GB)]
                for j in range(0, RB // GB, G3):
                    project_rows(r * RB // GB + j, wq, [query_blocks(q) for q in qs[j:j + G3]])
                return jnp.concatenate([jnp.concatenate([q[a, 0], q[a, 1]], axis=1)
                                        for q in qs for a in range(2)], axis=0)

            def a_head(h):
                wq = query_weight(h)
                wt = [t.astype(BF16) for t in _lhs_terms(_bf(awo[h]).astype(F32))]
                qs, ps, ctxs = {0: _bf(q0[...])}, {}, {}

                def project(r):
                    qs[r] = query(wq, r)

                def window(xref, mref, j):
                    return _bf(jnp.concatenate([xref[h, _half(j * AB, AB), :],
                                                mref[h, _half(j * 2 * M, 2 * M), :]], axis=0))

                def scores(r):
                    ps[r] = []
                    for j in range(RB // AB):
                        sc = _dot_nt(qs[r][j * AB:(j + 1) * AB], window(kx, km, r * RB // AB + j))
                        ps[r].append(_softmax2(jnp.where(amask, sc, NEG)))

                def context(r):
                    ctx = jnp.concatenate(
                        [_dot(p, window(vx, vm, r * RB // AB + j)) for j, p in enumerate(ps[r])], axis=0)
                    ctxs[r] = [context_terms(ctx[:GB]), context_terms(ctx[GB:])]

                def output(r):
                    for _ in add_output(acca, r * RB, lambda n, r0, m: wt[n], ctxs[r], 1, h > 0):
                        pass

                nr = S // RB
                project(1)
                ostage[_half(h * XC, XC), DP:] = _u32(
                    accb[DP - DM:, pl.ds(pl.multiple_of(h * XC, XC), XC)].astype(BF16).T)
                for r in range(nr):
                    scores(r)
                    if r > 0:
                        output(r - 1)
                    if r + 2 < nr:
                        project(r + 2)
                    context(r)
                q0[...] = _u32(query(query_weight(jnp.minimum(h + 1, H - 1)), 0))
                output(nr - 1)
                right_copy(h).start()

            q0[...] = _u32(query(query_weight(0), 0))
            pl.loop(0, H)(a_head)

            @pl.loop(0, NG)
            def _(r):
                cols = pl.ds(pl.multiple_of(r * GB, GB), GB)
                ostage[_half(r * GB, GB), :DP] = _u32(
                    jnp.concatenate([acca[:, cols], accb[:DP - DM, cols]], axis=0).astype(BF16).T)
                left_copy(r).start()

            pl.loop(0, H)(lambda h: right_copy(h).wait())
            pl.loop(0, NG)(lambda r: left_copy(r).wait())

        with jax.named_scope('phase3'):
            pl.run_scoped(phase3, pltpu.VMEM((DM, S), F32), packed(S, 2 * DM), packed(RB, DH))

    scratch = [
        packed(7, S // 2, DP // 2),
        pltpu.VMEM((M, DP), F32),
        packed(H, DM, DH),
        packed(NP * PT, KM, 128),
        packed(NP * PT // 2, 128, 128),
        packed(H * DH, KM),
        packed(H * DH // 2, 128),
        packed(H, S, DH),
        packed(H, S, DH),
        packed(H, NSEG * M, DH),
        packed(H, NSEG * M, DH),
        packed(7, S // 2, DP // 2),
        packed(7, S // 2, DC // 2),
        pltpu.VMEM((NP, DM, DH), U32),
        pltpu.VMEM((NP, DC, DH), U32),
        pltpu.VMEM((NP, DC, DH), U32),
        packed(H, DM, DH),
        pltpu.VMEM((DM, S), F32),
        pltpu.SemaphoreType.DMA((3 + S // RB,)),
    ] + [pltpu.SemaphoreType.DMA((NP,)) for _ in range(8)] + [pltpu.SemaphoreType.DMA((NG,)), pltpu.SemaphoreType.DMA((H,))]
    return kernel, scratch


@jax.jit
def pallas_concat_heads__memory_aug_recurrent_mem_tr__compressed_kv_cla__prompt_kernel(
    A_x, A_mem0, A_Wq, A_Wk, A_Wv, A_Wo, A_seg_len, B_x, B_c_kv, B_w_q, B_w_uk, B_w_uv, B_w_o,
):
    del A_seg_len
    _, S, DM = A_x.shape
    M = A_mem0.shape[1]
    H, DH = A_Wq.shape[1], A_Wq.shape[2]
    DC = B_c_kv.shape[2]
    kernel, scratch = _make_kernel(S, DM, H, DH, M, 32, DC)
    return pl.pallas_call(
        kernel,
        out_shape=jax.ShapeDtypeStruct((1, S, 2 * DM), BF16),
        in_specs=[pl.BlockSpec(memory_space=pl.ANY)] * 12,
        out_specs=pl.BlockSpec(memory_space=pl.ANY),
        scratch_shapes=scratch,
        compiler_params=pltpu.CompilerParams(vmem_limit_bytes=126 * 1024 * 1024),
    )(A_x[0].T, A_mem0, A_Wq, A_Wk, A_Wv, A_Wo.transpose(0, 2, 1),
      B_x[0].T, B_c_kv, B_w_q, B_w_uk, B_w_uv, B_w_o.transpose(0, 2, 1))
```

```python
import jax
import jax.numpy as jnp
import jax.experimental.pallas as pl
import jax.experimental.pallas.tpu as pltpu

F32 = jnp.float32
BF16 = jnp.bfloat16
U32 = jnp.uint32
LOG2E = 1.4426950408889634
NEG = -1e30
NN = (((1,), (0,)), ((), ()))
NT = (((1,), (1,)), ((), ()))


def _dot(a, b):
    return jax.lax.dot_general(a, b, NN, preferred_element_type=F32)


def _dot_nt(a, b):
    return jax.lax.dot_general(a, b, NT, preferred_element_type=F32)


def _bf(u):
    return pltpu.bitcast(u, BF16)


def _u32(x):
    return pltpu.bitcast(x.astype(BF16), U32)


def _half(start, size):
    if isinstance(start, int):
        return pl.ds(start // 2, size // 2)
    return pl.ds(pl.multiple_of(start // 2, 8), size // 2)


def _put(ref, lead, row, col, x):
    ref[(*lead, _half(row, x.shape[0]), pl.ds(col, x.shape[1]))] = _u32(x)


def _unpack(u, parity):
    if isinstance(parity, int):
        w = (u << 16) if parity == 0 else (u & jnp.uint32(0xFFFF0000))
    else:
        w = (u >> (16 * parity).astype(U32)) << 16
    return pltpu.bitcast(w, F32)


def _lhs_terms(x):
    r, k = x.shape[0] // 2, x.shape[1] // 2
    x11, x12, x21, x22 = x[:r, :k], x[:r, k:], x[r:, :k], x[r:, k:]
    return [x11 + x22, x22, x21 + x22, x11, x11 + x12, x12 - x22, x21 - x11]


def _rhs_terms(w, k):
    n, k2 = w.shape[1] // 2, w.shape[0] - k
    w11, w12, w21, w22 = w[:k, :n], w[:k, n:], w[k:, :n], w[k:, n:]

    def full(a):
        return a if k2 == k else jnp.concatenate([a, jnp.zeros((k - k2, n), a.dtype)], axis=0)
    return [w11 + full(w22), full(w21) - w11, w11, w12 - full(w22), w22, w21 + w22, w11 + w12]


_STRASSEN = (
    ((1, 0, 0), (1, 1, 1)), ((1, 0, 0), (1, 1, 0)), ((1, 1, 0), (-1, 1, 1)), ((1, 0, 1), (1, 1, 1)),
    ((1, 0, 1), (-1, 0, 0)), ((1, 0, 0),), ((1, 1, 1),))


def _block_product(product, finish, start=None):
    c = {}
    for n, uses in enumerate(_STRASSEN):
        multiply = product(n)
        yield
        p = multiply()
        for sign, a, b in uses:
            if start and (a, b) not in c:
                c[a, b] = start(a, b)
            c[a, b] = p if (a, b) not in c else c[a, b] + p if sign > 0 else c[a, b] - p
            if all((a, b) != use[1:] for later in _STRASSEN[n + 1:] for use in later):
                finish(a, b, c[a, b])
        yield


def _rhs_terms_t(wt):
    n, k = wt.shape[0] // 2, wt.shape[1] // 2
    w11, w12, w21, w22 = wt[:n, :k], wt[n:, :k], wt[:n, k:], wt[n:, k:]
    return [w11 + w22, w21 - w11, w11, w12 - w22, w22, w21 + w22, w11 + w12]


def _zeros(i, shape):
    return jnp.full(shape, (i >> 10).astype(F32))


def _softmax2(sc):
    p = jnp.exp2(sc - jnp.max(sc, axis=1, keepdims=True))
    return (p / jnp.sum(p, axis=1, keepdims=True)).astype(BF16)


def _order(counts):
    done = [0] * len(counts)
    live = [a for a, n in enumerate(counts) if n > 0]
    order = []
    for _ in range(sum(counts)):
        j = min(live, key=lambda a: ((done[a] + 0.5) / counts[a], a))
        done[j] += 1
        order.append(j)
    return order


def _finish(gens):
    for g in gens:
        for _ in g:
            raise AssertionError("stream longer than announced")


def _merge(*streams):
    for j in _order([n for _, n in streams]):
        for _ in range(2):
            next(streams[j][0])
            yield
    _finish([g for g, _ in streams])


def _make_kernel(S, DM, H, DH, M, SEG, DC):
    NP = H // 2
    NSEG = S // SEG
    DP = 512
    KM = DM // 128 * 128
    HT = DH // 128
    PT = 6 * HT
    STEPS = NSEG // H
    QB = 128
    PVR = 6
    MBK, MBV = 64, 64
    GAPS = (1, 2, 1, 1)
    RB = 512
    XC = S // H
    GB = 2 * QB
    NG = S // GB
    G1, G3 = 2, 2
    AB = 2 * SEG
    QSC = LOG2E * DH ** -0.5

    def packed(*shape):
        return pltpu.VMEM(shape[:-2] + (shape[-2] // 2, shape[-1]), U32)

    def kernel(ax_h, mem_h, awq_h, awk_h, awv_h, awo_h, bx_h, ckv_h, bwq_h, bwk_h, bwv_h, bwo_h,
               out_h,
               ax, mem_s, awo, wqkv, wqkv_t, wo, wo_t, kx, vx, km, vm,
               bx, ckv, bwq, bwk, bwv, bwo, accb,
               sem_x, sem_aq, sem_ak, sem_av, sem_ao, sem_bq, sem_bk, sem_bv, sem_bo, sem_l, sem_r):

        def pair_copy(src, dst, sem, i):
            return pltpu.make_async_copy(src.bitcast(U32).at[:, i, :], dst.at[i], sem.at[i])

        def wo_copy(src, dst, sem, i):
            return pltpu.make_async_copy(src.bitcast(U32).at[pl.ds(2 * i, 2)], dst.at[pl.ds(2 * i, 2)], sem.at[i])

        def head_weight(t):
            return _bf(jnp.concatenate(
                [jnp.concatenate([wqkv[t + j], wqkv_t[t // 2 + j // 2, _half((j % 2) * 64, 64), :]], axis=0)
                 for j in range(HT)], axis=1))

        def transposed(raw, c, n):
            xt = _bf(raw[:, pl.ds(c if isinstance(c, int) else pl.multiple_of(c, n), n)])
            return jnp.concatenate([xt, jnp.zeros((DP - DM, n), BF16)], axis=0).T

        def keep_terms(dst, g, x):
            for n, term in enumerate(_lhs_terms(x.astype(F32))):
                _put(dst, (n,), g * QB, 0, term)

        def project_rows(g, terms, finish):
            def product(n):
                x = _bf(ax[n, _half(g * QB, len(finish) * QB), :])[:, :terms[n].shape[0]]
                return lambda: _dot(x, terms[n])

            def finish_all(a, b, c):
                for j, fin in enumerate(finish):
                    fin(a, b, c[j * QB:(j + 1) * QB])
            for _ in _block_product(product, finish_all):
                pass

        def store_blocks(top, bottom):
            def finish(a, b, c):
                _put(*(top, bottom)[a], b * 128, c)
            return finish

        def query_blocks(blocks):
            def finish(a, b, c):
                blocks[a, b] = (c * QSC).astype(BF16)
            return finish

        def add_output(acc, col, wt, ctx, parts, keep=None):
            half = DM // 2

            def product(n):
                ws = [wt(n, r, half // parts) for r in range(0, half, half // parts)]
                return lambda: jnp.concatenate(
                    [jnp.concatenate([_dot_nt(w, c[n]) for w in ws], axis=0) for c in ctx], axis=1)

            def where(a, b, j):
                return slice(a * half, (a + 1) * half), slice(col + j * GB + b * QB, col + j * GB + (b + 1) * QB)

            def start(a, b):
                old = jnp.concatenate([acc[where(a, b, j)] for j in range(2)], axis=1)
                return old if keep is None else jnp.where(keep, old, 0.0)

            def finish(a, b, c):
                for j in range(2):
                    acc[where(a, b, j)] = c[:, j * QB:(j + 1) * QB]
            return _block_product(product, finish, start)

        def context_terms(ctx):
            return [t.astype(BF16) for t in _rhs_terms_t(ctx)]

        def weight_terms(t):
            return [w.astype(BF16) for w in _rhs_terms(head_weight(t).astype(F32), DP // 2)]

        def phase1(xraw, craw, mem0, awq, awk, awv):
            def cp_ax(r):
                cols = pl.ds(r * RB if isinstance(r, int) else pl.multiple_of(r * RB, RB), RB)
                return pltpu.make_async_copy(ax_h.bitcast(U32).at[:, cols], xraw.at[:, cols], sem_x.at[3 + r])

            cp_mem = pltpu.make_async_copy(mem_h.at[0], mem0, sem_x.at[0])
            cp_bx = pltpu.make_async_copy(bx_h.bitcast(U32), xraw.at[:, pl.ds(S, S)], sem_x.at[1])
            cp_ckv = pltpu.make_async_copy(ckv_h.bitcast(U32).at[0], craw, sem_x.at[2])

            def a_weights(i):
                pair_copy(awk_h, awk, sem_ak, i).start()
                pair_copy(awv_h, awv, sem_av, i).start()
                pair_copy(awq_h, awq, sem_aq, i).start()
                wo_copy(awo_h, awo, sem_ao, i).start()

            def b_weights(i):
                pair_copy(bwq_h, bwq, sem_bq, i).start()
                pair_copy(bwk_h, bwk, sem_bk, i).start()
                pair_copy(bwv_h, bwv, sem_bv, i).start()
                wo_copy(bwo_h, bwo, sem_bo, i).start()

            for r in range(S // RB):
                cp_ax(r).start()
            pair_copy(awk_h, awk, sem_ak, 0).start()
            pair_copy(awv_h, awv, sem_av, 0).start()

            def keep(w, t):
                for j in range(HT):
                    _put(wqkv, (t + j,), 0, 0, w[:KM, j * 128:(j + 1) * 128])
                    _put(wqkv_t, (t // 2 + j // 2,), (j % 2) * 64, 0, w[KM:, j * 128:(j + 1) * 128])

            def keep_kv(h):
                i = h // 2
                keep(_unpack(awk[i], h % 2), PT * i + (2 + h % 2) * HT)
                keep(_unpack(awv[i], h % 2), PT * i + (4 + h % 2) * HT)

            @pl.loop(0, S // RB)
            def _(r):
                cp_ax(r).wait()
                for j in range(RB // GB):
                    g = r * (RB // GB) + j
                    keep_terms(ax, g, transposed(xraw, g * GB, GB))
            pair_copy(awq_h, awq, sem_aq, 0).start()
            wo_copy(awo_h, awo, sem_ao, 0).start()
            pair_copy(awk_h, awk, sem_ak, 0).wait()
            pair_copy(awv_h, awv, sem_av, 0).wait()
            keep_kv(0)
            cp_bx.start()
            cp_mem.start()
            pl.loop(1, NP)(a_weights)
            cp_ckv.start()
            pl.loop(0, NP)(b_weights)

            @pl.loop(0, H)
            def _(h):
                i = h // 2
                par = h % 2

                @pl.when(par == 0)
                def _():
                    pair_copy(awq_h, awq, sem_aq, i).wait()
                    wo_copy(awo_h, awo, sem_ao, i).wait()

                @pl.when((par == 1) & (i + 1 < NP))
                def _():
                    pair_copy(awk_h, awk, sem_ak, i + 1).wait()
                    pair_copy(awv_h, awv, sem_av, i + 1).wait()

                @pl.when(h == 1)
                def _():
                    cp_bx.wait()

                @pl.when(h == H - NG)
                def _():
                    cp_ckv.wait()

                @pl.when(h >= H - NG)
                def _():
                    g = h - (H - NG)
                    keep_terms(ckv, g, _bf(craw[_half(g * GB, GB), :]))
                wk, wv = weight_terms(PT * i + (2 + par) * HT), weight_terms(PT * i + (4 + par) * HT)
                for g in range(0, NG, G1):
                    for dst, terms in ((kx, wk), (vx, wv)):
                        project_rows(g, terms, [
                            store_blocks((dst, (h,), j * GB), (dst, (h,), j * GB + QB))
                            for j in range(g, g + G1)])
                    if g == 0:
                        w = _u32(jnp.concatenate([_bf(awo[h]), jnp.zeros((DP - DM, DH), BF16)], axis=0).T)
                        wo[_half(h * DH, DH), :] = w[:, :KM]
                        wo_t[_half(h * 128, 128), :] = w[:64, KM:] | pltpu.roll(w[64:, KM:], 64, 1)
                    if g == 2:
                        src = jnp.where(h == 0, NG - 1, NG + (h - 1) % NG)
                        keep_terms(bx, (h + NG - 1) % NG, transposed(xraw, src * GB, GB))
                    if g == 2:
                        keep(_unpack(awq[i], par), PT * i + par * HT)
                        accb[:, pl.ds(pl.multiple_of(h * XC, XC), XC)] = jnp.zeros((DM, XC), F32)
                    if g == 4:
                        keep_kv(jnp.minimum(h + 1, H - 1))
            cp_mem.wait()
            mem_s[...] = jnp.concatenate([mem0[...].astype(F32), jnp.zeros((M, DP - DM), F32)], axis=1)

        with jax.named_scope('phase1'):
            pl.run_scoped(phase1, packed(DM, 2 * S), packed(S, DC), pltpu.VMEM((M, DM), BF16),
                          *[pltpu.VMEM((NP, DM, DH), U32)] * 3)

        def chain_step(s, held):
            mem = mem_s[...]
            zero = s >> 10
            mt = mem[:, KM:]
            mtail = jnp.concatenate([mt, pltpu.roll(mt, 64, 1)], axis=0).astype(BF16)
            t = []
            for g in range(0, NP * PT, 8):
                for t0 in (g, g + 4):
                    acc = _zeros(s, (M, 512))
                    for k0 in range(0, KM, 128):
                        w = jnp.concatenate([wqkv[t0 + j + zero, _half(k0, 128), :] for j in range(4)], axis=1)
                        yield
                        acc = acc + _dot(mem[:, k0:k0 + 128], _bf(w))
                        yield
                    t += [acc[:, j * 128:(j + 1) * 128] for j in range(4)]
                w = jnp.concatenate([wqkv_t[g // 2 + j + zero] for j in range(4)], axis=1)
                yield
                d = _dot(mtail, _bf(w))
                for j in range(8):
                    t[g + j] = t[g + j] + d[(j % 2) * M:(j % 2 + 1) * M, (j // 2) * 128:(j // 2 + 1) * 128]
                yield
            for _ in range(2 * GAPS[0]):
                yield

            def head_rows(i, which, par):
                t0 = PT * i + (2 * which + par) * HT
                return jnp.concatenate(t[t0:t0 + HT], axis=1)

            def pair_rows(i, which):
                return jnp.concatenate([head_rows(i, which, 0), head_rows(i, which, 1)], axis=0)

            def window(ref, i, which):
                xr = _half(s * SEG, SEG)
                return jnp.concatenate([_bf(ref[2 * i, xr, :]), _bf(ref[2 * i + 1, xr, :]),
                                        pair_rows(i, which).astype(BF16)], axis=0)

            now = [[head_rows(h // 2, which, h % 2) for h in range(H)] for which in (1, 2)]
            if held:
                for ref, old, new in zip((km, vm), held.pop(), now):
                    for h in range(H):
                        _put(ref, (h,), (s - 1) * M, 0, jnp.concatenate([old[h], new[h]], axis=0))
            else:
                held.append(now)
            sc = []
            for i0 in range(0, NP, 2):
                ops = [((pair_rows(i, 0) * QSC).astype(BF16), window(kx, i, 1)) for i in (i0, i0 + 1)]
                yield
                sc += [_dot_nt(q, k) for q, k in ops]
                yield
            for _ in range(2 * GAPS[1]):
                yield
            sc = jnp.concatenate(sc, axis=0)
            par = (jax.lax.broadcasted_iota(jnp.int32, sc.shape, 0) // M) % 2
            ci = jax.lax.broadcasted_iota(jnp.int32, sc.shape, 1)
            own = jnp.where(ci < 2 * SEG, ci // SEG, (ci - 2 * SEG) // M) == par
            p = _softmax2(jnp.where(own, sc, NEG))
            zt = []
            for i0 in range(0, NP, 2):
                ops = [(p[2 * M * i:2 * M * (i + 1)], window(vx, i, 2)) for i in (i0, i0 + 1)]
                yield
                for pp, v in ops:
                    o = _dot(pp, v)
                    zt += [o[par * M:(par + 1) * M, j * 128:(j + 1) * 128] for par in range(2) for j in range(HT)]
                yield
            for _ in range(2 * GAPS[2]):
                yield
            acc = [_zeros(s, (M, 128))] * 3 + [_zeros(s, (2 * M, 128))]
            for g in range(0, H * HT, 8):
                for t0 in (g, g + 4):
                    zp = jnp.concatenate(zt[t0:t0 + 4], axis=1).astype(BF16).astype(F32)
                    for n in range(KM // 128):
                        w = wo[_half((t0 + zero) * 128, 512), n * 128:(n + 1) * 128]
                        yield
                        acc[n] = acc[n] + _dot(zp, _bf(w))
                        yield
                zp = jnp.concatenate([jnp.concatenate(zt[g:g + 8:2], axis=1),
                                      jnp.concatenate(zt[g + 1:g + 8:2], axis=1)], axis=0).astype(BF16)
                w = wo_t[_half((g // 2 + zero) * 128, 512), :]
                yield
                acc[3] = acc[3] + _dot(zp, _bf(w))
                yield
            lane = jax.lax.broadcasted_iota(jnp.int32, (M, 128), 1)
            last = jnp.where(lane < 64, acc[3][:M] + pltpu.roll(acc[3][M:], 64, 1), 0.0)
            mem_s[...] = jnp.concatenate(acc[:3] + [last], axis=1).astype(BF16).astype(F32)
            for _ in range(2 * GAPS[3]):
                yield

        def chain(h):
            held = []
            for j in range(STEPS):
                yield from chain_step(h * STEPS + j, held)

        n_chain = STEPS * ((NP * PT + H * HT) // 8 * 7 + NP + sum(GAPS))
        n_qk, n_v = 7 * (1 + QB // MBK), 7 * (QB // MBV)

        def split(r):
            return 2 if r >= PVR else 1

        def n_scores(r):
            return (r + 2) // 2

        def n_context(r):
            return (r + 1) // 2 * split(r) + (r + 1) % 2

        n_head = (NG * (n_qk + n_v) + (NG // 2) * 7 - (S // QB // 2 - 1)
                  + sum(n_scores(r) + n_context(r) for r in range(S // QB)))

        def phase2(wq_s, wk_s, wv_s, wo_s, k_s, v_s):
            def b_head(h):
                i = h // 2
                par = h % 2
                for w_s, raw in ((wq_s, bwq), (wk_s, bwk), (wv_s, bwv)):
                    for n, term in enumerate(_rhs_terms(_unpack(raw[i], par), 2 * w_s.shape[1])):
                        _put(w_s, (n,), 0, 0, term)
                for n, term in enumerate(_lhs_terms(_bf(bwo[h]).astype(F32))):
                    _put(wo_s, (n,), 0, 0, term)
                qs, ss, ms, ctxs = {}, {}, {}, {}

                def chunks(r):
                    nk = (r + 1) * QB
                    return [(c0, min(c0 + 256, nk)) for c0 in range(0, nk, 256)]

                def project(g, r0, src, w_s, depth, mb, together, finish):
                    def product(n):
                        k = depth - 2 * w_s.shape[1] if n in (4, 5) else 2 * w_s.shape[1]
                        xs = [_bf(src[n, _half(g * QB + r0 + j * mb, mb), :])[:, :k] for j in range(together)]
                        w = _bf(w_s[n, _half(0, k), :])
                        return lambda: jnp.concatenate([_dot(x, w) for x in xs], axis=0)
                    return _block_product(product, finish)

                def project_qk(g):
                    q = {}
                    yield from project(g, 0, bx, wq_s, DM, QB // 2, 2, query_blocks(q))
                    for a in range(2):
                        qs[2 * g + a] = jnp.concatenate([q[a, 0], q[a, 1]], axis=1)
                    for r0 in range(0, QB, MBK):
                        yield from project(g, r0, ckv, wk_s, DC, MBK, 1, store_blocks((k_s[2 * g], (), r0), (k_s[2 * g + 1], (), r0)))

                def project_v(g):
                    for r0 in range(0, QB, MBV):
                        yield from project(g, r0, ckv, wv_s, DC, MBV, 1, store_blocks((v_s[2 * g], (), r0), (v_s[2 * g + 1], (), r0)))

                def blocks(refs, c0, c1):
                    return _bf(jnp.concatenate([refs[j][...] for j in range(c0 // QB, c1 // QB)], axis=0))

                def scores(r):
                    ss[r] = []
                    m = None
                    for c0, c1 in chunks(r):
                        k = blocks(k_s, c0, c1)
                        yield
                        sc = _dot_nt(qs[r], k)
                        if c1 == (r + 1) * QB:
                            ri = jax.lax.broadcasted_iota(jnp.int32, sc.shape, 0) + r * QB
                            ci = jax.lax.broadcasted_iota(jnp.int32, sc.shape, 1) + c0
                            sc = jnp.where(ci <= ri, sc, NEG)
                        ss[r].append(sc)
                        for t0 in range(0, c1 - c0, 128):
                            m = sc[:, t0:t0 + 128] if m is None else jnp.maximum(m, sc[:, t0:t0 + 128])
                        if c1 == (r + 1) * QB:
                            ms[r] = jnp.max(m, axis=1, keepdims=True)
                        yield

                def context(r):
                    ls = []

                    def weights(c):
                        p = jnp.exp2(ss[r][c] - ms[r])
                        for t0 in range(0, p.shape[1], 128):
                            ls[:] = [p[:, t0:t0 + 128] + ls[0] if ls else p[:, t0:t0 + 128]]
                        return p.astype(BF16)

                    acc = _zeros(h, (QB, DH))
                    nxt = weights(0)
                    for c, (c0, c1) in enumerate(chunks(r)):
                        mb = QB // split(r) if c1 - c0 == 256 else QB
                        p = nxt
                        v = blocks(v_s, c0, c1)
                        new = []
                        for r0 in range(0, QB, mb):
                            yield
                            new.append(acc[r0:r0 + mb] + _dot(p[r0:r0 + mb], v))
                            if r0 == 0 and c1 < (r + 1) * QB:
                                nxt = weights(c + 1)
                            if r0 + mb == QB:
                                acc = jnp.concatenate(new, axis=0)
                                if c1 == (r + 1) * QB:
                                    ctxs[r] = acc / jnp.sum(ls[0], axis=1, keepdims=True)
                                    if r % 2:
                                        ctxs[r] = context_terms(jnp.concatenate([ctxs[r - 1], ctxs[r]], axis=0))
                            yield

                def output(r):
                    yield from add_output(accb, (r - 3) * QB, lambda n, r0, m: _bf(wo_s[n, _half(r0, m), :]),
                                          (ctxs[r - 2], ctxs[r]), 2)

                def both(r):
                    a, b = scores(r), context(r - 2)
                    na, nc = n_scores(r) - 1, n_context(r - 2) - 1
                    for j in _order([na, nc]):
                        for _ in range(2):
                            next((a, b)[j])
                            yield
                    for _ in range(2):
                        next(a)
                        next(b)
                        yield
                    _finish([a, b])

                nb = S // QB
                for r in range(nb + 4):
                    parts = []
                    if r < nb:
                        parts.append((project_v(r // 2), n_v) if r % 2 else (project_qk(r // 2), n_qk))
                    if 0 <= r - 4 < nb and (r - 4) % 4 == 3:
                        parts.append((output(r - 4), 7))
                    if r % 2 == 1 and 3 <= r <= nb:
                        parts.append((both(r - 1), n_scores(r - 1) + n_context(r - 3) - 1))
                    else:
                        if 0 <= r - 1 < nb:
                            parts.append((scores(r - 1), n_scores(r - 1)))
                        if 0 <= r - 3 < nb:
                            parts.append((context(r - 3), n_context(r - 3)))
                    yield from _merge(*parts)

            def b_body(h, c):
                i = h // 2

                @pl.when(h % 2 == 0)
                def _():
                    pair_copy(bwq_h, bwq, sem_bq, i).wait()
                    pair_copy(bwk_h, bwk, sem_bk, i).wait()
                    pair_copy(bwv_h, bwv, sem_bv, i).wait()
                    wo_copy(bwo_h, bwo, sem_bo, i).wait()
                for _ in _merge((chain(h), n_chain), (b_head(h), n_head)):
                    pass
                return c
            jax.lax.fori_loop(0, H, b_body, 0)

        with jax.named_scope('phase2'):
            pl.run_scoped(phase2, packed(7, DP // 2, DH // 2), packed(7, DC // 2, DH // 2), packed(7, DC // 2, DH // 2),
                          packed(7, DM // 2, DH // 2), [packed(QB, DH)] * (S // QB), [packed(QB, DH)] * (S // QB))

        def phase3(acca, left, right, q0):
            ri = jax.lax.broadcasted_iota(jnp.int32, (AB, AB + 2 * M), 0)
            ci = jax.lax.broadcasted_iota(jnp.int32, (AB, AB + 2 * M), 1)
            amask = (((ci < AB) & ((ci // SEG) == (ri // SEG)) & (ci <= ri))
                     | ((ci >= AB) & (((ci - AB) // M) == (ri // SEG))))

            def out_copy(stage, row, n, col, sem):
                rows = _half(row, n)
                return pltpu.make_async_copy(
                    stage.at[rows, :], out_h.bitcast(U32).at[0, rows, pl.ds(col, stage.shape[1])], sem)

            def left_copy(r):
                return out_copy(left, r * GB, GB, 0, sem_l.at[r])

            def right_copy(h):
                return out_copy(right, h * XC, XC, DP, sem_r.at[h])

            def query_weight(h):
                return weight_terms(PT * (h // 2) + (h % 2) * HT)

            def query(wq, r):
                qs = [{} for _ in range(RB // GB)]
                for j in range(0, RB // GB, G3):
                    project_rows(r * RB // GB + j, wq, [query_blocks(q) for q in qs[j:j + G3]])
                return jnp.concatenate([jnp.concatenate([q[a, 0], q[a, 1]], axis=1)
                                        for q in qs for a in range(2)], axis=0)

            def a_head(h):
                wq = query_weight(h)
                wt = [t.astype(BF16) for t in _lhs_terms(_bf(awo[h]).astype(F32))]
                qs, ps, ctxs = {0: _bf(q0[...])}, {}, {}

                def project(r):
                    qs[r] = query(wq, r)

                def window(xref, mref, j):
                    return _bf(jnp.concatenate([xref[h, _half(j * AB, AB), :],
                                                mref[h, _half(j * 2 * M, 2 * M), :]], axis=0))

                def scores(r):
                    ps[r] = []
                    for j in range(RB // AB):
                        sc = _dot_nt(qs[r][j * AB:(j + 1) * AB], window(kx, km, r * RB // AB + j))
                        ps[r].append(_softmax2(jnp.where(amask, sc, NEG)))

                def context(r):
                    ctx = jnp.concatenate(
                        [_dot(p, window(vx, vm, r * RB // AB + j)) for j, p in enumerate(ps[r])], axis=0)
                    ctxs[r] = [context_terms(ctx[:GB]), context_terms(ctx[GB:])]

                def output(r):
                    for _ in add_output(acca, r * RB, lambda n, r0, m: wt[n], ctxs[r], 1, h > 0):
                        pass

                nr = S // RB
                project(1)
                right[_half(h * XC, XC), :] = _u32(
                    accb[DP - DM:, pl.ds(pl.multiple_of(h * XC, XC), XC)].astype(BF16).T)
                for r in range(nr):
                    scores(r)
                    if r > 0:
                        output(r - 1)
                    if r + 2 < nr:
                        project(r + 2)
                    context(r)
                _put(q0, (), 0, 0, query(query_weight(jnp.minimum(h + 1, H - 1)), 0))
                output(nr - 1)
                right_copy(h).start()

            _put(q0, (), 0, 0, query(query_weight(0), 0))
            pl.loop(0, H)(a_head)

            @pl.loop(0, NG)
            def _(r):
                cols = pl.ds(pl.multiple_of(r * GB, GB), GB)
                left[_half(r * GB, GB), :] = _u32(
                    jnp.concatenate([acca[:, cols], accb[:DP - DM, cols]], axis=0).astype(BF16).T)
                left_copy(r).start()

            pl.loop(0, H)(lambda h: right_copy(h).wait())
            pl.loop(0, NG)(lambda r: left_copy(r).wait())

        with jax.named_scope('phase3'):
            pl.run_scoped(phase3, pltpu.VMEM((DM, S), F32), packed(S, DP), packed(S, 2 * DM - DP), packed(RB, DH))

    scratch = [
        packed(7, S // 2, DP // 2),
        pltpu.VMEM((M, DP), F32),
        packed(H, DM, DH),
        packed(NP * PT, KM, 128),
        packed(NP * PT // 2, 128, 128),
        packed(H * DH, KM),
        packed(H * DH // 2, 128),
        packed(H, S, DH),
        packed(H, S, DH),
        packed(H, NSEG * M, DH),
        packed(H, NSEG * M, DH),
        packed(7, S // 2, DP // 2),
        packed(7, S // 2, DC // 2),
        pltpu.VMEM((NP, DM, DH), U32),
        pltpu.VMEM((NP, DC, DH), U32),
        pltpu.VMEM((NP, DC, DH), U32),
        packed(H, DM, DH),
        pltpu.VMEM((DM, S), F32),
        pltpu.SemaphoreType.DMA((3 + S // RB,)),
    ] + [pltpu.SemaphoreType.DMA((NP,)) for _ in range(8)] + [pltpu.SemaphoreType.DMA((NG,)), pltpu.SemaphoreType.DMA((H,))]
    return kernel, scratch


@jax.jit
def pallas_concat_heads__memory_aug_recurrent_mem_tr__compressed_kv_cla__prompt_kernel(
    A_x, A_mem0, A_Wq, A_Wk, A_Wv, A_Wo, A_seg_len, B_x, B_c_kv, B_w_q, B_w_uk, B_w_uv, B_w_o,
):
    del A_seg_len
    _, S, DM = A_x.shape
    M = A_mem0.shape[1]
    H, DH = A_Wq.shape[1], A_Wq.shape[2]
    DC = B_c_kv.shape[2]
    kernel, scratch = _make_kernel(S, DM, H, DH, M, 32, DC)
    return pl.pallas_call(
        kernel,
        out_shape=jax.ShapeDtypeStruct((1, S, 2 * DM), BF16),
        in_specs=[pl.BlockSpec(memory_space=pl.ANY)] * 12,
        out_specs=pl.BlockSpec(memory_space=pl.ANY),
        scratch_shapes=scratch,
        compiler_params=pltpu.CompilerParams(vmem_limit_bytes=126 * 1024 * 1024),
    )(A_x[0].T, A_mem0, A_Wq, A_Wk, A_Wv, A_Wo.transpose(0, 2, 1),
      B_x[0].T, B_c_kv, B_w_q, B_w_uk, B_w_uv, B_w_o.transpose(0, 2, 1))
```

```python
import functools

import jax
import jax.numpy as jnp
import jax.experimental.pallas as pl
import jax.experimental.pallas.tpu as pltpu

F32 = jnp.float32
BF16 = jnp.bfloat16
U32 = jnp.uint32
LOG2E = 1.4426950408889634
NEG = -1e30
NN = (((1,), (0,)), ((), ()))
NT = (((1,), (1,)), ((), ()))


def _dot(a, b):
    return jax.lax.dot_general(a, b, NN, preferred_element_type=F32)


def _dot_nt(a, b):
    return jax.lax.dot_general(a, b, NT, preferred_element_type=F32)


def _bf(u):
    return pltpu.bitcast(u, BF16)


def _u32(x):
    return pltpu.bitcast(x.astype(BF16), U32)


def _half(start, size):
    if isinstance(start, int):
        return pl.ds(start // 2, size // 2)
    return pl.ds(pl.multiple_of(start // 2, 8), size // 2)


def _unpack(u, parity):
    if isinstance(parity, int):
        w = (u << 16) if parity == 0 else (u & jnp.uint32(0xFFFF0000))
    else:
        w = (u >> (16 * parity).astype(U32)) << 16
    return pltpu.bitcast(w, F32).astype(BF16)


def _zeros(i, shape):
    return jnp.full(shape, (i >> 10).astype(F32))


def _softmax2(sc):
    p = jnp.exp2(sc - jnp.max(sc, axis=1, keepdims=True))
    return (p / jnp.sum(p, axis=1, keepdims=True)).astype(BF16)


def _order(counts):
    done = [0] * len(counts)
    live = [a for a, n in enumerate(counts) if n > 0]
    order = []
    for _ in range(sum(counts)):
        j = min(live, key=lambda a: ((done[a] + 0.5) / counts[a], a))
        done[j] += 1
        order.append(j)
    return order


def _finish(gens):
    for g in gens:
        for _ in g:
            raise AssertionError("stream longer than announced")


def _merge(*streams):
    for j in _order([n for _, n in streams]):
        for _ in range(2):
            next(streams[j][0])
            yield
    _finish([g for g, _ in streams])


def _make_kernel(S, DM, H, DH, M, SEG, DC):
    NP = H // 2
    NSEG = S // SEG
    DP = 512
    KM = DM // 128 * 128
    HT = DH // 128
    PT = 6 * HT
    STEPS = NSEG // H
    QB = 128
    OB = DM // 4
    PVR = 5
    MBQ, MBK, MBV = 128, 64, 64
    GAPS = (2, 3, 2, 2)
    RB = 512
    OUT = 256
    XC = S // H
    AB = 2 * SEG
    QSC = LOG2E * DH ** -0.5
    assert DM + 64 == DP and DH == 256 and M == 8 and H % 2 == 0 and DC % 256 == 0
    assert SEG % 16 == 0 and RB % AB == 0 and AB + 2 * M <= 128 and STEPS % 2 == 0
    assert S == H * STEPS * SEG and S % (2 * RB) == 0 and XC % 128 == 0 and NSEG < 1024

    def packed(*shape):
        return pltpu.VMEM(shape[:-2] + (shape[-2] // 2, shape[-1]), U32)

    def kernel(ax_h, mem_h, awq_h, awk_h, awv_h, awo_h, bx_h, ckv_h, bwq_h, bwk_h, bwv_h, bwo_h,
               out_h,
               ax, mem_s, awo, wqkv, wqkv_t, wo, wo_t, kx, vx, km, vm,
               bx, ckv, bwq, bwk, bwv, bwo, accb,
               sem_x, sem_aq, sem_ak, sem_av, sem_ao, sem_bq, sem_bk, sem_bv, sem_bo, sem_l, sem_r):

        def pair_copy(src, dst, sem, i):
            return pltpu.make_async_copy(src.bitcast(U32).at[:, i, :], dst.at[i], sem.at[i])

        def wo_copy(src, dst, sem, i):
            return pltpu.make_async_copy(src.bitcast(U32).at[pl.ds(2 * i, 2)], dst.at[pl.ds(2 * i, 2)], sem.at[i])

        def head_weight(t):
            return _bf(jnp.concatenate(
                [jnp.concatenate([wqkv[t + j], wqkv_t[t // 2 + j // 2, _half((j % 2) * 64, 64), :]], axis=0)
                 for j in range(HT)], axis=1))

        def transposed(raw, c, n):
            xt = _bf(raw[:, pl.ds(c if isinstance(c, int) else pl.multiple_of(c, n), n)])
            return _u32(jnp.concatenate([xt, jnp.zeros((DP - DM, n), BF16)], axis=0).T)

        def phase1(xraw, mem0, awq, awk, awv):
            def cp_ax(r):
                cols = pl.ds(r * RB if isinstance(r, int) else pl.multiple_of(r * RB, RB), RB)
                return pltpu.make_async_copy(ax_h.bitcast(U32).at[:, cols], xraw.at[:, cols], sem_x.at[3 + r])

            cp_mem = pltpu.make_async_copy(mem_h.at[0], mem0, sem_x.at[0])
            cp_bx = pltpu.make_async_copy(bx_h.bitcast(U32), xraw.at[:, pl.ds(S, S)], sem_x.at[1])
            cp_ckv = pltpu.make_async_copy(ckv_h.bitcast(U32).at[0], ckv, sem_x.at[2])

            def a_weights(i):
                pair_copy(awk_h, awk, sem_ak, i).start()
                pair_copy(awv_h, awv, sem_av, i).start()
                pair_copy(awq_h, awq, sem_aq, i).start()
                wo_copy(awo_h, awo, sem_ao, i).start()

            def b_weights(i):
                pair_copy(bwq_h, bwq, sem_bq, i).start()
                pair_copy(bwk_h, bwk, sem_bk, i).start()
                pair_copy(bwv_h, bwv, sem_bv, i).start()
                wo_copy(bwo_h, bwo, sem_bo, i).start()

            for r in range(S // RB):
                cp_ax(r).start()
            pair_copy(awk_h, awk, sem_ak, 0).start()
            pair_copy(awv_h, awv, sem_av, 0).start()

            def keep(w, t):
                u = _u32(w)
                for j in range(HT):
                    wqkv[t + j] = u[:KM // 2, j * 128:(j + 1) * 128]
                    wqkv_t[t // 2 + j // 2, _half((j % 2) * 64, 64), :] = u[KM // 2:, j * 128:(j + 1) * 128]

            def keep_kv(h):
                i = h // 2
                keep(_unpack(awk[i], h % 2), PT * i + (2 + h % 2) * HT)
                keep(_unpack(awv[i], h % 2), PT * i + (4 + h % 2) * HT)

            def keep_bx(j):
                bx[_half(j * XC, XC), :] = transposed(xraw, S + (j - 1) * XC, XC)

            @pl.loop(0, S // RB)
            def _(r):
                cp_ax(r).wait()
                for j in range(0, RB, 256):
                    ax[_half(r * RB + j, 256), :] = transposed(xraw, r * RB + j, 256)
            pair_copy(awq_h, awq, sem_aq, 0).start()
            wo_copy(awo_h, awo, sem_ao, 0).start()
            pair_copy(awk_h, awk, sem_ak, 0).wait()
            pair_copy(awv_h, awv, sem_av, 0).wait()
            keep_kv(0)
            cp_bx.start()
            cp_mem.start()
            pl.loop(1, NP)(a_weights)
            cp_ckv.start()
            pl.loop(0, NP)(b_weights)

            @pl.loop(0, H)
            def _(h):
                i = h // 2
                par = h % 2

                @pl.when(par == 0)
                def _():
                    pair_copy(awq_h, awq, sem_aq, i).wait()
                    wo_copy(awo_h, awo, sem_ao, i).wait()

                @pl.when((par == 1) & (i + 1 < NP))
                def _():
                    pair_copy(awk_h, awk, sem_ak, i + 1).wait()
                    pair_copy(awv_h, awv, sem_av, i + 1).wait()

                @pl.when(h == 1)
                def _():
                    cp_bx.wait()
                wk, wv = head_weight(PT * i + (2 + par) * HT), head_weight(PT * i + (4 + par) * HT)
                for r in range(S // RB):
                    rows = _half(r * RB, RB)
                    x = _bf(ax[rows, :])[:, :DM]
                    kx[h, rows, :] = _u32(_dot(x, wk))
                    vx[h, rows, :] = _u32(_dot(x, wv))
                    if r == 0:
                        w = _u32(jnp.concatenate([_bf(awo[h]), jnp.zeros((DP - DM, DH), BF16)], axis=0).T)
                        wo[_half(h * DH, DH), :] = w[:, :KM]
                        wo_t[_half(h * 128, 128), :] = w[:64, KM:] | pltpu.roll(w[64:, KM:], 64, 1)
                        keep_bx(h)
                    if r == 1:
                        keep(_unpack(awq[i], par), PT * i + par * HT)
                        accb[:, pl.ds(pl.multiple_of(h * XC, XC), XC)] = jnp.zeros((DM, XC), F32)
                    if r == 2:
                        keep_kv(jnp.minimum(h + 1, H - 1))
            keep_bx(H)
            cp_mem.wait()
            mem_s[...] = jnp.concatenate([mem0[...].astype(F32), jnp.zeros((M, DP - DM), F32)], axis=1)
            cp_ckv.wait()

        with jax.named_scope('phase1'):
            pl.run_scoped(phase1, packed(DM, 2 * S), pltpu.VMEM((M, DM), BF16),
                          *[pltpu.VMEM((NP, DM, DH), U32)] * 3)

        def chain_step(s, held):
            mem = mem_s[...]
            zero = s >> 10
            mt = mem[:, KM:]
            mtail = jnp.concatenate([mt, pltpu.roll(mt, 64, 1)], axis=0).astype(BF16)
            t = []
            for g in range(0, NP * PT, 8):
                for t0 in (g, g + 4):
                    acc = _zeros(s, (M, 512))
                    for k0 in range(0, KM, 128):
                        w = jnp.concatenate([wqkv[t0 + j + zero, _half(k0, 128), :] for j in range(4)], axis=1)
                        yield
                        acc = acc + _dot(mem[:, k0:k0 + 128], _bf(w))
                        yield
                    t += [acc[:, j * 128:(j + 1) * 128] for j in range(4)]
                w = jnp.concatenate([wqkv_t[g // 2 + j + zero] for j in range(4)], axis=1)
                yield
                d = _dot(mtail, _bf(w))
                for j in range(8):
                    t[g + j] = t[g + j] + d[(j % 2) * M:(j % 2 + 1) * M, (j // 2) * 128:(j // 2 + 1) * 128]
                yield
            for _ in range(2 * GAPS[0]):
                yield

            def head_rows(i, which, par):
                t0 = PT * i + (2 * which + par) * HT
                return jnp.concatenate(t[t0:t0 + HT], axis=1)

            def pair_rows(i, which):
                return jnp.concatenate([head_rows(i, which, 0), head_rows(i, which, 1)], axis=0)

            def window(ref, i, which):
                xr = _half(s * SEG, SEG)
                return jnp.concatenate([_bf(ref[2 * i, xr, :]), _bf(ref[2 * i + 1, xr, :]),
                                        pair_rows(i, which).astype(BF16)], axis=0)

            now = [[head_rows(h // 2, which, h % 2) for h in range(H)] for which in (1, 2)]
            if held:
                for ref, old, new in zip((km, vm), held.pop(), now):
                    for h in range(H):
                        ref[h, _half((s - 1) * M, 2 * M), :] = _u32(jnp.concatenate([old[h], new[h]], axis=0))
            else:
                held.append(now)
            sc = []
            for i0 in range(0, NP, 2):
                ops = [((pair_rows(i, 0) * QSC).astype(BF16), window(kx, i, 1)) for i in (i0, i0 + 1)]
                yield
                sc += [_dot_nt(q, k) for q, k in ops]
                yield
            for _ in range(2 * GAPS[1]):
                yield
            sc = jnp.concatenate(sc, axis=0)
            par = (jax.lax.broadcasted_iota(jnp.int32, sc.shape, 0) // M) % 2
            ci = jax.lax.broadcasted_iota(jnp.int32, sc.shape, 1)
            own = jnp.where(ci < 2 * SEG, ci // SEG, (ci - 2 * SEG) // M) == par
            p = _softmax2(jnp.where(own, sc, NEG))
            zt = []
            for i0 in range(0, NP, 2):
                ops = [(p[2 * M * i:2 * M * (i + 1)], window(vx, i, 2)) for i in (i0, i0 + 1)]
                yield
                for pp, v in ops:
                    o = _dot(pp, v)
                    zt += [o[par * M:(par + 1) * M, j * 128:(j + 1) * 128] for par in range(2) for j in range(HT)]
                yield
            for _ in range(2 * GAPS[2]):
                yield
            acc = [_zeros(s, (M, 128))] * 3 + [_zeros(s, (2 * M, 128))]
            for g in range(0, H * HT, 8):
                for t0 in (g, g + 4):
                    zp = jnp.concatenate(zt[t0:t0 + 4], axis=1).astype(BF16).astype(F32)
                    for n in range(KM // 128):
                        w = wo[_half((t0 + zero) * 128, 512), n * 128:(n + 1) * 128]
                        yield
                        acc[n] = acc[n] + _dot(zp, _bf(w))
                        yield
                zp = jnp.concatenate([jnp.concatenate(zt[g:g + 8:2], axis=1),
                                      jnp.concatenate(zt[g + 1:g + 8:2], axis=1)], axis=0).astype(BF16)
                w = wo_t[_half((g // 2 + zero) * 128, 512), :]
                yield
                acc[3] = acc[3] + _dot(zp, _bf(w))
                yield
            lane = jax.lax.broadcasted_iota(jnp.int32, (M, 128), 1)
            last = jnp.where(lane < 64, acc[3][:M] + pltpu.roll(acc[3][M:], 64, 1), 0.0)
            mem_s[...] = jnp.concatenate(acc[:3] + [last], axis=1).astype(BF16).astype(F32)
            for _ in range(2 * GAPS[3]):
                yield

        def chain(h):
            held = []
            for j in range(STEPS):
                yield from chain_step(h * STEPS + j, held)

        n_chain = STEPS * ((NP * PT + H * HT) // 8 * 7 + NP + sum(GAPS))
        n_proj = 2 * (QB // MBQ) + (DC // 256) * (QB // MBK + QB // MBV)

        def split(r):
            return 2 if r >= PVR else 1

        def n_scores(r):
            return (r + 2) // 2

        def n_context(r):
            return (r + 1) // 2 * split(r) + (r + 1) % 2

        n_head = ((S // QB) * n_proj + (S // QB // 2) * (DM // OB) - (S // QB // 2 - 1)
                  + sum(n_scores(r) + n_context(r) for r in range(S // QB)))

        def phase2(wq_s, wk_s, wv_s, k_s, v_s):
            def b_head(h):
                i = h // 2
                par = h % 2
                wq_s[...] = _u32(_unpack(bwq[i], par))
                wk_s[...] = _u32(_unpack(bwk[i], par))
                wv_s[...] = _u32(_unpack(bwv[i], par))
                qs, ss, ms, ctxs = {}, {}, {}, {}

                def chunks(r):
                    nk = (r + 1) * QB
                    return [(c0, min(c0 + 256, nk)) for c0 in range(0, nk, 256)]

                def project(r):
                    qp = []
                    for r0 in range(r * QB, (r + 1) * QB, MBQ):
                        acc = _zeros(h, (MBQ, DH))
                        for k0, k1 in ((0, 256), (256, DM)):
                            x = _bf(bx[_half(XC + r0, MBQ), k0:k0 + 256])[:, :k1 - k0]
                            w = _bf(wq_s[_half(k0, k1 - k0), :])
                            yield
                            acc = acc + _dot(x, w)
                            if k1 == DM:
                                qp.append((acc * QSC).astype(BF16))
                                qs[r] = jnp.concatenate(qp, axis=0)
                            yield
                    for w_s, dst, mb in ((wk_s, k_s, MBK), (wv_s, v_s, MBV)):
                        got = []
                        for r0 in range(r * QB, (r + 1) * QB, mb):
                            rows = _half(r0, mb)
                            acc = _zeros(h, (mb, DH))
                            for k0 in range(0, DC, 256):
                                x = _bf(ckv[rows, k0:k0 + 256])
                                w = _bf(w_s[_half(k0, 256), :])
                                yield
                                acc = acc + _dot(x, w)
                                if k0 + 256 == DC:
                                    got.append(acc.astype(BF16))
                                    if len(got) * mb == QB:
                                        blk = jnp.concatenate(got, axis=0)
                                        dst[r][...] = _u32(blk)
                                yield

                def blocks(refs, c0, c1):
                    return _bf(jnp.concatenate([refs[j][...] for j in range(c0 // QB, c1 // QB)], axis=0))

                def scores(r):
                    ss[r] = []
                    m = None
                    for c0, c1 in chunks(r):
                        k = blocks(k_s, c0, c1)
                        yield
                        sc = _dot_nt(qs[r], k)
                        if c1 == (r + 1) * QB:
                            ri = jax.lax.broadcasted_iota(jnp.int32, sc.shape, 0) + r * QB
                            ci = jax.lax.broadcasted_iota(jnp.int32, sc.shape, 1) + c0
                            sc = jnp.where(ci <= ri, sc, NEG)
                        ss[r].append(sc)
                        for t0 in range(0, c1 - c0, 128):
                            m = sc[:, t0:t0 + 128] if m is None else jnp.maximum(m, sc[:, t0:t0 + 128])
                        if c1 == (r + 1) * QB:
                            ms[r] = jnp.max(m, axis=1, keepdims=True)
                        yield

                def context(r):
                    ls = []

                    def weights(c):
                        p = jnp.exp2(ss[r][c] - ms[r])
                        for t0 in range(0, p.shape[1], 128):
                            ls[:] = [p[:, t0:t0 + 128] + ls[0] if ls else p[:, t0:t0 + 128]]
                        return p.astype(BF16)

                    acc = _zeros(h, (QB, DH))
                    nxt = weights(0)
                    for c, (c0, c1) in enumerate(chunks(r)):
                        mb = QB // split(r) if c1 - c0 == 256 else QB
                        p = nxt
                        v = blocks(v_s, c0, c1)
                        new = []
                        for r0 in range(0, QB, mb):
                            yield
                            new.append(acc[r0:r0 + mb] + _dot(p[r0:r0 + mb], v))
                            if r0 == 0 and c1 < (r + 1) * QB:
                                nxt = weights(c + 1)
                            if r0 + mb == QB:
                                acc = jnp.concatenate(new, axis=0)
                                if c1 == (r + 1) * QB:
                                    ctxs[r] = (acc / jnp.sum(ls[0], axis=1, keepdims=True)).astype(BF16)
                            yield

                def output(r):
                    ctx = jnp.concatenate([ctxs[r - 1], ctxs[r]], axis=0)
                    cols = pl.ds((r - 1) * QB, 2 * QB)
                    for n0 in range(0, DM, OB):
                        w = _bf(bwo[h, _half(n0, OB), :])
                        yield
                        accb[n0:n0 + OB, cols] += _dot_nt(w, ctx)
                        yield

                def both(r):
                    a, b = scores(r), context(r - 2)
                    na, nc = n_scores(r) - 1, n_context(r - 2) - 1
                    for j in _order([na, nc]):
                        for _ in range(2):
                            next((a, b)[j])
                            yield
                    for _ in range(2):
                        next(a)
                        next(b)
                        yield
                    _finish([a, b])

                nb = S // QB
                for r in range(nb + 4):
                    parts = []
                    if r < nb:
                        parts.append((project(r), n_proj))
                    if 0 <= r - 4 < nb and (r - 4) % 2 == 1:
                        parts.append((output(r - 4), DM // OB))
                    if r % 2 == 1 and 3 <= r <= nb:
                        parts.append((both(r - 1), n_scores(r - 1) + n_context(r - 3) - 1))
                    else:
                        if 0 <= r - 1 < nb:
                            parts.append((scores(r - 1), n_scores(r - 1)))
                        if 0 <= r - 3 < nb:
                            parts.append((context(r - 3), n_context(r - 3)))
                    yield from _merge(*parts)

            def b_body(h, c):
                i = h // 2

                @pl.when(h % 2 == 0)
                def _():
                    pair_copy(bwq_h, bwq, sem_bq, i).wait()
                    pair_copy(bwk_h, bwk, sem_bk, i).wait()
                    pair_copy(bwv_h, bwv, sem_bv, i).wait()
                    wo_copy(bwo_h, bwo, sem_bo, i).wait()
                for _ in _merge((chain(h), n_chain), (b_head(h), n_head)):
                    pass
                return c
            jax.lax.fori_loop(0, H, b_body, 0)

        with jax.named_scope('phase2'):
            pl.run_scoped(phase2, packed(DM, DH), packed(DC, DH), packed(DC, DH), [packed(QB, DH)] * (S // QB), [packed(QB, DH)] * (S // QB))

        def phase3(acca, left, right, q0):
            ri = jax.lax.broadcasted_iota(jnp.int32, (AB, AB + 2 * M), 0)
            ci = jax.lax.broadcasted_iota(jnp.int32, (AB, AB + 2 * M), 1)
            amask = (((ci < AB) & ((ci // SEG) == (ri // SEG)) & (ci <= ri))
                     | ((ci >= AB) & (((ci - AB) // M) == (ri // SEG))))

            def out_copy(stage, row, n, col, sem):
                rows = _half(row, n)
                return pltpu.make_async_copy(
                    stage.at[rows, :], out_h.bitcast(U32).at[0, rows, pl.ds(col, stage.shape[1])], sem)

            def left_copy(r):
                return out_copy(left, r * OUT, OUT, 0, sem_l.at[r])

            def right_copy(h):
                return out_copy(right, h * XC, XC, DP, sem_r.at[h])

            def query_weight(h):
                return head_weight(PT * (h // 2) + (h % 2) * HT)

            def query(wq, r):
                return (_dot(_bf(ax[_half(r * RB, RB), :])[:, :DM], wq) * QSC).astype(BF16)

            def a_head(h):
                wq = query_weight(h)
                qs, ps, ctxs = {0: _bf(q0[...])}, {}, {}

                def project(r):
                    qs[r] = query(wq, r)

                def window(xref, mref, j):
                    return _bf(jnp.concatenate([xref[h, _half(j * AB, AB), :],
                                                mref[h, _half(j * 2 * M, 2 * M), :]], axis=0))

                def scores(r):
                    ps[r] = []
                    for j in range(RB // AB):
                        sc = _dot_nt(qs[r][j * AB:(j + 1) * AB], window(kx, km, r * RB // AB + j))
                        ps[r].append(_softmax2(jnp.where(amask, sc, NEG)))

                def context(r):
                    ctxs[r] = jnp.concatenate(
                        [_dot(p, window(vx, vm, r * RB // AB + j)).astype(BF16) for j, p in enumerate(ps[r])],
                        axis=0)

                def output(r, c0, c1):
                    cols = slice(r * RB + c0, r * RB + c1)
                    acca[:, cols] = jnp.where(h > 0, acca[:, cols], 0.0) + _dot_nt(_bf(awo[h]), ctxs[r][c0:c1])

                nr = S // RB
                project(1)
                right[_half(h * XC, XC), :] = _u32(
                    accb[DP - DM:, pl.ds(pl.multiple_of(h * XC, XC), XC)].astype(BF16).T)
                for r in range(nr):
                    scores(r)
                    if r > 0:
                        output(r - 1, 0, RB)
                    if r + 2 < nr:
                        project(r + 2)
                    context(r)
                q0[...] = _u32(query(query_weight(jnp.minimum(h + 1, H - 1)), 0))
                output(nr - 1, 0, RB)
                right_copy(h).start()

            q0[...] = _u32(query(query_weight(0), 0))
            pl.loop(0, H)(a_head)

            @pl.loop(0, S // OUT)
            def _(r):
                cols = pl.ds(pl.multiple_of(r * OUT, OUT), OUT)
                left[_half(r * OUT, OUT), :] = _u32(
                    jnp.concatenate([acca[:, cols], accb[:DP - DM, cols]], axis=0).astype(BF16).T)
                left_copy(r).start()

            pl.loop(0, H)(lambda h: right_copy(h).wait())
            pl.loop(0, S // OUT)(lambda r: left_copy(r).wait())

        with jax.named_scope('phase3'):
            pl.run_scoped(phase3, pltpu.VMEM((DM, S), F32), packed(S, DP), packed(S, 2 * DM - DP), packed(RB, DH))

    scratch = [
        packed(S, DP),
        pltpu.VMEM((M, DP), F32),
        packed(H, DM, DH),
        packed(NP * PT, KM, 128),
        packed(NP * PT // 2, 128, 128),
        packed(H * DH, KM),
        packed(H * DH // 2, 128),
        packed(H, S, DH),
        packed(H, S, DH),
        packed(H, NSEG * M, DH),
        packed(H, NSEG * M, DH),
        packed(XC + S, DP),
        packed(S, DC),
        pltpu.VMEM((NP, DM, DH), U32),
        pltpu.VMEM((NP, DC, DH), U32),
        pltpu.VMEM((NP, DC, DH), U32),
        packed(H, DM, DH),
        pltpu.VMEM((DM, S), F32),
        pltpu.SemaphoreType.DMA((3 + S // RB,)),
    ] + [pltpu.SemaphoreType.DMA((NP,)) for _ in range(8)] + [pltpu.SemaphoreType.DMA((S // OUT,)), pltpu.SemaphoreType.DMA((H,))]
    return kernel, scratch


@functools.partial(jax.jit, static_argnames=("A_seg_len",))
def pallas_concat_heads__memory_aug_recurrent_mem_tr__compressed_kv_cla__prompt_kernel(
    A_x, A_mem0, A_Wq, A_Wk, A_Wv, A_Wo, A_seg_len, B_x, B_c_kv, B_w_q, B_w_uk, B_w_uv, B_w_o,
):
    _, S, DM = A_x.shape
    M = A_mem0.shape[1]
    H, DH = A_Wq.shape[1], A_Wq.shape[2]
    DC = B_c_kv.shape[2]
    kernel, scratch = _make_kernel(S, DM, H, DH, M, int(A_seg_len), DC)
    return pl.pallas_call(
        kernel,
        out_shape=jax.ShapeDtypeStruct((1, S, 2 * DM), BF16),
        in_specs=[pl.BlockSpec(memory_space=pl.ANY)] * 12,
        out_specs=pl.BlockSpec(memory_space=pl.ANY),
        scratch_shapes=scratch,
        compiler_params=pltpu.CompilerParams(vmem_limit_bytes=126 * 1024 * 1024),
    )(A_x[0].T, A_mem0, A_Wq, A_Wk, A_Wv, A_Wo.transpose(0, 2, 1),
      B_x[0].T, B_c_kv, B_w_q, B_w_uk, B_w_uv, B_w_o.transpose(0, 2, 1))
```
